```python
import jax
import jax.numpy as jnp

def _softmax(x, axis=-1):
    return jax.nn.softmax(x, axis=axis)
def _gelu(x):
    return jax.nn.gelu(x, approximate=True)
def _silu(x):
    return jax.nn.silu(x)
def _sigmoid(x):
    return jax.nn.sigmoid(x)
def _layernorm(x, axis=-1, eps=1e-5):
    m = jnp.mean(x, axis=axis, keepdims=True)
    v = jnp.var(x, axis=axis, keepdims=True)
    return (x - m) / jnp.sqrt(v + eps)
def _scatter_add(tgt, idx, src, axis=0):
    return tgt.at[idx].add(src)
def _segment_sum(src, seg, n):
    return jax.ops.segment_sum(src, seg, n)
class _Rng:
    def __init__(self, key):
        self._k = key
    def _next(self):
        self._k, sub = jax.random.split(self._k)
        return sub
    def normal(self, shape):
        return jax.random.normal(self._next(), shape, dtype=jnp.bfloat16)
    def randint(self, lo, hi, shape):
        return jax.random.randint(self._next(), shape, lo, hi, dtype=jnp.int32)
    def uniform(self, shape, lo=0.0, hi=1.0):
        return jax.random.uniform(self._next(), shape, jnp.bfloat16, lo, hi)
    def permutation(self, n):
        return jax.random.permutation(self._next(), n)


kernel_name = 'concat_heads__ssm_conv_h3__sliding_local_dilated__prompt'

def setup_inputs():
    _rng = _Rng(jax.random.key(int.from_bytes(__import__("os").urandom(4), "little")))
    _w = (lambda a: (lambda t: t.astype(jnp.bfloat16) if jnp.issubdtype(t.dtype, jnp.floating) else t)(jnp.asarray(a)))
    def _A_setup():
        B, S, D = 1, 2048, 1024
        ks = 4
        return {
            "q": _w((lambda *s: _rng.normal(s) * 0.05)(B, S, D)),
            "k": _w((lambda *s: _rng.normal(s) * 0.05)(B, S, D)),
            "v": _w((lambda *s: _rng.normal(s) * 0.05)(B, S, D)),
            "shift_k": _w((lambda *s: _rng.normal(s) * 0.05)(D, ks) * 0.5),
            "ssm_k": _w((lambda *s: _rng.normal(s) * 0.05)(D, S) * (1.0 / S ** 0.5)),
            "ssm_D": _w((lambda *s: _rng.normal(s) * 0.05)(D)),
        }
    _A_in = _A_setup()

    def _B_setup():
        B, S, D = 1, 2048, 1024
        return {
            "x": _w((lambda *s: _rng.normal(s) * 0.05)(B, S, D)),
            "wqkv": _w((lambda *s: _rng.normal(s) * 0.05)(D, 3 * D)),
            "wo": _w((lambda *s: _rng.normal(s) * 0.05)(D, D)),
        }
    _B_in = _B_setup()

    return {
        "A_q": _A_in["q"],
        "A_k": _A_in["k"],
        "A_v": _A_in["v"],
        "A_shift_k": _A_in["shift_k"],
        "A_ssm_k": _A_in["ssm_k"],
        "A_ssm_D": _A_in["ssm_D"],
        "B_x": _B_in["x"],
        "B_wqkv": _B_in["wqkv"],
        "B_wo": _B_in["wo"],
    }

def reference(A_q, A_k, A_v, A_shift_k, A_ssm_k, A_ssm_D, B_x, B_wqkv, B_wo):
    def _A_ref(q, k, v, shift_k, ssm_k, ssm_D):
        B, S, D = q.shape
        ks = shift_k.shape[-1]
        k_pad = jnp.pad(k, ((0, 0), (ks - 1, 0), (0, 0)))
        k_shift = jnp.zeros_like(k)
        for t in range(ks):
            k_shift = k_shift + k_pad[:, t:t + S, :] * shift_k[:, ks - 1 - t][None, None, :]
        kv = k_shift * v
        L = 2 * S
        kv_pad = jnp.pad(kv, ((0, 0), (0, S), (0, 0)))
        kf_pad = jnp.pad(ssm_k, ((0, 0), (0, S)))
        kv_f = (lambda x, axes=(-2,-1): jnp.fft.rfft2(x.astype(jnp.float32), axes=axes))(kv_pad[:, None, :, :], axes=(1, 2))
        kf_f = (lambda x, axes=(-2,-1): jnp.fft.rfft2(x.astype(jnp.float32), axes=axes))(kf_pad[:, None, :], axes=(1, 2))
        kf_f = (lambda x, *d: x.transpose(*d))(kf_f, 1, 2, 0)
        y_f = kv_f * kf_f[None, :, :, :]
        y = (lambda x, s, axes=(-2,-1): jnp.fft.irfft2(x, s=s, axes=axes).astype(jnp.bfloat16))(y_f, (1, L), axes=(1, 2))[:, 0, :S, :]
        y = y + kv * ssm_D[None, None, :]
        return q * y

    def _B_ref(x, wqkv, wo):
        B, S, D = x.shape
        H = 32; Dh = D // H
        W, dil = 8, 2
        qkv = (lambda x, *d: x.transpose(*d))((x @ wqkv).reshape(B, S, 3, H, Dh), 2, 0, 3, 1, 4)
        q, k, v = qkv[0], qkv[1], qkv[2]
        scale = Dh ** -0.5
        pos = jnp.arange(S)
        off = jnp.arange(W) * dil
        idx = pos[:, None] - off[None, :]
        mask = idx >= 0
        idx_c = jnp.where(mask, idx, 0).reshape(-1)
        kg = k[:, :, idx_c, :].reshape(B, H, S, W, Dh)
        vg = v[:, :, idx_c, :].reshape(B, H, S, W, Dh)
        logits = jnp.einsum("bhsd,bhswd->bhsw", q, kg) * scale
        logits = jnp.where(mask[None, None, :, :], logits, -1e9)
        attn = _softmax(logits, axis=-1)
        o = jnp.einsum("bhsw,bhswd->bhsd", attn, vg)
        return (lambda x, *d: x.transpose(*d))(o, 0, 2, 1, 3).reshape(B, S, D) @ wo

    a = _A_ref(A_q, A_k, A_v, A_shift_k, A_ssm_k, A_ssm_D)
    b = _B_ref(B_x, B_wqkv, B_wo)
    return jnp.concatenate([a, b], axis=-1)
```

```python
import numpy as np
import jax
import jax.numpy as jnp
from jax import lax
import jax.experimental.pallas as pl
import jax.experimental.pallas.tpu as pltpu

S = 2048
D = 1024
NG = D // 128
CH = 128
NCH = S // CH
TM = S // NG
HIST = 16
WIN, DIL, DH = 8, 2, 32
RT = 16
F32, BF16 = jnp.float32, jnp.bfloat16


def _dft_mats():
    k = np.concatenate([np.arange(0, CH, 2), np.arange(1, CH, 2)]).astype(np.float64)
    th = 2.0 * np.pi * (k + 0.5) / (2 * CH)
    ang = th[:, None] * np.arange(CH, dtype=np.float64)[None, :]
    fwd = np.concatenate([np.cos(ang), -np.sin(ang)], axis=0)
    inv = fwd.T / CH
    return jnp.asarray(fwd, BF16), jnp.asarray(inv, BF16)


def _permute_cols(w_ref, wp_ref):
    rows = 64
    lane = lax.broadcasted_iota(jnp.int32, (rows // 2, 128), 1)

    def body(i, carry):
        r0 = pl.multiple_of(i * rows, rows)
        for sec in range(3):
            v = [pltpu.bitcast(w_ref[pl.ds(r0, rows), sec * D + g * 128: sec * D + (g + 1) * 128], jnp.uint32)
                 for g in range(NG)]
            for st in range(3):
                gb, s = 1 << st, 2 << st
                bit = (lane & s) != 0
                for g in range(NG):
                    if g & gb:
                        continue
                    a, b = v[g], v[g + gb]
                    v[g] = jnp.where(bit, pltpu.roll(b, s, 1), a)
                    v[g + gb] = jnp.where(bit, b, pltpu.roll(a, 128 - s, 1))
            for g in range(NG):
                wp_ref[pl.ds(r0, rows), sec * D + g * 128: sec * D + (g + 1) * 128] = pltpu.bitcast(v[g], BF16)
        return carry

    lax.fori_loop(0, D // rows, body, 0)


def _permute_rows(wo_ref, tmp_ref, wop_ref):
    for g in range(NG):
        tmp_ref[g] = pltpu.bitcast(wo_ref[:, g * 128:(g + 1) * 128], jnp.uint32)
    for g in range(NG):
        for a in range(8):
            t = jnp.concatenate([tmp_ref[g, pl.ds(m * 8 + a, 8, stride=64), :] for m in range(8)], axis=0)
            wop_ref[a * 128:(a + 1) * 128, g * 128:(g + 1) * 128] = pltpu.bitcast(t, BF16)


def _kernel(q_ref, k_ref, v_ref, sk_ref, h_ref, dd_ref, x_ref, w_hbm, wo_hbm, fw_ref, iv_ref,
            o_hbm,
            w_raw, w_p, wo_raw, wo_tmp, wo_p, kf, us, hs, ys, qs, ks, vs, ob, oa_buf, obuf, sems):
    j = pl.program_id(0)
    nsteps = pl.num_programs(0)

    def out_a(step):
        return pltpu.make_async_copy(oa_buf, o_hbm.at[:, pl.ds(pl.multiple_of(step * 128, 128), 128)], sems.at[2])

    def out_b(step):
        return pltpu.make_async_copy(obuf, o_hbm.at[pl.ds(pl.multiple_of(step * TM, TM), TM), pl.ds(D, D)], sems.at[3])

    @pl.when(j == 0)
    def _():
        c1 = pltpu.make_async_copy(w_hbm, w_raw, sems.at[0])
        c2 = pltpu.make_async_copy(wo_hbm, wo_raw, sems.at[1])
        c1.start()
        c2.start()
        kf[0:8, :] = jnp.zeros((8, 128), F32)
        for g in range(NG):
            ks[g, 0:HIST, :] = jnp.zeros((HIST, 128), F32)
            vs[g, 0:HIST, :] = jnp.zeros((HIST, 128), F32)
        c1.wait()
        _permute_cols(w_raw, w_p)
        c2.wait()
        _permute_rows(wo_raw, wo_tmp, wo_p)

    @pl.when(j > 0)
    def _():
        out_a(j - 1).wait()
        out_b(j - 1).wait()

    eye = (lax.broadcasted_iota(jnp.int32, (8, 4), 0) == lax.broadcasted_iota(jnp.int32, (8, 4), 1)).astype(BF16)
    skt = lax.dot_general(eye, sk_ref[...], (((1,), (1,)), ((), ())), preferred_element_type=F32)
    kf[8:8 + S, :] = k_ref[...].astype(F32)
    kvs = []
    for c in range(NCH):
        r = 8 + c * CH
        acc = kf[r:r + CH, :] * skt[0:1, :]
        for t in range(1, 4):
            acc = acc + kf[r - t:r - t + CH, :] * skt[t:t + 1, :]
        kvs.append((acc * v_ref[c * CH:(c + 1) * CH, :].astype(F32)).astype(BF16))
    fw = fw_ref[...]
    us[...] = jnp.dot(fw, jnp.concatenate(kvs, axis=1), preferred_element_type=F32)
    hst = jnp.concatenate([h_ref[:, c * CH:(c + 1) * CH] for c in range(NCH)], axis=0)
    hs[...] = lax.dot_general(fw, hst, (((1,), (1,)), ((), ())), preferred_element_type=F32)

    x = x_ref[...]
    for g2 in range(NG // 2):
        for sec, dst, off in ((0, qs, 0), (1, ks, HIST), (2, vs, HIST)):
            r = jnp.dot(x, w_p[:, sec * D + g2 * 256: sec * D + (g2 + 1) * 256], preferred_element_type=F32)
            dst[2 * g2, off:off + TM, :] = r[:, :128]
            dst[2 * g2 + 1, off:off + TM, :] = r[:, 128:]

    dvec = dd_ref[...].astype(F32)
    for f in range(CH // 8):
        re, im = slice(8 * f, 8 * f + 8), slice(CH + 8 * f, CH + 8 * f + 8)
        col = lambda c: slice(c * 128, (c + 1) * 128)
        even = f < CH // 16
        hc = [hs[re, col(c)] for c in range(NCH)]
        hd = [hs[im, col(c)] for c in range(NCH)]
        gc = [hc[0] + dvec] + [(hc[c] - hd[c - 1]) if even else (hc[c] + hd[c - 1]) for c in range(1, NCH)]
        gd = [hd[0]] + [(hd[c] + hc[c - 1]) if even else (hd[c] - hc[c - 1]) for c in range(1, NCH)]
        ua = [us[re, col(c)] for c in range(NCH)]
        ub = [us[im, col(c)] for c in range(NCH)]

        def conv(u, g):
            out = []
            for i in range(NCH):
                acc = u[0] * g[i]
                for c in range(1, i + 1):
                    acc = acc + u[c] * g[i - c]
                out.append(acc)
            return out

        k1 = conv([a + b for a, b in zip(ua, ub)], gc)
        k2 = conv(ua, [d - c for c, d in zip(gc, gd)])
        for i in range(NCH):
            ys[im, col(i)] = k1[i] + k2[i]
        k3 = conv(ub, [d + c for c, d in zip(gc, gd)])
        for i in range(NCH):
            ys[re, col(i)] = k1[i] - k3[i]

    y = jnp.dot(iv_ref[...], ys[...].astype(BF16), preferred_element_type=F32)
    for c in range(NCH):
        oa_buf[c * CH:(c + 1) * CH, :] = (
            y[:, c * 128:(c + 1) * 128] * q_ref[c * CH:(c + 1) * CH, :].astype(F32)).astype(BF16)
    out_a(j).start()

    lane = lax.broadcasted_iota(jnp.int32, (RT, 128), 1)
    b4, b0 = (lane & 16) != 0, (lane & 1) != 0
    row = lax.broadcasted_iota(jnp.int32, (RT, 128), 0) + j * TM
    cexp = float(DH ** -0.5 * np.log2(np.e))
    for t in range(TM // RT):
        r0 = t * RT
        qv = [qs[g, r0:r0 + RT, :] for g in range(NG)]
        lg = []
        for w in range(WIN):
            o = HIST + r0 - DIL * w
            acc = qv[0] * ks[0, o:o + RT, :]
            for g in range(1, NG):
                acc = acc + qv[g] * ks[g, o:o + RT, :]
            acc = acc + jnp.where(b4, pltpu.roll(acc, 16, 1), pltpu.roll(acc, 112, 1))
            acc = acc + jnp.where(b0, pltpu.roll(acc, 1, 1), pltpu.roll(acc, 127, 1))
            if t == 0 and w > 0:
                acc = jnp.where(row >= DIL * w, acc, -1e9 * DH ** 0.5)
            lg.append(acc)
        m = lg[0]
        for w in range(1, WIN):
            m = jnp.maximum(m, lg[w])
        p = [jnp.exp2((l - m) * cexp) for l in lg]
        den = p[0]
        for w in range(1, WIN):
            den = den + p[w]
        inv = 1.0 / den
        p = [e * inv for e in p]
        for g in range(NG):
            o = HIST + r0
            acc = p[0] * vs[g, o:o + RT, :]
            for w in range(1, WIN):
                o = HIST + r0 - DIL * w
                acc = acc + p[w] * vs[g, o:o + RT, :]
            ob[r0:r0 + RT, g * 128:(g + 1) * 128] = acc.astype(BF16)
    for g in range(NG):
        ks[g, 0:HIST, :] = ks[g, TM:TM + HIST, :]
        vs[g, 0:HIST, :] = vs[g, TM:TM + HIST, :]
    obuf[...] = jnp.dot(ob[...], wo_p[...], preferred_element_type=F32).astype(BF16)
    out_b(j).start()

    @pl.when(j == nsteps - 1)
    def _():
        out_a(j).wait()
        out_b(j).wait()


@jax.jit
def pallas_concat_heads__ssm_conv_h3__sliding_local_dilated__prompt_kernel(
    A_q, A_k, A_v, A_shift_k, A_ssm_k, A_ssm_D, B_x, B_wqkv, B_wo,
):
    fw, iv = _dft_mats()
    colspec = pl.BlockSpec((S, 128), lambda j: (0, j))
    out = pl.pallas_call(
        _kernel,
        grid=(NG,),
        in_specs=[
            colspec, colspec, colspec,
            pl.BlockSpec((128, 4), lambda j: (j, 0)),
            pl.BlockSpec((128, S), lambda j: (j, 0)),
            pl.BlockSpec((1, 128), lambda j: (0, j)),
            pl.BlockSpec((TM, D), lambda j: (j, 0)),
            pl.BlockSpec(memory_space=pl.ANY),
            pl.BlockSpec(memory_space=pl.ANY),
            pl.BlockSpec((2 * CH, CH), lambda j: (0, 0)),
            pl.BlockSpec((CH, 2 * CH), lambda j: (0, 0)),
        ],
        out_specs=pl.BlockSpec(memory_space=pl.ANY),
        out_shape=jax.ShapeDtypeStruct((S, 2 * D), BF16),
        scratch_shapes=[
            pltpu.VMEM((D, 3 * D), BF16), pltpu.VMEM((D, 3 * D), BF16),
            pltpu.VMEM((D, D), BF16), pltpu.VMEM((NG, D // 2, 128), jnp.uint32), pltpu.VMEM((D, D), BF16),
            pltpu.VMEM((8 + S, 128), F32),
            pltpu.VMEM((2 * CH, S), F32), pltpu.VMEM((2 * CH, S), F32), pltpu.VMEM((2 * CH, S), F32),
            pltpu.VMEM((NG, TM, 128), F32), pltpu.VMEM((NG, HIST + TM, 128), F32), pltpu.VMEM((NG, HIST + TM, 128), F32),
            pltpu.VMEM((TM, D), BF16), pltpu.VMEM((S, 128), BF16), pltpu.VMEM((TM, D), BF16),
            pltpu.SemaphoreType.DMA((4,)),
        ],
        compiler_params=pltpu.CompilerParams(
            dimension_semantics=("arbitrary",), vmem_limit_bytes=100 * 2 ** 20),
    )(A_q.reshape(S, D), A_k.reshape(S, D), A_v.reshape(S, D), A_shift_k, A_ssm_k,
      A_ssm_D.reshape(1, D), B_x.reshape(S, D), B_wqkv, B_wo, fw, iv)
    return out.reshape(1, S, 2 * D)
```

```python
import os
import numpy as np
import jax
import jax.numpy as jnp
from jax import lax
import jax.experimental.pallas as pl
import jax.experimental.pallas.tpu as pltpu

S = 2048
D = 1024
NG = D // 128
CH = 128
NCH = S // CH
TM = S // NG
HIST = 16
WIN, DIL, DH = 8, 2, 32
RT = 16
NI = int(os.environ.get("NI", 4))
PER = NCH // NI
CB = int(os.environ.get('CB', 2))
LINK = int(os.environ.get('LINK', 1))
GPI = NG // NI
F32, BF16, U32 = jnp.float32, jnp.bfloat16, jnp.uint32


def _dft_mats():
    r = np.arange(CH)
    k = (16 * (r // 16) + 2 * (r % 8) + (r // 8) % 2).astype(np.float64)
    th = 2.0 * np.pi * (k + 0.5) / (2 * CH)
    ang = th[:, None] * np.arange(CH, dtype=np.float64)[None, :]
    fwd = np.concatenate([np.cos(ang), -np.sin(ang)], axis=0)
    inv = fwd.T / CH
    return jnp.asarray(fwd, BF16), jnp.asarray(np.stack([inv[:, :CH], inv[:, CH:]]), BF16)


def _permute_cols(w_ref, wp_ref, sec, r0, rows):
    lane = lax.broadcasted_iota(jnp.int32, (rows // 2, 128), 1)
    v = [pltpu.bitcast(w_ref[sec * NG + g, pl.ds(r0, rows), :], jnp.uint32) for g in range(NG)]
    v = [v[0]] + [pltpu.roll(v[g], 2 * g, 1) for g in range(1, NG)]
    t = [v[(-e) % NG] for e in range(NG)]
    for st in range(3):
        bit = (lane & (2 << st)) != 0
        t = [jnp.where(bit, t[(e - (1 << st)) % NG], t[e]) for e in range(NG)]
    t = [t[0]] + [pltpu.roll(t[e], 128 - 2 * e, 1) for e in range(1, NG)]
    for e in range(NG):
        wp_ref[sec * NG + e, pl.ds(pl.multiple_of(r0 // 2, rows // 2), rows // 2), :] = t[e]


def _permute_rows(wo_ref, tmp_ref, wp_ref):
    def body(g, carry):
        w = pltpu.bitcast(wo_ref[g], jnp.uint32)
        for b in range(8):
            tmp_ref[b * 72:b * 72 + 64, :] = w[b * 64:(b + 1) * 64, :]
        for a in range(8):
            t = jnp.concatenate([tmp_ref[pl.ds(m * 8 + a, 8, stride=72), :] for m in range(8)], axis=0)
            wp_ref[g, a * 64:(a + 1) * 64, :] = t
        return carry
    lax.fori_loop(0, NG, body, 0)


def _cat(parts, axis):
    return parts[0] if len(parts) == 1 else jnp.concatenate(parts, axis=axis)


def _bf(parts):
    return jnp.concatenate([pltpu.bitcast(x, BF16) for x in parts], axis=1)


def _kernel(q_ref, k_ref, v_ref, sk_ref, h_ref, dd_ref, x_ref, w_hbm, wo_hbm, fw_ref, iv_ref,
            o_hbm,
            w_r, wo_r, w_p, wo_p, wo_tmp, kf, xs, skt_s, hprev,
            us0, us1, hs0, hs1, ys0, ys1, qs0, qs1, ks0, ks1, vs0, vs1, ob0, ob1,
            oa_buf, obuf, wsem, osem):
    s = pl.program_id(0)
    us, hs, ys = (us0, us1), (hs0, hs1), (ys0, ys1)
    qs, ks, vs, ob = (qs0, qs1), (ks0, ks1), (vs0, vs1), (ob0, ob1)

    never = lax.broadcasted_iota(jnp.int32, (8, 128), 1) > s + 1000
    chain = [None]

    def link(x):
        if chain[0] is None or not LINK:
            return x
        head = jnp.where(never, chain[0], x[0:8])
        return head if x.shape[0] == 8 else jnp.concatenate([head, jnp.where(never, chain[0], x[8:16])], axis=0)

    def mark(x):
        chain[0] = x[x.shape[0] - 8:]

    def out_copies(step, par):
        t = step - 2
        cps = [pltpu.make_async_copy(oa_buf.at[par], o_hbm.at[:, pl.ds(pl.multiple_of(t * 128, 128), 128)],
                                     osem.at[par * (NG + 1)])]
        for g in range(NG):
            cps.append(pltpu.make_async_copy(
                obuf.at[par, g], o_hbm.at[pl.ds(pl.multiple_of(t * TM, TM), TM), pl.ds(D + g * 128, 128)],
                osem.at[par * (NG + 1) + 1 + g]))
        return cps

    def w_copy(n):
        if n < 3 * NG:
            return pltpu.make_async_copy(w_hbm.at[:, pl.ds(n * 128, 128)], w_r.at[n], wsem.at[n])
        return pltpu.make_async_copy(wo_hbm.at[:, pl.ds((n - 3 * NG) * 128, 128)], wo_r.at[n - 3 * NG], wsem.at[n])

    def a_fwd(par, u):
        skt = skt_s[...]
        kvs, hch = [], []
        for cc in range(PER):
            r = pl.multiple_of((u * PER + cc) * CH, CH)
            kf[pl.ds(8 + r, CH), :] = k_ref[pl.ds(r, CH), :].astype(F32)
            acc = kf[pl.ds(8 + r, CH), :] * skt[0:1, :]
            for t in range(1, 4):
                acc = acc + kf[pl.ds(8 + r - t, CH), :] * skt[t:t + 1, :]
            kvs.append((acc * v_ref[pl.ds(r, CH), :].astype(F32)).astype(BF16))
            hch.append(h_ref[:, pl.ds(r, CH)])
        fw = fw_ref[...]
        uu = jnp.dot(fw, _cat(kvs, 1), preferred_element_type=F32)
        hh = lax.dot_general(fw, _cat(hch, 0), (((1,), (1,)), ((), ())), preferred_element_type=F32)
        dvec = dd_ref[...].astype(F32)
        dsel = jnp.where(u == 0, dvec, 0.0)
        for cc in range(PER):
            c = u * PER + cc
            ua, ub = uu[:CH, cc * 128:(cc + 1) * 128], uu[CH:, cc * 128:(cc + 1) * 128]
            us[par][c, 0] = ua + ub
            us[par][c, 1] = ua
            us[par][c, 2] = ub
            hc, hd = hh[:CH, cc * 128:(cc + 1) * 128], hh[CH:, cc * 128:(cc + 1) * 128]
            if cc == 0:
                pc, pd = hprev[0], hprev[1]
            for f in range(CH // 8):
                t = slice(8 * f, 8 * f + 8)
                gc = (hc[t] - pd[t]) if f % 2 == 0 else (hc[t] + pd[t])
                gd = (hd[t] + pc[t]) if f % 2 == 0 else (hd[t] - pc[t])
                if cc == 0:
                    gc = gc + dsel
                hs[par][c, 0, t, :] = gc
                hs[par][c, 1, t, :] = gd - gc
                hs[par][c, 2, t, :] = gd + gc
            pc, pd = hc, hd
        hprev[0] = pc
        hprev[1] = pd

    def a_conv(par, u, ff, m):
        t = pl.ds(pl.multiple_of((u * PER + ff) * 8, 8), 8)
        for blk in range(NCH // CB):
            i0 = blk * CB
            acc = [None] * CB if m == 0 else [link(ys[par][i0 + j, 0, t, :]) for j in range(CB)]
            win = {}
            for c in range(i0 + CB):
                a = us[par][c, m, t, :]
                if m == 0 and c == 0:
                    a = link(a)
                for j in range(CB):
                    d = i0 + j - c
                    if d < 0:
                        continue
                    if d not in win:
                        win[d] = hs[par][d, m, t, :]
                    pr = a * win[d]
                    acc[j] = pr if acc[j] is None else (acc[j] - pr if m == 2 else acc[j] + pr)
            for j in range(CB):
                ys[par][i0 + j, m % 2, t, :] = acc[j]
            mark(acc[CB - 1])

    def a_inv(par, u):
        yy = _cat([_cat([ys[par][u * PER + cc, 0], ys[par][u * PER + cc, 1]], 0).astype(BF16) for cc in range(PER)], 1)
        y = jnp.dot(_cat([iv_ref[0], iv_ref[1]], 1), yy, preferred_element_type=F32)
        for cc in range(PER):
            r = pl.multiple_of((u * PER + cc) * CH, CH)
            oa_buf[par, pl.ds(r, CH), :] = (
                y[:, cc * 128:(cc + 1) * 128] * q_ref[pl.ds(r, CH), :].astype(F32)).astype(BF16)

    def b_qkv(par, sec, g, first):
        x = _bf([xs[c] for c in range(NG)])
        r = jnp.dot(x, _bf([w_p[sec * NG + g], w_p[sec * NG + g + 1]]), preferred_element_type=F32)
        for e in range(2):
            rr = r[:, e * 128:(e + 1) * 128]
            if sec == 0:
                qs[par][g + e] = rr
            else:
                dst = (ks, vs)[sec - 1]
                dst[par][g + e, HIST:HIST + TM, :] = rr
                dst[par][g + e, 0:HIST, :] = (jnp.zeros((HIST, 128), F32) if first
                                              else dst[1 - par][g + e, TM:TM + HIST, :])

    def b_qk(par, u, tt, first):
        lane = lax.broadcasted_iota(jnp.int32, (RT, 128), 1)
        b4, b0 = (lane & 16) != 0, (lane & 1) != 0
        cexp = float(DH ** -0.5 * np.log2(np.e))
        r0 = pl.multiple_of((u * PER + tt) * RT, RT)
        lg = []
        for w in range(WIN):
            o = pl.ds(HIST + r0 - DIL * w, RT)
            acc = link(ks[par][0, o, :]) * qs[par][0, pl.ds(r0, RT), :]
            for g in range(1, NG):
                acc = acc + qs[par][g, pl.ds(r0, RT), :] * ks[par][g, o, :]
            mark(acc)
            lg.append(acc + jnp.where(b4, pltpu.roll(acc, 16, 1), pltpu.roll(acc, 112, 1)))
        lg = [l + jnp.where(b0, pltpu.roll(l, 1, 1), pltpu.roll(l, 127, 1)) for l in lg]
        if first and tt == 0:
            row = lax.broadcasted_iota(jnp.int32, (RT, 128), 0) + r0
            lg = [jnp.where(row >= DIL * w, lg[w], -1e9 * DH ** 0.5) for w in range(WIN)]
        m = lg[0]
        for w in range(1, WIN):
            m = jnp.maximum(m, lg[w])
        p = [jnp.exp2((l - m) * cexp) for l in lg]
        den = p[0]
        for w in range(1, WIN):
            den = den + p[w]
        inv = pl.reciprocal(den, approx=True)
        inv = inv * (2.0 - den * inv)
        return [e * inv for e in p]

    def b_pv(par, u, tt, p):
        r0 = pl.multiple_of((u * PER + tt) * RT, RT)
        for g in range(NG):
            acc = p[0] * link(vs[par][g, pl.ds(HIST + r0, RT), :])
            for w in range(1, WIN):
                acc = acc + p[w] * vs[par][g, pl.ds(HIST + r0 - DIL * w, RT), :]
            mark(acc)
            ob[par][g, pl.ds(pl.multiple_of((u * PER + tt) * (RT // 2), RT // 2), RT // 2), :] = (
                pltpu.bitcast(acc.astype(BF16), U32))

    def b_out(par, g):
        o = _bf([ob[par][c] for c in range(NG)])
        r = jnp.dot(o, _bf([wo_p[g], wo_p[g + 1]]), preferred_element_type=F32)
        obuf[par, g] = r[:, :128].astype(BF16)
        obuf[par, g + 1] = r[:, 128:].astype(BF16)

    def step(par, s1, s2, s3, first1=False, first2=False):
        if s1:
            eye = (lax.broadcasted_iota(jnp.int32, (8, 4), 0)
                   == lax.broadcasted_iota(jnp.int32, (8, 4), 1)).astype(BF16)
            skt_s[...] = lax.dot_general(eye, sk_ref[...], (((1,), (1,)), ((), ())), preferred_element_type=F32)
            hprev[...] = jnp.zeros((2, CH, 128), F32)
            for c in range(NG):
                xs[c] = pltpu.bitcast(x_ref[:, c * 128:(c + 1) * 128], U32)

        def body(u, carry):
            chain[0] = None
            mm = []
            if s1:
                mm += [lambda sec=sec, g2=g2: b_qkv(par, sec, u * GPI + 2 * g2, first1)
                       for g2 in range(GPI // 2) for sec in range(3)]
            if s3:
                mm += [lambda g2=g2: b_out(par, u * GPI + 2 * g2) for g2 in range(GPI // 2)]
            if s3:
                a_inv(par, u)
            for i in range(PER):
                if i < len(mm):
                    mm[i]()
                if s2:
                    p = b_qk(1 - par, u, i, first2)
                    for m in range(3):
                        a_conv(1 - par, u, i, m)
                    b_pv(1 - par, u, i, p)
                if s1 and i == PER // 2 - 1:
                    a_fwd(par, u)
            return carry

        if NI == 1:
            body(0, 0)
        else:
            lax.fori_loop(0, NI, body, 0)
        if s3:
            for cp in out_copies(s, par):
                cp.start()

    @pl.when(s == 0)
    def _():
        for n in range(4 * NG):
            w_copy(n).start()
        kf[0:8, :] = jnp.zeros((8, 128), F32)
        for sec in range(3):
            for n in range(NG):
                w_copy(sec * NG + n).wait()

            def pbody(i, carry):
                _permute_cols(w_r, w_p, sec, pl.multiple_of(i * 64, 64), 64)
                return carry
            lax.fori_loop(0, D // 64, pbody, 0)
        for n in range(NG):
            w_copy(3 * NG + n).wait()
        _permute_rows(wo_r, wo_tmp, wo_p)
        step(0, True, False, False, first1=True)

    @pl.when(s == 1)
    def _():
        step(1, True, True, False, first2=True)

    for par in range(2):
        @pl.when(jnp.logical_and(s >= 4, s % 2 == par))
        def _():
            for cp in out_copies(s - 2, par):
                cp.wait()

        @pl.when(jnp.logical_and(jnp.logical_and(s >= 2, s < NG), s % 2 == par))
        def _():
            step(par, True, True, True)

    @pl.when(s == NG)
    def _():
        step(0, False, True, True)

    @pl.when(s == NG + 1)
    def _():
        step(1, False, False, True)
        for cp in out_copies(s - 1, 0) + out_copies(s, 1):
            cp.wait()


@jax.jit
def pallas_concat_heads__ssm_conv_h3__sliding_local_dilated__prompt_kernel(
    A_q, A_k, A_v, A_shift_k, A_ssm_k, A_ssm_D, B_x, B_wqkv, B_wo,
):
    fw, iv = _dft_mats()
    cl = lambda j: jnp.clip(j, 0, NG - 1)
    sp3, sp2 = pltpu.VMEM((NCH, 3, CH, 128), F32), pltpu.VMEM((NCH, 2, CH, 128), F32)
    qsp, ksp = pltpu.VMEM((NG, TM, 128), F32), pltpu.VMEM((NG, HIST + TM, 128), F32)
    osp = pltpu.VMEM((NG, TM // 2, 128), U32)
    out = pl.pallas_call(
        _kernel,
        grid=(NG + 2,),
        in_specs=[
            pl.BlockSpec((S, 128), lambda j: (0, cl(j - 2))),
            pl.BlockSpec((S, 128), lambda j: (0, cl(j))),
            pl.BlockSpec((S, 128), lambda j: (0, cl(j))),
            pl.BlockSpec((128, 4), lambda j: (cl(j), 0)),
            pl.BlockSpec((128, S), lambda j: (cl(j), 0)),
            pl.BlockSpec((1, 128), lambda j: (0, cl(j))),
            pl.BlockSpec((TM, D), lambda j: (cl(j), 0)),
            pl.BlockSpec(memory_space=pl.ANY),
            pl.BlockSpec(memory_space=pl.ANY),
            pl.BlockSpec((2 * CH, CH), lambda j: (0, 0)),
            pl.BlockSpec((2, CH, CH), lambda j: (0, 0, 0)),
        ],
        out_specs=pl.BlockSpec(memory_space=pl.ANY),
        out_shape=jax.ShapeDtypeStruct((S, 2 * D), BF16),
        scratch_shapes=[
            pltpu.VMEM((3 * NG, D, 128), BF16), pltpu.VMEM((NG, D, 128), BF16),
            pltpu.VMEM((3 * NG, D // 2, 128), U32), pltpu.VMEM((NG, D // 2, 128), U32), pltpu.VMEM((8 * 72, 128), U32),
            pltpu.VMEM((8 + S, 128), F32), osp, pltpu.VMEM((8, 128), F32), pltpu.VMEM((2, CH, 128), F32),
            sp3, sp3, sp3, sp3, sp2, sp2, qsp, qsp, ksp, ksp, ksp, ksp, osp, osp,
            pltpu.VMEM((2, S, 128), BF16), pltpu.VMEM((2, NG, TM, 128), BF16),
            pltpu.SemaphoreType.DMA((4 * NG,)), pltpu.SemaphoreType.DMA((2 * (NG + 1),)),
        ],
        compiler_params=pltpu.CompilerParams(
            dimension_semantics=("arbitrary",), vmem_limit_bytes=100 * 2 ** 20),
    )(A_q.reshape(S, D), A_k.reshape(S, D), A_v.reshape(S, D), A_shift_k, A_ssm_k,
      A_ssm_D.reshape(1, D), B_x.reshape(S, D), B_wqkv, B_wo, fw, iv)
    return out.reshape(1, S, 2 * D)
```

```python
import os
import numpy as np
import jax
import jax.numpy as jnp
from jax import lax
import jax.experimental.pallas as pl
import jax.experimental.pallas.tpu as pltpu

S = 2048
D = 1024
NG = D // 128
CH = 128
NCH = S // CH
TM = S // NG
HIST = 112
PITCH = 24
LA = int(os.environ.get('LA', 2))
WIN, DIL, DH = 8, 2, 32
RT = 16
NI = int(os.environ.get("NI", 4))
PER = NCH // NI
CB = int(os.environ.get('CB', 2))
LINK = int(os.environ.get('LINK', 1))
DLK = int(os.environ.get('DLK', 0))
NOCSE = int(os.environ.get('NOCSE', 1))
QG = int(os.environ.get('QG', 8))
GATE = int(os.environ.get('GATE', 1))
GPI = NG // NI
F32, BF16, U32 = jnp.float32, jnp.bfloat16, jnp.uint32


def _dft_mats():
    r = np.arange(CH)
    k = (16 * (r // 16) + 2 * (r % 8) + (r // 8) % 2).astype(np.float64)
    th = 2.0 * np.pi * (k + 0.5) / (2 * CH)
    ang = th[:, None] * np.arange(CH, dtype=np.float64)[None, :]
    fwd = np.concatenate([np.cos(ang), -np.sin(ang)], axis=0)
    inv = fwd.T / CH
    return jnp.asarray(fwd, BF16), jnp.asarray(np.stack([inv[:, :CH], inv[:, CH:]]), BF16)


def _permute_cols(w_ref, wp_ref, sec, q):
    lane = lax.broadcasted_iota(jnp.int32, (8, 128), 1)
    bits = [(lane & (2 << st)) != 0 for st in range(3)]

    def first(i):
        r = pl.ds(pl.multiple_of(q * 256 + i * 16, 16), 16)
        v = [pltpu.bitcast(w_ref[sec, r, g * 128:(g + 1) * 128], U32) for g in range(NG)]
        return [v[0]] + [pltpu.roll(v[g], 2 * g, 1) for g in range(1, NG)]

    def second(i, v):
        t = [v[(-e) % NG] for e in range(NG)]
        for st in range(3):
            t = [jnp.where(bits[st], t[(e - (1 << st)) % NG], t[e]) for e in range(NG)]
        t = [t[0]] + [pltpu.roll(t[e], 128 - 2 * e, 1) for e in range(1, NG)]
        for e in range(NG):
            wp_ref[sec * NG + e, pl.ds(pl.multiple_of(q * 128 + i * 8, 8), 8), :] = t[e]

    ahead = 2
    vs = [first(i) for i in range(ahead)]
    for i in range(16):
        if i + ahead < 16:
            vs.append(first(i + ahead))
        second(i, vs[i])


def _permute_rows(wo_ref, tmp_ref, wp_ref, q):
    for e in range(2):
        w = pltpu.bitcast(wo_ref[q, :, e * 128:(e + 1) * 128], U32)
        for b in range(8):
            tmp_ref[e, b * 72:b * 72 + 64, :] = w[b * 64:(b + 1) * 64, :]
        for a in range(8):
            t = jnp.concatenate([tmp_ref[e, pl.ds(m * 8 + a, 8, stride=72), :] for m in range(8)], axis=0)
            wp_ref[2 * q + e, a * 64:(a + 1) * 64, :] = t


def _cat(parts, axis):
    return parts[0] if len(parts) == 1 else jnp.concatenate(parts, axis=axis)


def _bf(parts):
    return jnp.concatenate([pltpu.bitcast(x, BF16) for x in parts], axis=1)


def _kernel(q_hbm, k_hbm, v_hbm, sk_ref, h_hbm, dd_ref, x_hbm, w_hbm, wo_hbm, fw_ref, iv_ref,
            o_hbm,
            w_r, wo_r, w_p, wo_p, wo_tmp, qb, kb, vb, hb, xb, kf, xn, xs0, xs1, hprev,
            us0, us1, hs0, hs1, ys0, ys1, qs0, qs1, ks0, ks1, vs0, vs1, ob0, ob1,
            oa_buf, obuf, wsem, isem, osem):
    us, hs, ys, xs = (us0, us1), (hs0, hs1), (ys0, ys1), (xs0, xs1)
    qs, ks, vs, ob = (qs0, qs1), (ks0, ks1), (vs0, vs1), (ob0, ob1)
    cur = {}

    chain = [None]

    def link(x):
        if chain[0] is None or not cur['link']:
            return x
        head = jnp.where(cur['never'], chain[0], x[0:8])
        return head if x.shape[0] == 8 else jnp.concatenate([head, jnp.where(cur['never'], chain[0], x[8:16])], axis=0)

    def mark(*xs_):
        parts = [x[r:r + 8] for x in xs_ for r in range(0, x.shape[0], 8)]
        t = parts[-1]
        if cur['link']:
            for y in parts[:-1]:
                t = jnp.where(cur['never'], y, t)
        chain[0] = t

    dl = [None]

    def zero(i):
        return lax.shift_right_logical(cur['u'] + i, 8) if cur['link'] else 0

    def dead(w):
        if dl[0] is None or DLK < 0:
            return w
        r = DLK * 64
        mid = jnp.where(cur['never'], pltpu.bitcast(dl[0], U32), w[r:r + 8])
        return jnp.concatenate(([w[:r]] if r else []) + [mid, w[r + 8:]], axis=0)

    def gate(r):
        dl[0] = chain[0]
        if GATE:
            t = r[r.shape[0] - 8:, r.shape[1] - 128:]
            chain[0] = t if chain[0] is None else jnp.where(cur['never'], t, chain[0])

    def out_copies(step, par):
        t = step - 2
        cps = [pltpu.make_async_copy(oa_buf.at[par], o_hbm.at[:, pl.ds(pl.multiple_of(t * 128, 128), 128)],
                                     osem.at[par * (NG + 1)])]
        for g in range(NG):
            cps.append(pltpu.make_async_copy(
                obuf.at[par, g], o_hbm.at[pl.ds(pl.multiple_of(t * TM, TM), TM), pl.ds(D + g * 128, 128)],
                osem.at[par * (NG + 1) + 1 + g]))
        return cps

    def w_copy(n):
        sec, r = n // 4, pl.ds(pl.multiple_of((n % 4) * 256, 256), 256)
        return pltpu.make_async_copy(w_hbm.at[r, pl.ds(pl.multiple_of(sec * D, D), D)], w_r.at[sec, r], wsem.at[n])

    def wo_copy(n):
        return pltpu.make_async_copy(wo_hbm.at[:, pl.ds(pl.multiple_of(n * 256, 256), 256)], wo_r.at[n],
                                     wsem.at[12 + n])

    def a_in(t, par):
        c = pl.ds(pl.multiple_of(t * 128, 128), 128)
        return [pltpu.make_async_copy(k_hbm.at[:, c], kb.at[par], isem.at[par * 5]),
                pltpu.make_async_copy(v_hbm.at[:, c], vb.at[par], isem.at[par * 5 + 1]),
                pltpu.make_async_copy(h_hbm.at[c, :], hb.at[par], isem.at[par * 5 + 2])]

    def q_in(t, par):
        return [pltpu.make_async_copy(q_hbm.at[:, pl.ds(pl.multiple_of(t * 128, 128), 128)], qb.at[par],
                                      isem.at[par * 5 + 3])]

    def x_in(t, par):
        return [pltpu.make_async_copy(x_hbm.at[pl.ds(pl.multiple_of(t * TM, TM), TM), :], xb.at[par],
                                      isem.at[par * 5 + 4])]

    def start(cps):
        for cp in cps:
            cp.start()

    def wait(cps):
        for cp in cps:
            cp.wait()

    def x_prep(par, u):
        for e in range(GPI):
            g = u * GPI + e
            xv = pltpu.bitcast(xb[par, :, pl.ds(pl.multiple_of(g * 128, 128), 128)], U32)
            for b in range(8):
                xn[e, b * PITCH:b * PITCH + 16, :] = xv[b * 16:(b + 1) * 16]
            xs[par][g] = jnp.concatenate([xn[e, pl.ds(n, 8, stride=PITCH), :] for n in range(16)], axis=0)

    def a_fwd(par, t, u):
        ch = pl.ds(pl.multiple_of(t * 128, 128), 128)
        skt = sk_ref[:, ch].astype(F32)
        kvs, hch = [], []
        for cc in range(PER):
            r = pl.multiple_of((u * PER + cc) * CH, CH)
            kf[pl.ds(8 + r, CH), :] = kb[par, pl.ds(r, CH), :].astype(F32)
            acc = kf[pl.ds(8 + r, CH), :] * skt[0:1, :]
            for j in range(1, 4):
                acc = acc + kf[pl.ds(8 + r - j, CH), :] * skt[j:j + 1, :]
            kvs.append((acc * vb[par, pl.ds(r, CH), :].astype(F32)).astype(BF16))
            hch.append(hb[par, :, pl.ds(r, CH)])
        fw = fw_ref[...]
        uu = jnp.dot(fw, _cat(kvs, 1), preferred_element_type=F32)
        hh = lax.dot_general(fw, _cat(hch, 0), (((1,), (1,)), ((), ())), preferred_element_type=F32)
        dvec = dd_ref[:, ch].astype(F32)
        dsel = jnp.where(u == 0, dvec, 0.0)
        for cc in range(PER):
            c = u * PER + cc
            ua, ub = uu[:CH, cc * 128:(cc + 1) * 128], uu[CH:, cc * 128:(cc + 1) * 128]
            us[par][c, 0] = ua + ub
            us[par][c, 1] = ua
            us[par][c, 2] = ub
            hc, hd = hh[:CH, cc * 128:(cc + 1) * 128], hh[CH:, cc * 128:(cc + 1) * 128]
            if cc == 0:
                pc, pd = jnp.where(u == 0, 0.0, hprev[0]), jnp.where(u == 0, 0.0, hprev[1])
            for f in range(CH // 8):
                t = slice(8 * f, 8 * f + 8)
                gc = (hc[t] - pd[t]) if f % 2 == 0 else (hc[t] + pd[t])
                gd = (hd[t] + pc[t]) if f % 2 == 0 else (hd[t] - pc[t])
                if cc == 0:
                    gc = gc + dsel
                hs[par][c, 0, t, :] = gc
                hs[par][c, 1, t, :] = gd - gc
                hs[par][c, 2, t, :] = gd + gc
            pc, pd = hc, hd
        hprev[0] = pc
        hprev[1] = pd
        return hh

    def a_conv(par, u, ff, m):
        for blk in range(NCH // CB):
            i0 = blk * CB
            t = pl.ds(pl.multiple_of((u * PER + ff + zero(blk)) * 8, 8), 8)
            acc = [None] * CB if m == 0 else [link(ys[par][i0 + j, 0, t, :]) for j in range(CB)]
            win = {}
            for c in range(i0 + CB):
                a = us[par][c, m, t, :]
                if m == 0 and c == 0:
                    a = link(a)
                for j in range(CB):
                    d = i0 + j - c
                    if d < 0:
                        continue
                    if d not in win:
                        win[d] = hs[par][d, m, t, :]
                    pr = a * win[d]
                    acc[j] = pr if acc[j] is None else (acc[j] - pr if m == 2 else acc[j] + pr)
            for j in range(CB):
                ys[par][i0 + j, m % 2, t, :] = acc[j]
            mark(*acc)

    def a_inv(par, u):
        yy = _cat([_cat([ys[par][u * PER + cc, 0], ys[par][u * PER + cc, 1]], 0).astype(BF16) for cc in range(PER)], 1)
        y = jnp.dot(_cat([iv_ref[0], iv_ref[1]], 1), yy, preferred_element_type=F32)
        for cc in range(PER):
            r = pl.multiple_of((u * PER + cc) * CH, CH)
            oa_buf[par, pl.ds(r, CH), :] = (
                y[:, cc * 128:(cc + 1) * 128] * qb[par, pl.ds(r, CH), :].astype(F32)).astype(BF16)

    def b_qkv(par, sec, g, first):
        x = _bf([xs[par][c] for c in range(NG)])
        r = jnp.dot(x, _bf([dead(w_p[sec * NG + g]), w_p[sec * NG + g + 1]]), preferred_element_type=F32)
        for e in range(2):
            rr = r[:, e * 128:(e + 1) * 128]
            if sec == 0:
                qs[par][g + e] = rr
            else:
                dst = (ks, vs)[sec - 1]
                dst[par][g + e, HIST:HIST + TM, :] = rr
                top = lax.broadcasted_iota(jnp.int32, (8, 128), 0) < 2
                for j in range(HIST // RT):
                    o = TM + RT * j
                    prev = 0.0 if first else dst[1 - par][g + e, o + 14:o + 22, :]
                    dst[par][g + e, RT * j:RT * j + 8, :] = jnp.where(top, prev, dst[par][g + e, o - 2:o + 6, :])
                    dst[par][g + e, RT * j + 8:RT * j + 16, :] = dst[par][g + e, o + 6:o + 14, :]
        return r

    def b_qk(par, u, tt, first):
        lane = lax.broadcasted_iota(jnp.int32, (RT, 128), 1)
        b4, b0 = (lane & 16) != 0, (lane & 1) != 0
        cexp = float(DH ** -0.5 * np.log2(np.e))
        r0 = pl.multiple_of((u * PER + tt) * RT, RT)
        lg = []
        for w in range(WIN):
            o = pl.ds(HIST + r0 - RT * w, RT)
            rq = pl.ds(pl.multiple_of(r0 + RT * zero(w // QG), RT), RT)
            acc = link(ks[par][0, o, :]) * qs[par][0, rq, :]
            for g in range(1, NG):
                acc = acc + qs[par][g, rq, :] * ks[par][g, o, :]
            mark(acc)
            lg.append(acc + jnp.where(b4, pltpu.roll(acc, 16, 1), pltpu.roll(acc, 112, 1)))
        lg = [l + jnp.where(b0, pltpu.roll(l, 1, 1), pltpu.roll(l, 127, 1)) for l in lg]
        if first:
            pair = (lax.broadcasted_iota(jnp.int32, (RT, 128), 0) // DIL) * RT + (u * PER + tt)
            lg = [jnp.where(pair >= w, lg[w], -1e9 * DH ** 0.5) for w in range(WIN)]
        m = lg[0]
        for w in range(1, WIN):
            m = jnp.maximum(m, lg[w])
        p = [jnp.exp2((l - m) * cexp) for l in lg]
        den = p[0]
        for w in range(1, WIN):
            den = den + p[w]
        inv = pl.reciprocal(den, approx=True)
        inv = inv * (2.0 - den * inv)
        return [e * inv for e in p]

    def b_pv(par, u, tt, p):
        r0 = pl.multiple_of((u * PER + tt) * RT, RT)
        for g in range(NG):
            acc = p[0] * link(vs[par][g, pl.ds(HIST + r0, RT), :])
            for w in range(1, WIN):
                acc = acc + p[w] * vs[par][g, pl.ds(HIST + r0 - RT * w, RT), :]
            mark(acc)
            ob[par][g, pl.ds(u * PER + tt, 8, stride=PITCH), :] = pltpu.bitcast(acc.astype(BF16), U32)

    def b_out(par, g):
        o = _bf([_cat([ob[par][c, b * PITCH:b * PITCH + 16, :] for b in range(8)], 0) for c in range(NG)])
        r = jnp.dot(o, _bf([dead(wo_p[g]), wo_p[g + 1]]), preferred_element_type=F32)
        obuf[par, g] = r[:, :128].astype(BF16)
        obuf[par, g + 1] = r[:, 128:].astype(BF16)
        return r

    def loop(fn, link_on=True):
        def body(u, carry):
            chain[0] = dl[0] = None
            cur.update(u=u, link=link_on and LINK,
                       never=lax.broadcasted_iota(jnp.int32, (8, 128), 1) > u + 1000)
            fn(u)
            return carry
        lax.fori_loop(0, NI, body, 0)

    def step(s, par, s1, s2, s3, first2=False):
        def body(u):
            if first2:
                wo_copy(u).wait()
                _permute_rows(wo_r, wo_tmp, wo_p, u)
            mm = []
            if s1:
                mm += [lambda sec=sec: b_qkv(par, sec, u * GPI, False) for sec in range(3)]
            if s3:
                mm += [lambda: b_out(par, u * GPI)]
                a_inv(par, u)
            for i in range(PER):
                tok = mm[i]() if i < len(mm) else None
                if s2:
                    p = b_qk(1 - par, u, i, first2)
                    for m in range(3):
                        a_conv(1 - par, u, i, m)
                    b_pv(1 - par, u, i, p)
                if s1 and i == PER // 2 - 1:
                    tok = a_fwd(par, s, u)
                if tok is not None and s1 and s2 and s3:
                    gate(tok)
            if s1:
                x_prep(1 - par, u)

        loop(body, s1)
        if s3:
            start(out_copies(s, par))

    start(x_in(0, 0))
    for n in range(LA):
        w_copy(n).start()
    kf[0:8, :] = jnp.zeros((8, 128), F32)
    wait(x_in(0, 0))

    def head(sec, u):
        if sec < 3:
            n = sec * 4 + u
            w_copy(n).wait()

            @pl.when(n + LA < 12)
            def _():
                w_copy(n + LA).start()
        if sec > 0:
            b_qkv(0, sec - 1, u * GPI, True)
        if sec < 3:
            _permute_cols(w_r, w_p, sec, u)
        if sec == 3:
            a_fwd(0, 0, u)
        if sec % 3 == 0:
            x_prep(sec // 3, u)

    for sec in range(4):
        if sec == 2:
            start(a_in(0, 0) + x_in(1, 1))
        if sec == 3:
            start(a_in(1, 1) + x_in(2, 0) + [wo_copy(n) for n in range(4)])
            wait(a_in(0, 0) + x_in(1, 1))
        loop(lambda u, sec=sec: head(sec, u))

    wait(a_in(1, 1) + x_in(2, 0))
    start(a_in(2, 0) + x_in(3, 1) + q_in(0, 0))
    step(1, 1, True, True, False, first2=True)

    def steady(j, carry):
        for par in range(2):
            s = 2 * j + par
            wait(a_in(s, par) + q_in(s - 2, par))
            start(q_in(s - 1, 1 - par))

            if par == 0:
                wait(x_in(s + 1, 1))
                start(a_in(s + 1, 1))

            @pl.when(j < NG // 2 - 1)
            def _():
                if par == 1:
                    wait(x_in(s + 1, 0))
                    start(a_in(s + 1, 0))
                start(x_in(s + 2, par))

            @pl.when(j > 1)
            def _():
                wait(out_copies(s - 2, par))
            step(s, par, True, True, True)
        return carry

    lax.fori_loop(1, NG // 2, steady, 0)
    wait(q_in(NG - 2, 0) + out_copies(NG - 2, 0))
    start(q_in(NG - 1, 1))
    step(NG, 0, False, True, True)
    wait(q_in(NG - 1, 1) + out_copies(NG - 1, 1))
    step(NG + 1, 1, False, False, True)
    wait(out_copies(NG, 0) + out_copies(NG + 1, 1))


@jax.jit
def pallas_concat_heads__ssm_conv_h3__sliding_local_dilated__prompt_kernel(
    A_q, A_k, A_v, A_shift_k, A_ssm_k, A_ssm_D, B_x, B_wqkv, B_wo,
):
    fw, iv = _dft_mats()
    sp3, sp2 = pltpu.VMEM((NCH, 3, CH, 128), F32), pltpu.VMEM((NCH, 2, CH, 128), F32)
    qsp, ksp = pltpu.VMEM((NG, TM, 128), F32), pltpu.VMEM((NG, HIST + TM + 8, 128), F32)
    xsp, osp = pltpu.VMEM((NG, TM // 2, 128), U32), pltpu.VMEM((NG, 8 * PITCH, 128), U32)
    col = pltpu.VMEM((2, S, 128), BF16)
    hbm, vmem = pl.BlockSpec(memory_space=pl.ANY), pl.BlockSpec(memory_space=pltpu.VMEM)
    out = pl.pallas_call(
        _kernel,
        in_specs=[hbm, hbm, hbm, vmem, hbm, vmem, hbm, hbm, hbm, vmem, vmem],
        out_specs=hbm,
        out_shape=jax.ShapeDtypeStruct((S, 2 * D), BF16),
        scratch_shapes=[
            pltpu.VMEM((3, D, D), BF16), pltpu.VMEM((4, D, 256), BF16),
            pltpu.VMEM((3 * NG, D // 2, 128), U32), pltpu.VMEM((NG, D // 2, 128), U32),
            pltpu.VMEM((2, 8 * 72, 128), U32),
            col, col, col, pltpu.VMEM((2, 128, S), BF16), pltpu.VMEM((2, TM, D), BF16),
            pltpu.VMEM((8 + S, 128), F32), pltpu.VMEM((GPI, 8 * PITCH, 128), U32), xsp, xsp,
            pltpu.VMEM((2, CH, 128), F32),
            sp3, sp3, sp3, sp3, sp2, sp2, qsp, qsp, ksp, ksp, ksp, ksp, osp, osp,
            col, pltpu.VMEM((2, NG, TM, 128), BF16),
            pltpu.SemaphoreType.DMA((16,)), pltpu.SemaphoreType.DMA((10,)),
            pltpu.SemaphoreType.DMA((2 * (NG + 1),)),
        ],
        compiler_params=pltpu.CompilerParams(vmem_limit_bytes=100 * 2 ** 20),
    )(A_q.reshape(S, D), A_k.reshape(S, D), A_v.reshape(S, D), A_shift_k.T, A_ssm_k,
      A_ssm_D.reshape(1, D), B_x.reshape(S, D), B_wqkv, B_wo, fw, iv)
    return out.reshape(1, S, 2 * D)
```

```python
import os
import numpy as np
import jax
import jax.numpy as jnp
from jax import lax
import jax.experimental.pallas as pl
import jax.experimental.pallas.tpu as pltpu

S = 2048
D = 1024
NG = D // 128
CH = 128
NCH = S // CH
TM = S // NG
HIST = 112
PITCH = 24
LA = int(os.environ.get('LA', 2))
WIN, DIL, DH = 8, 2, 32
RT = 16
NI = int(os.environ.get("NI", 4))
PER = NCH // NI
CB = int(os.environ.get('CB', 4))
LINK = int(os.environ.get('LINK', 1))
DLK = int(os.environ.get('DLK', 0))
NOCSE = int(os.environ.get('NOCSE', 1))
QG = int(os.environ.get('QG', 8))
LB = int(os.environ.get('LB', 2))
REP = int(os.environ.get('REP', 1))
ABL = int(os.environ.get('ABL', 0))
GATE = int(os.environ.get('GATE', 1))
GPI = NG // NI
F32, BF16, U32 = jnp.float32, jnp.bfloat16, jnp.uint32


def _dft_mats():
    r = np.arange(CH)
    k = (16 * (r // 16) + 2 * (r % 8) + (r // 8) % 2).astype(np.float64)
    th = 2.0 * np.pi * (k + 0.5) / (2 * CH)
    ang = th[:, None] * np.arange(CH, dtype=np.float64)[None, :]
    fwd = np.concatenate([np.cos(ang), -np.sin(ang)], axis=0)
    inv = fwd.T / CH
    return jnp.asarray(fwd, BF16), jnp.asarray(np.stack([inv[:, :CH], inv[:, CH:]]), BF16)


def _permute_cols(w_ref, wp_ref, sec, q):
    lane = lax.broadcasted_iota(jnp.int32, (8, 128), 1)
    bits = [(lane & (2 << st)) != 0 for st in range(3)]

    def first(i):
        r = pl.ds(pl.multiple_of(q * 256 + i * 16, 16), 16)
        v = [pltpu.bitcast(w_ref[sec, r, g * 128:(g + 1) * 128], U32) for g in range(NG)]
        return [v[0]] + [pltpu.roll(v[g], 2 * g, 1) for g in range(1, NG)]

    def second(i, v):
        t = [v[(-e) % NG] for e in range(NG)]
        for st in range(3):
            t = [jnp.where(bits[st], t[(e - (1 << st)) % NG], t[e]) for e in range(NG)]
        t = [t[0]] + [pltpu.roll(t[e], 128 - 2 * e, 1) for e in range(1, NG)]
        for e in range(NG):
            wp_ref[sec * NG + e, pl.ds(pl.multiple_of(q * 128 + i * 8, 8), 8), :] = t[e]

    ahead = 2
    vs = [first(i) for i in range(ahead)]
    for i in range(16):
        if i + ahead < 16:
            vs.append(first(i + ahead))
        second(i, vs[i])


def _permute_rows(wo_ref, tmp_ref, wp_ref, q):
    for e in range(2):
        w = pltpu.bitcast(wo_ref[q, :, e * 128:(e + 1) * 128], U32)
        for b in range(8):
            tmp_ref[e, b * 72:b * 72 + 64, :] = w[b * 64:(b + 1) * 64, :]
        for a in range(8):
            t = jnp.concatenate([tmp_ref[e, pl.ds(m * 8 + a, 8, stride=72), :] for m in range(8)], axis=0)
            wp_ref[2 * q + e, a * 64:(a + 1) * 64, :] = t


def _cat(parts, axis):
    return parts[0] if len(parts) == 1 else jnp.concatenate(parts, axis=axis)


def _bf(parts):
    return jnp.concatenate([pltpu.bitcast(x, BF16) for x in parts], axis=1)


def _kernel(q_hbm, k_hbm, v_hbm, sk_ref, h_hbm, dd_ref, x_hbm, w_hbm, wo_hbm, fw_ref, iv_ref,
            o_hbm,
            w_r, wo_r, w_p, wo_p, wo_tmp, qb, kb, vb, hb, xb, kf, xn, xs0, xs1, hprev,
            us0, us1, hs0, hs1, ys0, ys1, qs0, qs1, ks0, ks1, vs0, vs1, ob0, ob1,
            oa_buf, obuf, wsem, isem, osem):
    us, hs, ys, xs = (us0, us1), (hs0, hs1), (ys0, ys1), (xs0, xs1)
    qs, ks, vs, ob = (qs0, qs1), (ks0, ks1), (vs0, vs1), (ob0, ob1)
    cur = {}

    chain = []

    def link(x):
        if len(chain) < LB or not cur['link']:
            return x
        return jnp.where(cur['never'], chain.pop(0), x)

    def mark(x, must=False):
        if must or len(chain) < LB:
            chain.append(x)

    dl = [None]

    def zero(i):
        return lax.shift_right_logical(cur['u'] + i, 8) if cur['link'] else 0

    def dead(w):
        if dl[0] is None or DLK < 0:
            return w
        r = DLK * 64
        mid = jnp.where(cur['never'], pltpu.bitcast(dl[0], U32), w[r:r + 8])
        return jnp.concatenate(([w[:r]] if r else []) + [mid, w[r + 8:]], axis=0)

    def gate(r):
        dl[0] = chain[-1]
        if GATE:
            t = r[r.shape[0] - 8:, r.shape[1] - 128:]
            chain[:] = [jnp.where(cur['lane'] > cur['u'] + 1001, t, y) for y in chain]

    def out_copies(step, par):
        t = step - 2
        cps = [pltpu.make_async_copy(oa_buf.at[par], o_hbm.at[:, pl.ds(pl.multiple_of(t * 128, 128), 128)],
                                     osem.at[par * (NG + 1)])]
        for g in range(NG):
            cps.append(pltpu.make_async_copy(
                obuf.at[par, g], o_hbm.at[pl.ds(pl.multiple_of(t * TM, TM), TM), pl.ds(D + g * 128, 128)],
                osem.at[par * (NG + 1) + 1 + g]))
        return cps

    def w_copy(n):
        sec, r = n // 4, pl.ds(pl.multiple_of((n % 4) * 256, 256), 256)
        return pltpu.make_async_copy(w_hbm.at[r, pl.ds(pl.multiple_of(sec * D, D), D)], w_r.at[sec, r], wsem.at[n])

    def wo_copy(n):
        return pltpu.make_async_copy(wo_hbm.at[:, pl.ds(pl.multiple_of(n * 256, 256), 256)], wo_r.at[n],
                                     wsem.at[12 + n])

    def a_in(t, par):
        c = pl.ds(pl.multiple_of(t * 128, 128), 128)
        return [pltpu.make_async_copy(k_hbm.at[:, c], kb.at[par], isem.at[par * 5]),
                pltpu.make_async_copy(v_hbm.at[:, c], vb.at[par], isem.at[par * 5 + 1]),
                pltpu.make_async_copy(h_hbm.at[c, :], hb.at[par], isem.at[par * 5 + 2])]

    def q_in(t, par):
        return [pltpu.make_async_copy(q_hbm.at[:, pl.ds(pl.multiple_of(t * 128, 128), 128)], qb.at[par],
                                      isem.at[par * 5 + 3])]

    def x_in(t, par):
        return [pltpu.make_async_copy(x_hbm.at[pl.ds(pl.multiple_of(t * TM, TM), TM), :], xb.at[par],
                                      isem.at[par * 5 + 4])]

    def start(cps):
        for cp in cps:
            cp.start()

    def wait(cps):
        for cp in cps:
            cp.wait()

    def x_prep(par, u):
        for e in range(GPI):
            g = u * GPI + e
            xv = pltpu.bitcast(xb[par, :, pl.ds(pl.multiple_of(g * 128, 128), 128)], U32)
            for b in range(8):
                xn[e, b * PITCH:b * PITCH + 16, :] = xv[b * 16:(b + 1) * 16]
            xs[par][g] = jnp.concatenate([xn[e, pl.ds(n, 8, stride=PITCH), :] for n in range(16)], axis=0)

    def a_fwd(par, t, u):
        ch = pl.ds(pl.multiple_of(t * 128, 128), 128)
        skt = sk_ref[:, ch].astype(F32)
        kvs, hch = [], []
        for cc in range(PER):
            r = pl.multiple_of((u * PER + cc) * CH, CH)
            kf[pl.ds(8 + r, CH), :] = kb[par, pl.ds(r, CH), :].astype(F32)
            acc = kf[pl.ds(8 + r, CH), :] * skt[0:1, :]
            for j in range(1, 4):
                acc = acc + kf[pl.ds(8 + r - j, CH), :] * skt[j:j + 1, :]
            kvs.append((acc * vb[par, pl.ds(r, CH), :].astype(F32)).astype(BF16))
            hch.append(hb[par, :, pl.ds(r, CH)])
        fw = fw_ref[...]
        uu = jnp.dot(fw, _cat(kvs, 1), preferred_element_type=F32)
        hh = lax.dot_general(fw, _cat(hch, 0), (((1,), (1,)), ((), ())), preferred_element_type=F32)
        dvec = dd_ref[:, ch].astype(F32)
        dsel = jnp.where(u == 0, dvec, 0.0)
        for cc in range(PER):
            c = u * PER + cc
            ua, ub = uu[:CH, cc * 128:(cc + 1) * 128], uu[CH:, cc * 128:(cc + 1) * 128]
            us[par][c, 0, 0:CH, :] = ua + ub
            us[par][c, 1, 0:CH, :] = ua
            us[par][c, 2, 0:CH, :] = ub
            hc, hd = hh[:CH, cc * 128:(cc + 1) * 128], hh[CH:, cc * 128:(cc + 1) * 128]
            if cc == 0:
                pc, pd = jnp.where(u == 0, 0.0, hprev[0]), jnp.where(u == 0, 0.0, hprev[1])
            for f in range(CH // 8):
                t = slice(8 * f, 8 * f + 8)
                gc = (hc[t] - pd[t]) if f % 2 == 0 else (hc[t] + pd[t])
                gd = (hd[t] + pc[t]) if f % 2 == 0 else (hd[t] - pc[t])
                if cc == 0:
                    gc = gc + dsel
                hs[par][c, 0, t, :] = gc
                hs[par][c, 1, t, :] = gd - gc
                hs[par][c, 2, t, :] = gd + gc
            pc, pd = hc, hd
        hprev[0] = pc
        hprev[1] = pd
        return hh

    def a_conv(par, u, ff, m):
        t0 = pl.ds(pl.multiple_of((u * PER + ff) * 8, 8), 8)
        for blk in range(NCH // CB):
            i0 = blk * CB
            t = pl.ds(pl.multiple_of((u * PER + ff + zero(blk)) * 8, 8), 8)
            acc = [None] * CB if m == 0 else [ys[par][i0 + j, 0, t0, :] for j in range(CB)]
            win = {}
            for c in range(i0 + CB):
                a = link(us[par][c, m, t, :])
                for j in range(CB):
                    d = i0 + j - c
                    if d < 0:
                        continue
                    if d not in win:
                        win[d] = hs[par][d, m, t, :]
                    pr = a * win[d]
                    acc[j] = pr if acc[j] is None else (acc[j] - pr if m == 2 else acc[j] + pr)
                mark(acc[c % CB], c >= i0)
            for j in range(CB):
                ys[par][i0 + j, m % 2, t0, :] = acc[j]

    def a_inv(par, u):
        yy = _cat([_cat([ys[par][u * PER + cc, 0], ys[par][u * PER + cc, 1]], 0).astype(BF16) for cc in range(PER)], 1)
        y = jnp.dot(_cat([iv_ref[0], iv_ref[1]], 1), yy, preferred_element_type=F32)
        for cc in range(PER):
            r = pl.multiple_of((u * PER + cc) * CH, CH)
            oa_buf[par, pl.ds(r, CH), :] = (
                y[:, cc * 128:(cc + 1) * 128] * qb[par, pl.ds(r, CH), :].astype(F32)).astype(BF16)

    def b_qkv(par, sec, g, first):
        x = _bf([xs[par][c] for c in range(NG)])
        r = jnp.dot(x, _bf([dead(w_p[sec * NG + g]), w_p[sec * NG + g + 1]]), preferred_element_type=F32)
        for e in range(2):
            rr = r[:, e * 128:(e + 1) * 128]
            if sec == 0:
                qs[par][g + e, 0:TM, :] = rr
            else:
                dst = (ks, vs)[sec - 1]
                dst[par][g + e, HIST:HIST + TM, :] = rr
                top = lax.broadcasted_iota(jnp.int32, (8, 128), 0) < 2
                for j in range(HIST // RT):
                    o = TM + RT * j
                    prev = 0.0 if first else dst[1 - par][g + e, o + 14:o + 22, :]
                    dst[par][g + e, RT * j:RT * j + 8, :] = jnp.where(top, prev, dst[par][g + e, o - 2:o + 6, :])
                    dst[par][g + e, RT * j + 8:RT * j + 16, :] = dst[par][g + e, o + 6:o + 14, :]
        return r

    def b_qk(par, u, tt, first):
        lane = lax.broadcasted_iota(jnp.int32, (RT, 128), 1)
        b4, b0 = (lane & 16) != 0, (lane & 1) != 0
        cexp = float(DH ** -0.5 * np.log2(np.e))
        r0 = pl.multiple_of((u * PER + tt) * RT, RT)
        acc = [[None] * WIN for _ in range(2)]
        for wg in range(0, WIN, CB):
            for hf in range(2):
                rq = pl.ds(pl.multiple_of(r0 + 8 * hf + 8 * zero(wg), 8), 8)
                for g in range(NG):
                    q = link(qs[par][g, rq, :])
                    for w in range(wg, wg + CB):
                        pr = q * ks[par][g, pl.ds(HIST + r0 - RT * w + 8 * hf, 8), :]
                        acc[hf][w] = pr if g == 0 else acc[hf][w] + pr
                    if g < NG - 1:
                        mark(acc[hf][wg + g % CB])
                for w in range(wg, wg + CB):
                    mark(acc[hf][w], True)
        lg = [jnp.concatenate([acc[0][w], acc[1][w]], axis=0) for w in range(WIN)]
        lg = [l + jnp.where(b4, pltpu.roll(l, 16, 1), pltpu.roll(l, 112, 1)) for l in lg]
        lg = [l + jnp.where(b0, pltpu.roll(l, 1, 1), pltpu.roll(l, 127, 1)) for l in lg]
        if first:
            pair = (lax.broadcasted_iota(jnp.int32, (RT, 128), 0) // DIL) * RT + (u * PER + tt)
            lg = [jnp.where(pair >= w, lg[w], -1e9 * DH ** 0.5) for w in range(WIN)]
        m = lg[0]
        for w in range(1, WIN):
            m = jnp.maximum(m, lg[w])
        p = [jnp.exp2((l - m) * cexp) for l in lg]
        den = p[0]
        for w in range(1, WIN):
            den = den + p[w]
        inv = pl.reciprocal(den, approx=True)
        inv = inv * (2.0 - den * inv)
        return [e * inv for e in p]

    def b_pv(par, u, tt, p):
        r0 = pl.multiple_of((u * PER + tt) * RT, RT)
        for gg in range(0, NG, CB):
            acc = [[None] * CB for _ in range(2)]
            for hf in range(2):
                for w in range(WIN):
                    pw = link(p[w][8 * hf:8 * hf + 8])
                    for j in range(CB):
                        pr = pw * vs[par][gg + j, pl.ds(HIST + r0 - RT * w + 8 * hf, 8), :]
                        acc[hf][j] = pr if w == 0 else acc[hf][j] + pr
                    if w < WIN - 1:
                        mark(acc[hf][w % CB])
                for j in range(CB):
                    mark(acc[hf][j], True)
            for j in range(CB):
                o = jnp.concatenate([acc[0][j], acc[1][j]], axis=0).astype(BF16)
                ob[par][gg + j, pl.ds(u * PER + tt, 8, stride=PITCH), :] = pltpu.bitcast(o, U32)

    def b_out(par, g):
        o = _bf([_cat([ob[par][c, b * PITCH:b * PITCH + 16, :] for b in range(8)], 0) for c in range(NG)])
        r = jnp.dot(o, _bf([dead(wo_p[g]), wo_p[g + 1]]), preferred_element_type=F32)
        obuf[par, g] = r[:, :128].astype(BF16)
        obuf[par, g + 1] = r[:, 128:].astype(BF16)
        return r

    def loop(fn, link_on=True, rep=1):
        def body(u, carry):
            if rep > 1:
                u = u & (NI - 1)
            chain[:] = []
            dl[0] = None
            cur.update(u=u, link=link_on and LINK, lane=lax.broadcasted_iota(jnp.int32, (8, 128), 1),
                       never=lax.broadcasted_iota(jnp.int32, (8, 128), 1) > u + 1000)
            fn(u)
            return carry
        lax.fori_loop(0, NI * rep, body, 0)

    def step(s, par, s1, s2, s3, first2=False):
        abl = ABL if (s1 and s2 and s3) else 0
        def body(u):
            cur['abl'] = abl
            if first2:
                wo_copy(u).wait()
                _permute_rows(wo_r, wo_tmp, wo_p, u)
            mm = []
            if s1:
                mm += [lambda sec=sec: b_qkv(par, sec, u * GPI, False) for sec in range(3)]
            if s3:
                mm += [lambda: b_out(par, u * GPI)]
                a_inv(par, u)
            for i in range(PER):
                tok = mm[i]() if i < len(mm) else None
                if s2:
                    p = None if abl & 8 else b_qk(1 - par, u, i, first2)
                    for m in range(0 if abl & 4 else 3):
                        a_conv(1 - par, u, i, m)
                    if p is not None:
                        b_pv(1 - par, u, i, p)
                if s1 and i == PER // 2 - 1:
                    tok = a_fwd(par, s, u)
                if tok is not None and s1 and s2 and s3:
                    gate(tok)
            if s1 and not abl & 1:
                x_prep(1 - par, u)

        loop(body, s1, REP if (s1 and s3) else 1)
        if s3:
            start(out_copies(s, par))

    start(x_in(0, 0))
    for n in range(LA):
        w_copy(n).start()
    kf[0:8, :] = jnp.zeros((8, 128), F32)
    wait(x_in(0, 0))

    def head(sec, u):
        if sec < 3:
            n = sec * 4 + u
            w_copy(n).wait()

            @pl.when(n + LA < 12)
            def _():
                w_copy(n + LA).start()
        if sec > 0:
            b_qkv(0, sec - 1, u * GPI, True)
        if sec < 3:
            _permute_cols(w_r, w_p, sec, u)
        if sec == 3:
            a_fwd(0, 0, u)
        if sec % 3 == 0:
            x_prep(sec // 3, u)

    for sec in range(4):
        if sec == 2:
            start(a_in(0, 0) + x_in(1, 1))
        if sec == 3:
            start(a_in(1, 1) + x_in(2, 0) + [wo_copy(n) for n in range(4)])
            wait(a_in(0, 0) + x_in(1, 1))
        loop(lambda u, sec=sec: head(sec, u))

    wait(a_in(1, 1) + x_in(2, 0))
    start(a_in(2, 0) + x_in(3, 1) + q_in(0, 0))
    step(1, 1, True, True, False, first2=True)

    def steady(j, carry):
        for par in range(2):
            s = 2 * j + par
            wait(a_in(s, par) + q_in(s - 2, par))
            start(q_in(s - 1, 1 - par))

            if par == 0:
                wait(x_in(s + 1, 1))
                start(a_in(s + 1, 1))

            @pl.when(j < NG // 2 - 1)
            def _():
                if par == 1:
                    wait(x_in(s + 1, 0))
                    start(a_in(s + 1, 0))
                start(x_in(s + 2, par))

            @pl.when(j > 1)
            def _():
                wait(out_copies(s - 2, par))
            step(s, par, True, True, True)
        return carry

    lax.fori_loop(1, NG // 2, steady, 0)
    wait(q_in(NG - 2, 0) + out_copies(NG - 2, 0))
    start(q_in(NG - 1, 1))
    step(NG, 0, False, True, True)
    wait(q_in(NG - 1, 1) + out_copies(NG - 1, 1))
    step(NG + 1, 1, False, False, True)
    wait(out_copies(NG, 0) + out_copies(NG + 1, 1))


@jax.jit
def pallas_concat_heads__ssm_conv_h3__sliding_local_dilated__prompt_kernel(
    A_q, A_k, A_v, A_shift_k, A_ssm_k, A_ssm_D, B_x, B_wqkv, B_wo,
):
    fw, iv = _dft_mats()
    sp3, sp2 = pltpu.VMEM((NCH, 3, CH + 8, 128), F32), pltpu.VMEM((NCH, 2, CH, 128), F32)
    qsp, ksp = pltpu.VMEM((NG, TM + 8, 128), F32), pltpu.VMEM((NG, HIST + TM + 8, 128), F32)
    xsp, osp = pltpu.VMEM((NG, TM // 2, 128), U32), pltpu.VMEM((NG, 8 * PITCH, 128), U32)
    col = pltpu.VMEM((2, S, 128), BF16)
    hbm, vmem = pl.BlockSpec(memory_space=pl.ANY), pl.BlockSpec(memory_space=pltpu.VMEM)
    out = pl.pallas_call(
        _kernel,
        in_specs=[hbm, hbm, hbm, vmem, hbm, vmem, hbm, hbm, hbm, vmem, vmem],
        out_specs=hbm,
        out_shape=jax.ShapeDtypeStruct((S, 2 * D), BF16),
        scratch_shapes=[
            pltpu.VMEM((3, D, D), BF16), pltpu.VMEM((4, D, 256), BF16),
            pltpu.VMEM((3 * NG, D // 2, 128), U32), pltpu.VMEM((NG, D // 2, 128), U32),
            pltpu.VMEM((2, 8 * 72, 128), U32),
            col, col, col, pltpu.VMEM((2, 128, S), BF16), pltpu.VMEM((2, TM, D), BF16),
            pltpu.VMEM((8 + S, 128), F32), pltpu.VMEM((GPI, 8 * PITCH, 128), U32), xsp, xsp,
            pltpu.VMEM((2, CH, 128), F32),
            sp3, sp3, sp3, sp3, sp2, sp2, qsp, qsp, ksp, ksp, ksp, ksp, osp, osp,
            col, pltpu.VMEM((2, NG, TM, 128), BF16),
            pltpu.SemaphoreType.DMA((16,)), pltpu.SemaphoreType.DMA((10,)),
            pltpu.SemaphoreType.DMA((2 * (NG + 1),)),
        ],
        compiler_params=pltpu.CompilerParams(vmem_limit_bytes=100 * 2 ** 20),
    )(A_q.reshape(S, D), A_k.reshape(S, D), A_v.reshape(S, D), A_shift_k.T, A_ssm_k,
      A_ssm_D.reshape(1, D), B_x.reshape(S, D), B_wqkv, B_wo, fw, iv)
    return out.reshape(1, S, 2 * D)
```

```python
import os
import numpy as np
import jax
import jax.numpy as jnp
from jax import lax
import jax.experimental.pallas as pl
import jax.experimental.pallas.tpu as pltpu

S = 2048
D = 1024
NG = D // 128
CH = 128
NCH = S // CH
TM = S // NG
HIST = 112
PITCH = int(os.environ.get('PITCH', 24))
LA = int(os.environ.get('LA', 2))
WIN, DIL, DH = 8, 2, 32
RT = 16
NI = int(os.environ.get("NI", 4))
PER = NCH // NI
CB = int(os.environ.get('CB', 4))
LINK = int(os.environ.get('LINK', 1))
DLK = int(os.environ.get('DLK', -1))
NOCSE = int(os.environ.get('NOCSE', 1))
QG = int(os.environ.get('QG', 8))
LB = int(os.environ.get('LB', 1))
REP = int(os.environ.get('REP', 1))
ABL = int(os.environ.get('ABL', 0))
UNR = int(os.environ.get('UNR', 2))
FWD = int(os.environ.get('FWD', 3))
GATE = int(os.environ.get('GATE', 8))
GPI = NG // NI
F32, BF16, U32 = jnp.float32, jnp.bfloat16, jnp.uint32


def _dft_mats():
    r = np.arange(CH)
    k = (16 * (r // 16) + 2 * (r % 8) + (r // 8) % 2).astype(np.float64)
    th = 2.0 * np.pi * (k + 0.5) / (2 * CH)
    ang = th[:, None] * np.arange(CH, dtype=np.float64)[None, :]
    fwd = np.concatenate([np.cos(ang), -np.sin(ang)], axis=0)
    inv = fwd.T / CH
    return jnp.asarray(fwd, BF16), jnp.asarray(np.stack([inv[:, :CH], inv[:, CH:]]), BF16)


def _permute_cols(w_ref, wp_ref, sec, q):
    lane = lax.broadcasted_iota(jnp.int32, (8, 128), 1)
    bits = [(lane & (2 << st)) != 0 for st in range(3)]

    def first(i):
        r = pl.ds(pl.multiple_of(q * 256 + i * 16, 16), 16)
        v = [pltpu.bitcast(w_ref[sec, r, g * 128:(g + 1) * 128], U32) for g in range(NG)]
        return [v[0]] + [pltpu.roll(v[g], 2 * g, 1) for g in range(1, NG)]

    def second(i, v):
        t = [v[(-e) % NG] for e in range(NG)]
        for st in range(3):
            t = [jnp.where(bits[st], t[(e - (1 << st)) % NG], t[e]) for e in range(NG)]
        t = [t[0]] + [pltpu.roll(t[e], 128 - 2 * e, 1) for e in range(1, NG)]
        for e in range(NG):
            wp_ref[sec * NG + e, pl.ds(pl.multiple_of(q * 128 + i * 8, 8), 8), :] = t[e]

    ahead = 2
    vs = [first(i) for i in range(ahead)]
    for i in range(16):
        if i + ahead < 16:
            vs.append(first(i + ahead))
        second(i, vs[i])


def _permute_rows(wo_ref, tmp_ref, wp_ref, q):
    for e in range(2):
        w = pltpu.bitcast(wo_ref[q, :, e * 128:(e + 1) * 128], U32)
        for b in range(8):
            tmp_ref[e, b * 72:b * 72 + 64, :] = w[b * 64:(b + 1) * 64, :]
        for a in range(8):
            t = jnp.concatenate([tmp_ref[e, pl.ds(m * 8 + a, 8, stride=72), :] for m in range(8)], axis=0)
            wp_ref[2 * q + e, a * 64:(a + 1) * 64, :] = t


def _cat(parts, axis):
    return parts[0] if len(parts) == 1 else jnp.concatenate(parts, axis=axis)


def _bf(parts):
    return jnp.concatenate([pltpu.bitcast(x, BF16) for x in parts], axis=1)


def _kernel(q_hbm, k_hbm, v_hbm, sk_ref, h_hbm, dd_ref, x_hbm, w_hbm, wo_hbm, fw_ref, iv_ref,
            o_hbm,
            w_r, wo_r, w_p, wo_p, wo_tmp, qb, kb, vb, hb, xb, kf, xn, xs0, xs1, hprev,
            us0, us1, hs0, hs1, ys0, ys1, qs0, qs1, ks0, ks1, vs0, vs1, ob0, ob1,
            oa_buf, obuf, wsem, isem, osem):
    us, hs, ys, xs = (us0, us1), (hs0, hs1), (ys0, ys1), (xs0, xs1)
    qs, ks, vs, ob = (qs0, qs1), (ks0, ks1), (vs0, vs1), (ob0, ob1)
    cur = {}

    chain = []

    def link(x):
        if len(chain) < LB or not cur['link']:
            return x
        return jnp.where(cur['never'], chain.pop(0), x)

    def mark(x, must=False):
        if must or len(chain) < LB:
            chain.append(x)

    dl = [None]

    def zero(i):
        return lax.shift_right_logical(cur['u'] + i, 8) if cur['link'] else 0

    def dead(w):
        if dl[0] is None or DLK < 0:
            return w
        r = DLK * 64
        mid = jnp.where(cur['never'], pltpu.bitcast(dl[0], U32), w[r:r + 8])
        return jnp.concatenate(([w[:r]] if r else []) + [mid, w[r + 8:]], axis=0)

    def gate(r):
        dl[0] = chain[-1]
        if GATE:
            t = r[r.shape[0] - 8:, r.shape[1] - 128:]
            chain[:] = [jnp.where(cur['lane'] > cur['u'] + 1001, t, y) for y in chain]

    def out_copies(step, par):
        t = step - 2
        cps = [pltpu.make_async_copy(oa_buf.at[par], o_hbm.at[:, pl.ds(pl.multiple_of(t * 128, 128), 128)],
                                     osem.at[par * (NG + 1)])]
        for g in range(NG):
            cps.append(pltpu.make_async_copy(
                obuf.at[par, g], o_hbm.at[pl.ds(pl.multiple_of(t * TM, TM), TM), pl.ds(D + g * 128, 128)],
                osem.at[par * (NG + 1) + 1 + g]))
        return cps

    def w_copy(n):
        sec, r = n // 4, pl.ds(pl.multiple_of((n % 4) * 256, 256), 256)
        return pltpu.make_async_copy(w_hbm.at[r, pl.ds(pl.multiple_of(sec * D, D), D)], w_r.at[sec, r], wsem.at[n])

    def wo_copy(n):
        return pltpu.make_async_copy(wo_hbm.at[:, pl.ds(pl.multiple_of(n * 256, 256), 256)], wo_r.at[n],
                                     wsem.at[12 + n])

    def a_in(t, par):
        c = pl.ds(pl.multiple_of(t * 128, 128), 128)
        return [pltpu.make_async_copy(k_hbm.at[:, c], kb.at[par], isem.at[par * 5]),
                pltpu.make_async_copy(v_hbm.at[:, c], vb.at[par], isem.at[par * 5 + 1]),
                pltpu.make_async_copy(h_hbm.at[c, :], hb.at[par], isem.at[par * 5 + 2])]

    def q_in(t, par):
        return [pltpu.make_async_copy(q_hbm.at[:, pl.ds(pl.multiple_of(t * 128, 128), 128)], qb.at[par],
                                      isem.at[par * 5 + 3])]

    def x_in(t, par):
        return [pltpu.make_async_copy(x_hbm.at[pl.ds(pl.multiple_of(t * TM, TM), TM), :], xb.at[par],
                                      isem.at[par * 5 + 4])]

    def start(cps):
        for cp in cps:
            cp.start()

    def wait(cps):
        for cp in cps:
            cp.wait()

    def x_prep(par, u):
        for e in range(GPI):
            g = u * GPI + e
            xv = pltpu.bitcast(xb[par, :, pl.ds(pl.multiple_of(g * 128, 128), 128)], U32)
            for b in range(8):
                xn[e, b * PITCH:b * PITCH + 16, :] = xv[b * 16:(b + 1) * 16]
            rows = [xn[e, pl.ds(n, 8, stride=PITCH), :] for n in range(16)]
            xs[par][g] = jnp.concatenate(rows, axis=0)
            mark(pltpu.bitcast(rows[-1], F32), True)

    def a_fwd(par, t, u):
        ch = pl.ds(pl.multiple_of(t * 128, 128), 128)
        skt = sk_ref[:, ch].astype(F32)
        skt = [jnp.broadcast_to(skt[j:j + 1, :], (8, 128)) for j in range(4)]
        kvs, hch = [], []
        for cc in range(PER):
            r = pl.multiple_of((u * PER + cc) * CH, CH)
            kf[pl.ds(8 + r, CH), :] = kb[par, pl.ds(r, CH), :].astype(F32)
            vv = vb[par, pl.ds(r, CH), :].astype(F32)
            kv = []
            for f in range(0, CH, 8):
                k0 = kf[pl.ds(8 + r + f, 8), :]
                if f % 16 == 0:
                    tk = link(skt[0])
                pr = [k0 * tk] + [kf[pl.ds(8 + r + f - j, 8), :] * skt[j] for j in range(1, 4)]
                kv.append(((pr[0] + pr[1]) + (pr[2] + pr[3])) * vv[f:f + 8])
                if f % 16 == 8:
                    mark(kv[-1 - (f // 16) % 2])
            kvs.append(_cat(kv, 0))
            hch.append(hb[par, :, pl.ds(r, CH)])
        fw = fw_ref[...]
        hh = lax.dot_general(fw, _cat(hch, 0), (((1,), (1,)), ((), ())), preferred_element_type=F32)
        uu = jnp.dot(fw, _cat(kvs, 1).astype(BF16), preferred_element_type=F32)
        dvec = dd_ref[:, ch].astype(F32)
        dsel = jnp.where(u == 0, dvec, 0.0)
        for cc in range(PER):
            c = u * PER + cc
            ua, ub = uu[:CH, cc * 128:(cc + 1) * 128], uu[CH:, cc * 128:(cc + 1) * 128]
            us[par][c, 0, 0:CH, :] = ua + ub
            us[par][c, 1, 0:CH, :] = ua
            us[par][c, 2, 0:CH, :] = ub
            hc, hd = hh[:CH, cc * 128:(cc + 1) * 128], hh[CH:, cc * 128:(cc + 1) * 128]
            if cc == 0:
                pc, pd = jnp.where(u == 0, 0.0, hprev[0]), jnp.where(u == 0, 0.0, hprev[1])
            for f in range(CH // 8):
                t = slice(8 * f, 8 * f + 8)
                gc = (hc[t] - pd[t]) if f % 2 == 0 else (hc[t] + pd[t])
                gd = (hd[t] + pc[t]) if f % 2 == 0 else (hd[t] - pc[t])
                if cc == 0:
                    gc = gc + dsel
                hs[par][c, 0, t, :] = gc
                hs[par][c, 1, t, :] = gd - gc
                hs[par][c, 2, t, :] = gd + gc
            pc, pd = hc, hd
        hprev[0] = pc
        hprev[1] = pd
        return uu

    def a_conv(par, u, ff, m):
        t0 = pl.ds(pl.multiple_of((u * PER + ff) * 8, 8), 8)
        for blk in range(NCH // CB):
            i0 = blk * CB
            t = pl.ds(pl.multiple_of((u * PER + ff + zero(blk)) * 8, 8), 8)
            acc = [None] * CB if m == 0 else [ys[par][i0 + j, 0, t0, :] for j in range(CB)]
            win = {}
            for c in range(i0 + CB):
                a = link(us[par][c, m, t, :])
                for j in range(CB):
                    d = i0 + j - c
                    if d < 0:
                        continue
                    if d not in win:
                        win[d] = hs[par][d, m, t, :]
                    pr = a * win[d]
                    acc[j] = pr if acc[j] is None else (acc[j] - pr if m == 2 else acc[j] + pr)
                mark(acc[c % CB], c >= i0)
            for j in range(CB):
                ys[par][i0 + j, m % 2, t0, :] = acc[j]

    def a_inv(par, u):
        yy = _cat([_cat([ys[par][u * PER + cc, 0], ys[par][u * PER + cc, 1]], 0) for cc in range(PER)], 1).astype(BF16)
        y = jnp.dot(_cat([iv_ref[0], iv_ref[1]], 1), yy, preferred_element_type=F32)
        for cc in range(PER):
            r = pl.multiple_of((u * PER + cc) * CH, CH)
            oa_buf[par, pl.ds(r, CH), :] = (
                y[:, cc * 128:(cc + 1) * 128] * qb[par, pl.ds(r, CH), :].astype(F32)).astype(BF16)

    def b_qkv(par, sec, g, first):
        x = _bf([xs[par][c] for c in range(NG)])
        r = jnp.dot(x, _bf([dead(w_p[sec * NG + g]), w_p[sec * NG + g + 1]]), preferred_element_type=F32)
        for e in range(2):
            rr = r[:, e * 128:(e + 1) * 128]
            if sec == 0:
                qs[par][g + e, 0:TM, :] = rr
            else:
                dst = (ks, vs)[sec - 1]
                dst[par][g + e, HIST:HIST + TM, :] = rr
                top = lax.broadcasted_iota(jnp.int32, (8, 128), 0) < 2
                for j in range(HIST // RT):
                    o = TM + RT * j
                    prev = 0.0 if first else dst[1 - par][g + e, o + 14:o + 22, :]
                    dst[par][g + e, RT * j:RT * j + 8, :] = jnp.where(top, prev, dst[par][g + e, o - 2:o + 6, :])
                    dst[par][g + e, RT * j + 8:RT * j + 16, :] = dst[par][g + e, o + 6:o + 14, :]
        return r

    def b_qk(par, u, tt, first):
        lane = lax.broadcasted_iota(jnp.int32, (RT, 128), 1)
        b4, b0 = (lane & 16) != 0, (lane & 1) != 0
        cexp = float(DH ** -0.5 * np.log2(np.e))
        r0 = pl.multiple_of((u * PER + tt) * RT, RT)
        acc = [[None] * WIN for _ in range(2)]
        for wg in range(0, WIN, CB):
            for hf in range(2):
                rq = pl.ds(pl.multiple_of(r0 + 8 * hf + 8 * zero(wg), 8), 8)
                for g in range(NG):
                    q = link(qs[par][g, rq, :])
                    for w in range(wg, wg + CB):
                        pr = q * ks[par][g, pl.ds(HIST + r0 - RT * w + 8 * hf, 8), :]
                        acc[hf][w] = pr if g == 0 else acc[hf][w] + pr
                    if g < NG - 1:
                        mark(acc[hf][wg + g % CB])
                for w in range(wg, wg + CB):
                    mark(acc[hf][w], True)
        lg = [jnp.concatenate([acc[0][w], acc[1][w]], axis=0) for w in range(WIN)]
        lg = [l + jnp.where(b4, pltpu.roll(l, 16, 1), pltpu.roll(l, 112, 1)) for l in lg]
        lg = [l + jnp.where(b0, pltpu.roll(l, 1, 1), pltpu.roll(l, 127, 1)) for l in lg]
        if first:
            pair = (lax.broadcasted_iota(jnp.int32, (RT, 128), 0) // DIL) * RT + (u * PER + tt)
            lg = [jnp.where(pair >= w, lg[w], -1e9 * DH ** 0.5) for w in range(WIN)]
        m = lg[0]
        for w in range(1, WIN):
            m = jnp.maximum(m, lg[w])
        p = [jnp.exp2((l - m) * cexp) for l in lg]
        den = p[0]
        for w in range(1, WIN):
            den = den + p[w]
        inv = pl.reciprocal(den, approx=True)
        inv = inv * (2.0 - den * inv)
        return [e * inv for e in p]

    def b_pv(par, u, tt, p):
        r0 = pl.multiple_of((u * PER + tt) * RT, RT)
        for gg in range(0, NG, CB):
            acc = [[None] * CB for _ in range(2)]
            for hf in range(2):
                for w in range(WIN):
                    pw = link(p[w][8 * hf:8 * hf + 8])
                    for j in range(CB):
                        pr = pw * vs[par][gg + j, pl.ds(HIST + r0 - RT * w + 8 * hf, 8), :]
                        acc[hf][j] = pr if w == 0 else acc[hf][j] + pr
                    if w < WIN - 1:
                        mark(acc[hf][w % CB])
                for j in range(CB):
                    mark(acc[hf][j], True)
            for j in range(CB):
                o = jnp.concatenate([acc[0][j], acc[1][j]], axis=0).astype(BF16)
                ob[par][gg + j, pl.ds(u * PER + tt, 8, stride=PITCH), :] = pltpu.bitcast(o, U32)

    def b_out(par, g):
        o = _bf([_cat([ob[par][c, b * PITCH:b * PITCH + 16, :] for b in range(8)], 0) for c in range(NG)])
        r = jnp.dot(o, _bf([dead(wo_p[g]), wo_p[g + 1]]), preferred_element_type=F32)
        obuf[par, g] = r[:, :128].astype(BF16)
        obuf[par, g + 1] = r[:, 128:].astype(BF16)
        return r

    def loop(fn, link_on=True, rep=1, unr=1):
        def body(u, carry):
            if rep > 1:
                u = u & (NI // unr - 1)
            chain[:] = []
            dl[0] = None
            lane = lax.broadcasted_iota(jnp.int32, (8, 128), 1)
            cur.update(u=u, link=link_on and LINK, lane=lane, never=lane > u + 1000)
            for j in range(unr):
                fn(u * unr + j)
            return carry
        lax.fori_loop(0, NI * rep // unr, body, 0)

    def step(s, par, s1, s2, s3, first2=False):
        abl = ABL if (s1 and s2 and s3) else 0
        def body(u):
            cur['abl'] = abl
            if first2:
                wo_copy(u).wait()
                _permute_rows(wo_r, wo_tmp, wo_p, u)
            mm = []
            if s1:
                mm += [lambda sec=sec: b_qkv(par, sec, u * GPI, False) for sec in range(3)]
            if s3:
                mm += [lambda: b_out(par, u * GPI)]
                if not abl & 32:
                    a_inv(par, u)
            for i in range(PER):
                tok = mm[i]() if i < len(mm) else None
                if s2:
                    p = None if abl & 8 else b_qk(1 - par, u, i, first2)
                    for m in range(0 if abl & 4 else 3):
                        a_conv(1 - par, u, i, m)
                    if p is not None:
                        b_pv(1 - par, u, i, p)
                if s1 and i == 2 and not abl & 1:
                    x_prep(1 - par, u)
                if s1 and i == FWD and not abl & 16:
                    tok = a_fwd(par, s, u)
                if tok is not None and s1 and s2 and chain and (GATE >> i) & 1:
                    gate(tok)

        loop(body, s1, REP if (s1 and s3) else 1, UNR if (s1 and s3) else 1)
        if s3:
            start(out_copies(s, par))

    start(x_in(0, 0))
    for n in range(LA):
        w_copy(n).start()
    kf[0:8, :] = jnp.zeros((8, 128), F32)
    wait(x_in(0, 0))

    def head(sec, u):
        if sec < 3:
            n = sec * 4 + u
            w_copy(n).wait()

            @pl.when(n + LA < 12)
            def _():
                w_copy(n + LA).start()
        if sec > 0:
            b_qkv(0, sec - 1, u * GPI, True)
        if sec < 3:
            _permute_cols(w_r, w_p, sec, u)
        if sec == 3:
            a_fwd(0, 0, u)
        if sec % 3 == 0:
            x_prep(sec // 3, u)

    for sec in range(4):
        if sec == 2:
            start(a_in(0, 0) + x_in(1, 1))
        if sec == 3:
            start(a_in(1, 1) + x_in(2, 0) + [wo_copy(n) for n in range(4)])
            wait(a_in(0, 0) + x_in(1, 1))
        loop(lambda u, sec=sec: head(sec, u))

    wait(a_in(1, 1) + x_in(2, 0))
    start(a_in(2, 0) + x_in(3, 1) + q_in(0, 0))
    step(1, 1, True, True, False, first2=True)

    def steady(j, carry):
        for par in range(2):
            s = 2 * j + par
            wait(a_in(s, par) + q_in(s - 2, par))
            start(q_in(s - 1, 1 - par))

            if par == 0:
                wait(x_in(s + 1, 1))
                start(a_in(s + 1, 1))

            @pl.when(j < NG // 2 - 1)
            def _():
                if par == 1:
                    wait(x_in(s + 1, 0))
                    start(a_in(s + 1, 0))
                start(x_in(s + 2, par))

            @pl.when(j > 1)
            def _():
                wait(out_copies(s - 2, par))
            step(s, par, True, True, True)
        return carry

    lax.fori_loop(1, NG // 2, steady, 0)
    wait(q_in(NG - 2, 0) + out_copies(NG - 2, 0))
    start(q_in(NG - 1, 1))
    step(NG, 0, False, True, True)
    wait(q_in(NG - 1, 1) + out_copies(NG - 1, 1))
    step(NG + 1, 1, False, False, True)
    wait(out_copies(NG, 0) + out_copies(NG + 1, 1))


@jax.jit
def pallas_concat_heads__ssm_conv_h3__sliding_local_dilated__prompt_kernel(
    A_q, A_k, A_v, A_shift_k, A_ssm_k, A_ssm_D, B_x, B_wqkv, B_wo,
):
    fw, iv = _dft_mats()
    sp3, sp2 = pltpu.VMEM((NCH, 3, CH + 8, 128), F32), pltpu.VMEM((NCH, 2, CH, 128), F32)
    qsp, ksp = pltpu.VMEM((NG, TM + 8, 128), F32), pltpu.VMEM((NG, HIST + TM + 8, 128), F32)
    xsp, osp = pltpu.VMEM((NG, TM // 2, 128), U32), pltpu.VMEM((NG, 8 * PITCH, 128), U32)
    col = pltpu.VMEM((2, S, 128), BF16)
    hbm, vmem = pl.BlockSpec(memory_space=pl.ANY), pl.BlockSpec(memory_space=pltpu.VMEM)
    out = pl.pallas_call(
        _kernel,
        in_specs=[hbm, hbm, hbm, vmem, hbm, vmem, hbm, hbm, hbm, vmem, vmem],
        out_specs=hbm,
        out_shape=jax.ShapeDtypeStruct((S, 2 * D), BF16),
        scratch_shapes=[
            pltpu.VMEM((3, D, D), BF16), pltpu.VMEM((4, D, 256), BF16),
            pltpu.VMEM((3 * NG, D // 2, 128), U32), pltpu.VMEM((NG, D // 2, 128), U32),
            pltpu.VMEM((2, 8 * 72, 128), U32),
            col, col, col, pltpu.VMEM((2, 128, S), BF16), pltpu.VMEM((2, TM, D), BF16),
            pltpu.VMEM((8 + S, 128), F32), pltpu.VMEM((GPI, 8 * PITCH, 128), U32), xsp, xsp,
            pltpu.VMEM((2, CH, 128), F32),
            sp3, sp3, sp3, sp3, sp2, sp2, qsp, qsp, ksp, ksp, ksp, ksp, osp, osp,
            col, pltpu.VMEM((2, NG, TM, 128), BF16),
            pltpu.SemaphoreType.DMA((16,)), pltpu.SemaphoreType.DMA((10,)),
            pltpu.SemaphoreType.DMA((2 * (NG + 1),)),
        ],
        compiler_params=pltpu.CompilerParams(vmem_limit_bytes=100 * 2 ** 20),
    )(A_q.reshape(S, D), A_k.reshape(S, D), A_v.reshape(S, D), A_shift_k.T, A_ssm_k,
      A_ssm_D.reshape(1, D), B_x.reshape(S, D), B_wqkv, B_wo, fw, iv)
    return out.reshape(1, S, 2 * D)
```

```python
import os
import numpy as np
import jax
import jax.numpy as jnp
from jax import lax
import jax.experimental.pallas as pl
import jax.experimental.pallas.tpu as pltpu

S = 2048
D = 1024
NG = D // 128
CH = 128
NCH = S // CH
TM = S // NG
HIST = 112
PITCH = int(os.environ.get('PITCH', 24))
LA = int(os.environ.get('LA', 2))
WIN, DIL, DH = 8, 2, 32
RT = 16
NI = int(os.environ.get("NI", 4))
PER = NCH // NI
CB = int(os.environ.get('CB', 4))
LINK = int(os.environ.get('LINK', 1))
DLK = int(os.environ.get('DLK', -1))
NOCSE = int(os.environ.get('NOCSE', 1))
QG = int(os.environ.get('QG', 8))
LB = int(os.environ.get('LB', 1))
REP = int(os.environ.get('REP', 1))
ABL = int(os.environ.get('ABL', 0))
UNR = int(os.environ.get('UNR', 2))
UNH = int(os.environ.get('UNH', 1))
L8 = int(os.environ.get('L8', 0))
FWD = int(os.environ.get('FWD', 3))
GATE = int(os.environ.get('GATE', 8))
GPI = NG // NI
F32, BF16, U32 = jnp.float32, jnp.bfloat16, jnp.uint32


def _dft_mats():
    r = np.arange(CH)
    k = (16 * (r // 16) + 2 * (r % 8) + (r // 8) % 2).astype(np.float64)
    th = 2.0 * np.pi * (k + 0.5) / (2 * CH)
    ang = th[:, None] * np.arange(CH, dtype=np.float64)[None, :]
    fwd = np.concatenate([np.cos(ang), -np.sin(ang)], axis=0)
    inv = fwd.T / CH
    fwd = fwd.reshape(2, CH // 8, 8, CH).transpose(1, 0, 2, 3).reshape(2 * CH, CH)
    return jnp.asarray(fwd, BF16), jnp.asarray(np.stack([inv[:, :CH], inv[:, CH:]]), BF16)


def _permute_cols(w_ref, wp_ref, sec, q):
    lane = lax.broadcasted_iota(jnp.int32, (8, 128), 1)
    bits = [(lane & (2 << st)) != 0 for st in range(3)]

    def first(i):
        r = pl.ds(pl.multiple_of(q * 256 + i * 16, 16), 16)
        v = [pltpu.bitcast(w_ref[sec, r, g * 128:(g + 1) * 128], U32) for g in range(NG)]
        return [v[0]] + [pltpu.roll(v[g], 2 * g, 1) for g in range(1, NG)]

    def second(i, v):
        t = [v[(-e) % NG] for e in range(NG)]
        for st in range(3):
            t = [jnp.where(bits[st], t[(e - (1 << st)) % NG], t[e]) for e in range(NG)]
        t = [t[0]] + [pltpu.roll(t[e], 128 - 2 * e, 1) for e in range(1, NG)]
        for e in range(NG):
            wp_ref[sec * NG + e, pl.ds(pl.multiple_of(q * 128 + i * 8, 8), 8), :] = t[e]

    ahead = 2
    vs = [first(i) for i in range(ahead)]
    for i in range(16):
        if i + ahead < 16:
            vs.append(first(i + ahead))
        second(i, vs[i])


def _permute_rows(wo_ref, tmp_ref, wp_ref, q):
    for e in range(2):
        w = pltpu.bitcast(wo_ref[q, :, e * 128:(e + 1) * 128], U32)
        for b in range(8):
            tmp_ref[e, b * 72:b * 72 + 64, :] = w[b * 64:(b + 1) * 64, :]
        for a in range(8):
            t = jnp.concatenate([tmp_ref[e, pl.ds(m * 8 + a, 8, stride=72), :] for m in range(8)], axis=0)
            wp_ref[2 * q + e, a * 64:(a + 1) * 64, :] = t


def _cat(parts, axis):
    return parts[0] if len(parts) == 1 else jnp.concatenate(parts, axis=axis)


def _bf(parts):
    return jnp.concatenate([pltpu.bitcast(x, BF16) for x in parts], axis=1)


def _kernel(q_hbm, k_hbm, v_hbm, sk_ref, h_hbm, dd_ref, x_hbm, w_hbm, wo_hbm, fw_ref, iv_ref,
            o_hbm,
            w_r, wo_r, w_p, wo_p, wo_tmp, qb, kb, vb, hb, xb, kf, xn, xs0, xs1, hprev,
            us0, us1, hs0, hs1, ys0, ys1, qs0, qs1, ks0, ks1, vs0, vs1, ob0, ob1,
            oa_buf, obuf, wsem, isem, osem):
    us, hs, ys, xs = (us0, us1), (hs0, hs1), (ys0, ys1), (xs0, xs1)
    qs, ks, vs, ob = (qs0, qs1), (ks0, ks1), (vs0, vs1), (ob0, ob1)
    cur = {}

    chain = []

    def link(x):
        if len(chain) < cur['lb'] or not cur['link']:
            return x
        return jnp.where(cur['never'], chain.pop(0), x)

    def mark(x, must=False):
        if must or len(chain) < cur['lb']:
            chain.append(x)

    dl = [None]

    def zero(i):
        return lax.shift_right_logical(cur['u'] + i, 8) if cur['link'] else 0

    def dead(w):
        if dl[0] is None or DLK < 0:
            return w
        r = DLK * 64
        mid = jnp.where(cur['never'], pltpu.bitcast(dl[0], U32), w[r:r + 8])
        return jnp.concatenate(([w[:r]] if r else []) + [mid, w[r + 8:]], axis=0)

    def gate(r):
        dl[0] = chain[-1]
        if GATE:
            t = r[r.shape[0] - 8:, r.shape[1] - 128:]
            chain[:] = [jnp.where(cur['lane'] > cur['u'] + 1001, t, y) for y in chain]

    def out_copies(step, par, u=None):
        t = step - 2
        n, k = (1, 2 * par) if u is None else (NI, 4 + 2 * u)
        ra = pl.ds(0 if u is None else pl.multiple_of(u * (S // n), S // n), S // n)
        cb = 0 if u is None else pl.multiple_of(u * (D // n), D // n)
        return [pltpu.make_async_copy(oa_buf.at[par, ra], o_hbm.at[ra, pl.ds(pl.multiple_of(t * 128, 128), 128)],
                                      osem.at[k]),
                pltpu.make_async_copy(obuf.at[par, :, pl.ds(cb, D // n)],
                                      o_hbm.at[pl.ds(pl.multiple_of(t * TM, TM), TM), pl.ds(D + cb, D // n)],
                                      osem.at[k + 1])]

    def w_copy(n):
        sec, r = n // 4, pl.ds(pl.multiple_of((n % 4) * 256, 256), 256)
        return pltpu.make_async_copy(w_hbm.at[r, pl.ds(pl.multiple_of(sec * D, D), D)], w_r.at[sec, r], wsem.at[n])

    def wo_copy(n):
        return pltpu.make_async_copy(wo_hbm.at[:, pl.ds(pl.multiple_of(n * 256, 256), 256)], wo_r.at[n],
                                     wsem.at[12 + n])

    def a_in(t, par):
        c = pl.ds(pl.multiple_of(t * 128, 128), 128)
        return [pltpu.make_async_copy(k_hbm.at[:, c], kb.at[par], isem.at[par * 5]),
                pltpu.make_async_copy(v_hbm.at[:, c], vb.at[par], isem.at[par * 5 + 1]),
                pltpu.make_async_copy(h_hbm.at[c, :], hb.at[par], isem.at[par * 5 + 2])]

    def q_in(t, par):
        return [pltpu.make_async_copy(q_hbm.at[:, pl.ds(pl.multiple_of(t * 128, 128), 128)], qb.at[par],
                                      isem.at[par * 5 + 3])]

    def x_in(t, par):
        return [pltpu.make_async_copy(x_hbm.at[pl.ds(pl.multiple_of(t * TM, TM), TM), :], xb.at[par],
                                      isem.at[par * 5 + 4])]

    def start(cps):
        for cp in cps:
            cp.start()

    def wait(cps):
        for cp in cps:
            cp.wait()

    def pin(x):
        x = link(pltpu.bitcast(x, F32))
        mark(x, True)
        return pltpu.bitcast(x, U32)

    def x_prep(par, u):
        for e in range(GPI):
            g = u * GPI + e
            for b in range(8):
                xv = pltpu.bitcast(xb[par, b * 32:(b + 1) * 32, pl.ds(pl.multiple_of(g * 128, 128), 128)], U32)
                xn[e, b * PITCH:b * PITCH + 8, :] = pin(xv[:8])
                xn[e, b * PITCH + 8:b * PITCH + 16, :] = xv[8:]
                yield
        for e in range(GPI):
            for n in range(16):
                xs[par][u * GPI + e, n * 8:(n + 1) * 8, :] = pin(xn[e, pl.ds(n, 8, stride=PITCH), :])
                yield

    def a_fwd(par, t, u):
        ch = pl.ds(pl.multiple_of(t * 128, 128), 128)
        skt = sk_ref[:, ch].astype(F32)
        skt = [jnp.broadcast_to(skt[j:j + 1, :], (8, 128)) for j in range(4)]
        kvs, hch = [], []
        for cc in range(PER):
            r = pl.multiple_of((u * PER + cc) * CH, CH)
            kf[pl.ds(8 + r, CH), :] = kb[par, pl.ds(r, CH), :].astype(F32)
            vv = vb[par, pl.ds(r, CH), :].astype(F32)
            kv = []
            for f in range(0, CH, 8):
                k0 = kf[pl.ds(8 + r + f, 8), :]
                if f % 16 == 0:
                    tk = link(skt[0])
                pr = [k0 * tk] + [kf[pl.ds(8 + r + f - j, 8), :] * skt[j] for j in range(1, 4)]
                kv.append(((pr[0] + pr[1]) + (pr[2] + pr[3])) * vv[f:f + 8])
                if f % 16 == 8:
                    mark(kv[-1 - (f // 16) % 2])
            kvs.append(_cat(kv, 0))
            hch.append(hb[par, :, pl.ds(r, CH)])
        fw = fw_ref[...]
        hh = lax.dot_general(fw, _cat(hch, 0), (((1,), (1,)), ((), ())), preferred_element_type=F32)
        uu = jnp.dot(fw, _cat(kvs, 1).astype(BF16), preferred_element_type=F32)
        dvec = dd_ref[:, ch].astype(F32)
        dsel = jnp.where(u == 0, dvec, 0.0)
        for f in range(CH // 8):
            t, re, im = slice(8 * f, 8 * f + 8), slice(16 * f, 16 * f + 8), slice(16 * f + 8, 16 * f + 16)
            pc, pd = jnp.where(u == 0, 0.0, hprev[0, t, :]), jnp.where(u == 0, 0.0, hprev[1, t, :])
            for cc in range(PER):
                c, l = u * PER + cc, slice(cc * 128, (cc + 1) * 128)
                hc, hd = hh[re, l], hh[im, l]
                gc = (hc - pd) if f % 2 == 0 else (hc + pd)
                gd = (hd + pc) if f % 2 == 0 else (hd - pc)
                if cc == 0:
                    gc = gc + dsel
                hs[par][c, 0, t, :] = gc
                hs[par][c, 1, t, :] = gd - gc
                hs[par][c, 2, t, :] = gd + gc
                pc, pd = hc, hd
                us[par][c, 0, t, :] = uu[re, l] + uu[im, l]
                us[par][c, 1, t, :] = uu[re, l]
                us[par][c, 2, t, :] = uu[im, l]
            hprev[0, t, :] = pc
            hprev[1, t, :] = pd
        return uu

    def a_conv(par, u, ff, m):
        t0 = pl.ds(pl.multiple_of((u * PER + ff) * 8, 8), 8)
        for blk in range(NCH // CB):
            i0 = blk * CB
            t = pl.ds(pl.multiple_of((u * PER + ff + zero(blk)) * 8, 8), 8)
            acc = [None] * CB if m == 0 else [ys[par][i0 + j, 0, t0, :] for j in range(CB)]
            win = {}
            for c in range(i0 + CB):
                a = link(us[par][c, m, t, :])
                for j in range(CB):
                    d = i0 + j - c
                    if d < 0:
                        continue
                    if d not in win:
                        win[d] = hs[par][d, m, t, :]
                    pr = a * win[d]
                    acc[j] = pr if acc[j] is None else (acc[j] - pr if m == 2 else acc[j] + pr)
                mark(acc[c % CB], c >= i0)
            for j in range(CB):
                ys[par][i0 + j, m % 2, t0, :] = acc[j]
            next(cur['side'], None)

    def a_inv(par, u):
        yy = _cat([_cat([ys[par][u * PER + cc, 0], ys[par][u * PER + cc, 1]], 0) for cc in range(PER)], 1).astype(BF16)
        y = jnp.dot(_cat([iv_ref[0], iv_ref[1]], 1), yy, preferred_element_type=F32)
        for cc in range(PER):
            r = pl.multiple_of((u * PER + cc) * CH, CH)
            oa_buf[par, pl.ds(r, CH), :] = (
                y[:, cc * 128:(cc + 1) * 128] * qb[par, pl.ds(r, CH), :].astype(F32)).astype(BF16)

    def b_qkv(par, sec, g, first):
        x = _bf([xs[par][c] for c in range(NG)])
        r = jnp.dot(x, _bf([dead(w_p[sec * NG + g]), w_p[sec * NG + g + 1]]), preferred_element_type=F32)
        for e in range(2):
            rr = r[:, e * 128:(e + 1) * 128]
            if sec == 0:
                qs[par][g + e, 0:TM, :] = rr
            else:
                dst = (ks, vs)[sec - 1]
                dst[par][g + e, HIST:HIST + TM, :] = rr
                top = lax.broadcasted_iota(jnp.int32, (8, 128), 0) < 2
                for j in range(HIST // RT):
                    o = TM + RT * j
                    prev = 0.0 if first else dst[1 - par][g + e, o + 14:o + 22, :]
                    dst[par][g + e, RT * j:RT * j + 8, :] = jnp.where(top, prev, dst[par][g + e, o - 2:o + 6, :])
                    dst[par][g + e, RT * j + 8:RT * j + 16, :] = dst[par][g + e, o + 6:o + 14, :]
        return r

    def b_qk(par, u, tt, first):
        lane = lax.broadcasted_iota(jnp.int32, (RT, 128), 1)
        b4, b0 = (lane & 16) != 0, (lane & 1) != 0
        cexp = float(DH ** -0.5 * np.log2(np.e))
        r0 = pl.multiple_of((u * PER + tt) * RT, RT)
        acc = [[None] * WIN for _ in range(2)]
        for wg in range(0, WIN, CB):
            for hf in range(2):
                rq = pl.ds(pl.multiple_of(r0 + 8 * hf + 8 * zero(wg), 8), 8)
                for g in range(NG):
                    q = link(qs[par][g, rq, :])
                    for w in range(wg, wg + CB):
                        pr = q * ks[par][g, pl.ds(HIST + r0 - RT * w + 8 * hf, 8), :]
                        acc[hf][w] = pr if g == 0 else acc[hf][w] + pr
                    if g < NG - 1:
                        mark(acc[hf][wg + g % CB])
                for w in range(wg, wg + CB):
                    mark(acc[hf][w], True)
        lg = [jnp.concatenate([acc[0][w], acc[1][w]], axis=0) for w in range(WIN)]
        lg = [l + jnp.where(b4, pltpu.roll(l, 16, 1), pltpu.roll(l, 112, 1)) for l in lg]
        lg = [l + jnp.where(b0, pltpu.roll(l, 1, 1), pltpu.roll(l, 127, 1)) for l in lg]
        if first:
            pair = (lax.broadcasted_iota(jnp.int32, (RT, 128), 0) // DIL) * RT + (u * PER + tt)
            lg = [jnp.where(pair >= w, lg[w], -1e9 * DH ** 0.5) for w in range(WIN)]
        m = lg[0]
        for w in range(1, WIN):
            m = jnp.maximum(m, lg[w])
        p = [jnp.exp2((l - m) * cexp) for l in lg]
        den = p[0]
        for w in range(1, WIN):
            den = den + p[w]
        inv = pl.reciprocal(den, approx=True)
        inv = inv * (2.0 - den * inv)
        return [e * inv for e in p]

    def b_pv(par, u, tt, p):
        r0 = pl.multiple_of((u * PER + tt) * RT, RT)
        for gg in range(0, NG, CB):
            acc = [[None] * CB for _ in range(2)]
            for hf in range(2):
                for w in range(WIN):
                    pw = link(p[w][8 * hf:8 * hf + 8])
                    for j in range(CB):
                        pr = pw * vs[par][gg + j, pl.ds(HIST + r0 - RT * w + 8 * hf, 8), :]
                        acc[hf][j] = pr if w == 0 else acc[hf][j] + pr
                    if w < WIN - 1:
                        mark(acc[hf][w % CB])
                for j in range(CB):
                    mark(acc[hf][j], True)
            for j in range(CB):
                o = jnp.concatenate([acc[0][j], acc[1][j]], axis=0).astype(BF16)
                ob[par][gg + j, pl.ds(u * PER + tt, 8, stride=PITCH), :] = pltpu.bitcast(o, U32)

    def b_out(par, g):
        o = _bf([_cat([ob[par][c, b * PITCH:b * PITCH + 16, :] for b in range(8)], 0) for c in range(NG)])
        r = jnp.dot(o, _bf([dead(wo_p[g]), wo_p[g + 1]]), preferred_element_type=F32)
        obuf[par, :, pl.ds(pl.multiple_of(g * 128, 256), 256)] = r.astype(BF16)
        return r

    def loop(fn, link_on=True, rep=1, unr=1):
        def body(u, carry):
            if rep > 1:
                u = u & (NI // unr - 1)
            chain[:] = []
            dl[0] = None
            lane = lax.broadcasted_iota(jnp.int32, (8, 128), 1)
            cur.update(lb=LB if link_on is True else max(link_on, 1), u=u, link=link_on and LINK, lane=lane, never=lane > u + 1000)
            for j in range(unr):
                fn(u * unr + j)
            return carry
        lax.fori_loop(0, NI * rep // unr, body, 0)

    def step(s, par, s1, s2, s3, first2=False):
        abl = ABL if (s1 and s2 and s3) else 0
        def body(u):
            cur['side'] = x_prep(1 - par, u) if s1 else iter(())
            if first2:
                wo_copy(u).wait()
                _permute_rows(wo_r, wo_tmp, wo_p, u)
            mm = []
            if s1:
                mm += [lambda sec=sec: b_qkv(par, sec, u * GPI, False) for sec in range(3)]
            if s3:
                mm += [lambda: b_out(par, u * GPI)]
                if not abl & 32:
                    a_inv(par, u)
            for i in range(PER):
                tok = mm[i]() if i < len(mm) else None
                if s2:
                    p = None if abl & 8 else b_qk(1 - par, u, i, first2)
                    for m in range(0 if abl & 4 else 3):
                        a_conv(1 - par, u, i, m)
                    if p is not None:
                        b_pv(1 - par, u, i, p)
                if s1 and i == FWD and not abl & 16:
                    tok = a_fwd(par, s, u)
                if tok is not None and s1 and s2 and chain and (GATE >> i) & 1:
                    gate(tok)
            if not s2:
                start(out_copies(s, par, u))

        loop(body, s1 or L8, REP if (s1 and s3) else 1, UNR if (s1 and s3) else 1)
        if s2 and s3:
            start(out_copies(s, par))

    start(x_in(0, 0))
    for n in range(LA):
        w_copy(n).start()
    kf[0:8, :] = jnp.zeros((8, 128), F32)
    wait(x_in(0, 0))

    def head(sec, u):
        if sec < 3:
            n = sec * 4 + u
            w_copy(n).wait()

            @pl.when(n + LA < 12)
            def _():
                w_copy(n + LA).start()
        if sec > 0:
            b_qkv(0, sec - 1, u * GPI, True)
        if sec < 3:
            _permute_cols(w_r, w_p, sec, u)
        if sec == 3:
            a_fwd(0, 0, u)
        if sec % 3 == 0:
            list(x_prep(sec // 3, u))

    for sec in range(4):
        if sec == 2:
            start(a_in(0, 0) + x_in(1, 1))
        if sec == 3:
            start(a_in(1, 1) + x_in(2, 0) + [wo_copy(n) for n in range(4)])
            wait(a_in(0, 0) + x_in(1, 1))
        loop(lambda u, sec=sec: head(sec, u), False, 1, UNH if sec else 1)

    wait(a_in(1, 1) + x_in(2, 0))
    start(a_in(2, 0) + x_in(3, 1) + q_in(0, 0))
    step(1, 1, True, True, False, first2=True)

    def steady(j, carry):
        for par in range(2):
            s = 2 * j + par
            wait(a_in(s, par) + q_in(s - 2, par))
            start(q_in(s - 1, 1 - par))

            if par == 0:
                wait(x_in(s + 1, 1))
                start(a_in(s + 1, 1))

            @pl.when(j < NG // 2 - 1)
            def _():
                if par == 1:
                    wait(x_in(s + 1, 0))
                    start(a_in(s + 1, 0))
                start(x_in(s + 2, par))

            @pl.when(j > 1)
            def _():
                wait(out_copies(s - 2, par))
            step(s, par, True, True, True)
        return carry

    lax.fori_loop(1, NG // 2, steady, 0)
    wait(q_in(NG - 2, 0) + out_copies(NG - 2, 0))
    start(q_in(NG - 1, 1))
    step(NG, 0, False, True, True)
    wait(q_in(NG - 1, 1) + out_copies(NG - 1, 1))
    step(NG + 1, 1, False, False, True)
    wait(out_copies(NG, 0) + sum([out_copies(NG + 1, 1, u) for u in range(NI)], []))


@jax.jit
def pallas_concat_heads__ssm_conv_h3__sliding_local_dilated__prompt_kernel(
    A_q, A_k, A_v, A_shift_k, A_ssm_k, A_ssm_D, B_x, B_wqkv, B_wo,
):
    fw, iv = _dft_mats()
    sp3, sp2 = pltpu.VMEM((NCH, 3, CH + 8, 128), F32), pltpu.VMEM((NCH, 2, CH, 128), F32)
    qsp, ksp = pltpu.VMEM((NG, TM + 8, 128), F32), pltpu.VMEM((NG, HIST + TM + 8, 128), F32)
    xsp, osp = pltpu.VMEM((NG, TM // 2, 128), U32), pltpu.VMEM((NG, 8 * PITCH, 128), U32)
    col = pltpu.VMEM((2, S, 128), BF16)
    hbm, vmem = pl.BlockSpec(memory_space=pl.ANY), pl.BlockSpec(memory_space=pltpu.VMEM)
    out = pl.pallas_call(
        _kernel,
        in_specs=[hbm, hbm, hbm, vmem, hbm, vmem, hbm, hbm, hbm, vmem, vmem],
        out_specs=hbm,
        out_shape=jax.ShapeDtypeStruct((S, 2 * D), BF16),
        scratch_shapes=[
            pltpu.VMEM((3, D, D), BF16), pltpu.VMEM((4, D, 256), BF16),
            pltpu.VMEM((3 * NG, D // 2, 128), U32), pltpu.VMEM((NG, D // 2, 128), U32),
            pltpu.VMEM((2, 8 * 72, 128), U32),
            col, col, col, pltpu.VMEM((2, 128, S), BF16), pltpu.VMEM((2, TM, D), BF16),
            pltpu.VMEM((8 + S, 128), F32), pltpu.VMEM((GPI, 8 * PITCH, 128), U32), xsp, xsp,
            pltpu.VMEM((2, CH, 128), F32),
            sp3, sp3, sp3, sp3, sp2, sp2, qsp, qsp, ksp, ksp, ksp, ksp, osp, osp,
            col, pltpu.VMEM((2, TM, D), BF16),
            pltpu.SemaphoreType.DMA((16,)), pltpu.SemaphoreType.DMA((10,)),
            pltpu.SemaphoreType.DMA((4 + 2 * NI,)),
        ],
        compiler_params=pltpu.CompilerParams(vmem_limit_bytes=100 * 2 ** 20),
    )(A_q.reshape(S, D), A_k.reshape(S, D), A_v.reshape(S, D), A_shift_k.T, A_ssm_k,
      A_ssm_D.reshape(1, D), B_x.reshape(S, D), B_wqkv, B_wo, fw, iv)
    return out.reshape(1, S, 2 * D)
```

```python
import numpy as np
import jax
import jax.numpy as jnp
from jax import lax
import jax.experimental.pallas as pl
import jax.experimental.pallas.tpu as pltpu

S = 2048
D = 1024
NG = D // 128
CH = 128
NCH = S // CH
TM = S // NG
HIST = 112
PITCH = 24
WIN, DIL, DH = 8, 2, 32
RT = 16
NI = 4
PER = NCH // NI
CB = 4
UNR = 2
LA = 3
SUB = 2
EXT = (2, 4, 6, 8, 9, 10, 11, 12, 13, 14, 15, 16)
GPI = NG // NI
F32, BF16, U32 = jnp.float32, jnp.bfloat16, jnp.uint32


def _dft_mats():
    r = np.arange(CH)
    k = (16 * (r // 16) + 2 * (r % 8) + (r // 8) % 2).astype(np.float64)
    th = 2.0 * np.pi * (k + 0.5) / (2 * CH)
    ang = th[:, None] * np.arange(CH, dtype=np.float64)[None, :]
    fwd = np.concatenate([np.cos(ang), -np.sin(ang)], axis=0)
    inv = fwd.T / CH
    fwd = fwd.reshape(2, CH // 8, 8, CH).transpose(1, 0, 2, 3).reshape(2 * CH, CH)
    return jnp.asarray(fwd, BF16), jnp.asarray(np.stack([inv[:, :CH], inv[:, CH:]]), BF16)


def _permute_cols(w_ref, wp_ref, sec, q):
    lane = lax.broadcasted_iota(jnp.int32, (8, 128), 1)
    bits = [(lane & (2 << st)) != 0 for st in range(3)]

    def first(i):
        r = pl.ds(pl.multiple_of(q * 256 + i * 16, 16), 16)
        v = [pltpu.bitcast(w_ref[sec, r, g * 128:(g + 1) * 128], U32) for g in range(NG)]
        return [v[0]] + [pltpu.roll(v[g], 2 * g, 1) for g in range(1, NG)]

    def second(i, v):
        t = [v[(-e) % NG] for e in range(NG)]
        for st in range(3):
            t = [jnp.where(bits[st], t[(e - (1 << st)) % NG], t[e]) for e in range(NG)]
        t = [t[0]] + [pltpu.roll(t[e], 128 - 2 * e, 1) for e in range(1, NG)]
        for e in range(NG):
            wp_ref[sec * NG + e, pl.ds(pl.multiple_of(q * 128 + i * 8, 8), 8), :] = t[e]

    ahead = 2
    vs = [first(i) for i in range(ahead)]
    for i in range(16):
        if i + ahead < 16:
            vs.append(first(i + ahead))
        second(i, vs[i])


def _permute_rows(wo_ref, tmp_ref, wp_ref, q):
    for e in range(2):
        w = pltpu.bitcast(wo_ref[q, :, e * 128:(e + 1) * 128], U32)
        for b in range(8):
            tmp_ref[e, b * 72:b * 72 + 64, :] = w[b * 64:(b + 1) * 64, :]
        for a in range(8):
            t = jnp.concatenate([tmp_ref[e, pl.ds(m * 8 + a, 8, stride=72), :] for m in range(8)], axis=0)
            wp_ref[2 * q + e, a * 64:(a + 1) * 64, :] = t


def _cat(parts, axis):
    return parts[0] if len(parts) == 1 else jnp.concatenate(parts, axis=axis)


def _bf(parts):
    return jnp.concatenate([pltpu.bitcast(x, BF16) for x in parts], axis=1)


def _kernel(q_hbm, k_hbm, v_hbm, sk_ref, h_hbm, dd_ref, x_hbm, w_hbm, wo_hbm, fw_ref, iv_ref,
            o_hbm,
            w_r, wo_r, w_p, wo_p, wo_tmp, qb, kb, vb, hb, xb, kf, xn, xs0, xs1, hprev,
            us0, us1, hs0, hs1, ys0, ys1, qs0, qs1, ks0, ks1, vs0, vs1, ob0, ob1,
            oa_buf, obuf, wsem, isem, osem):
    us, hs, ys, xs = (us0, us1), (hs0, hs1), (ys0, ys1), (xs0, xs1)
    qs, ks, vs, ob = (qs0, qs1), (ks0, ks1), (vs0, vs1), (ob0, ob1)
    cur = {}

    chain = []

    def link(x):
        if len(chain) < cur['lb'] or not cur['link']:
            return x
        return jnp.where(cur['never'], chain.pop(0), x)

    def mark(x, must=False):
        if must or len(chain) < cur['lb']:
            chain.append(x)

    def zero(i):
        return lax.shift_right_logical(cur['u'] + i, 8) if cur['link'] else 0

    def gate(r):
        t = r[r.shape[0] - 8:, r.shape[1] - 128:]
        chain[:] = [jnp.where(cur['lane'] > cur['u'] + 1001, t, y) for y in chain]

    def out_copies(step, par, u=None):
        t = step - 2
        n, k = (1, 2 * par) if u is None else (NI, 4 + 2 * u)
        ra = pl.ds(0 if u is None else pl.multiple_of(u * (S // n), S // n), S // n)
        cb = 0 if u is None else pl.multiple_of(u * (D // n), D // n)
        return [pltpu.make_async_copy(oa_buf.at[par, ra], o_hbm.at[ra, pl.ds(pl.multiple_of(t * 128, 128), 128)],
                                      osem.at[k]),
                pltpu.make_async_copy(obuf.at[par, :, pl.ds(cb, D // n)],
                                      o_hbm.at[pl.ds(pl.multiple_of(t * TM, TM), TM), pl.ds(D + cb, D // n)],
                                      osem.at[k + 1])]

    def w_copy(n):
        sec, m = n // 4, 256 // SUB
        rows = [pl.ds(pl.multiple_of((n % 4) * 256 + j * m, m), m) for j in range(SUB)]
        return [pltpu.make_async_copy(w_hbm.at[r, pl.ds(pl.multiple_of(sec * D, D), D)], w_r.at[sec, r], wsem.at[n])
                for r in rows]

    def wo_copy(n):
        return pltpu.make_async_copy(wo_hbm.at[:, pl.ds(pl.multiple_of(n * 256, 256), 256)], wo_r.at[n],
                                     wsem.at[12 + n])

    def a_in(t, par):
        c = pl.ds(pl.multiple_of(t * 128, 128), 128)
        return [pltpu.make_async_copy(k_hbm.at[:, c], kb.at[par], isem.at[par * 5]),
                pltpu.make_async_copy(v_hbm.at[:, c], vb.at[par], isem.at[par * 5 + 1]),
                pltpu.make_async_copy(h_hbm.at[c, :], hb.at[par], isem.at[par * 5 + 2])]

    def q_in(t, par):
        return [pltpu.make_async_copy(q_hbm.at[:, pl.ds(pl.multiple_of(t * 128, 128), 128)], qb.at[par],
                                      isem.at[par * 5 + 3])]

    def x_in(t, par):
        return [pltpu.make_async_copy(x_hbm.at[pl.ds(pl.multiple_of(t * TM, TM), TM), :], xb.at[par],
                                      isem.at[par * 5 + 4])]

    def start(cps):
        for cp in cps:
            cp.start()

    def wait(cps):
        for cp in cps:
            cp.wait()

    def pin(x):
        x = link(pltpu.bitcast(x, F32))
        mark(x, True)
        return pltpu.bitcast(x, U32)

    def x_prep(par, u):
        for e in range(GPI):
            g = u * GPI + e
            for b in range(8):
                xv = pltpu.bitcast(xb[par, b * 32:(b + 1) * 32, pl.ds(pl.multiple_of(g * 128, 128), 128)], U32)
                xn[e, b * PITCH:b * PITCH + 8, :] = pin(xv[:8])
                xn[e, b * PITCH + 8:b * PITCH + 16, :] = xv[8:]
                yield
        for e in range(GPI):
            for n in range(16):
                xs[par][u * GPI + e, n * 8:(n + 1) * 8, :] = pin(xn[e, pl.ds(n, 8, stride=PITCH), :])
                yield

    def a_fwd(par, t, u):
        ch = pl.ds(pl.multiple_of(t * 128, 128), 128)
        skt = sk_ref[:, ch].astype(F32)
        skt = [jnp.broadcast_to(skt[j:j + 1, :], (8, 128)) for j in range(4)]
        kvs, hch = [], []
        for cc in range(PER):
            r = pl.multiple_of((u * PER + cc) * CH, CH)
            kf[pl.ds(8 + r, CH), :] = kb[par, pl.ds(r, CH), :].astype(F32)
            vv = vb[par, pl.ds(r, CH), :].astype(F32)
            kv = []
            for f in range(0, CH, 8):
                k0 = kf[pl.ds(8 + r + f, 8), :]
                if f % 16 == 0:
                    tk = link(skt[0])
                pr = [k0 * tk] + [kf[pl.ds(8 + r + f - j, 8), :] * skt[j] for j in range(1, 4)]
                kv.append(((pr[0] + pr[1]) + (pr[2] + pr[3])) * vv[f:f + 8])
                if f % 16 == 8:
                    mark(kv[-1 - (f // 16) % 2])
            kvs.append(_cat(kv, 0))
            hch.append(hb[par, :, pl.ds(r, CH)])
        fw = fw_ref[...]
        hh = lax.dot_general(fw, _cat(hch, 0), (((1,), (1,)), ((), ())), preferred_element_type=F32)
        uu = jnp.dot(fw, _cat(kvs, 1).astype(BF16), preferred_element_type=F32)
        dvec = dd_ref[:, ch].astype(F32)
        dsel = jnp.where(u == 0, dvec, 0.0)
        for f in range(CH // 8):
            t, re, im = slice(8 * f, 8 * f + 8), slice(16 * f, 16 * f + 8), slice(16 * f + 8, 16 * f + 16)
            pc, pd = jnp.where(u == 0, 0.0, hprev[0, t, :]), jnp.where(u == 0, 0.0, hprev[1, t, :])
            for cc in range(PER):
                c, l = u * PER + cc, slice(cc * 128, (cc + 1) * 128)
                hc, hd = hh[re, l], hh[im, l]
                gc = (hc - pd) if f % 2 == 0 else (hc + pd)
                gd = (hd + pc) if f % 2 == 0 else (hd - pc)
                if cc == 0:
                    gc = gc + dsel
                hs[par][c, 0, t, :] = gc
                hs[par][c, 1, t, :] = gd - gc
                hs[par][c, 2, t, :] = gd + gc
                pc, pd = hc, hd
                us[par][c, 0, t, :] = uu[re, l] + uu[im, l]
                us[par][c, 1, t, :] = uu[re, l]
                us[par][c, 2, t, :] = uu[im, l]
            hprev[0, t, :] = pc
            hprev[1, t, :] = pd
        return uu

    def a_conv(par, u, ff, m):
        t0 = pl.ds(pl.multiple_of((u * PER + ff) * 8, 8), 8)
        for blk in range(NCH // CB):
            i0 = blk * CB
            t = pl.ds(pl.multiple_of((u * PER + ff + zero(blk)) * 8, 8), 8)
            acc = [None] * CB if m == 0 else [ys[par][i0 + j, 0, t0, :] for j in range(CB)]
            win = {}
            for c in range(i0 + CB):
                a = link(us[par][c, m, t, :])
                for j in range(CB):
                    d = i0 + j - c
                    if d < 0:
                        continue
                    if d not in win:
                        win[d] = hs[par][d, m, t, :]
                    pr = a * win[d]
                    acc[j] = pr if acc[j] is None else (acc[j] - pr if m == 2 else acc[j] + pr)
                mark(acc[c % CB], c >= i0)
            for j in range(CB):
                ys[par][i0 + j, m % 2, t0, :] = acc[j]
            next(cur['side'], None)

    def a_inv(par, u):
        yy = _cat([_cat([ys[par][u * PER + cc, 0], ys[par][u * PER + cc, 1]], 0) for cc in range(PER)], 1).astype(BF16)
        y = jnp.dot(_cat([iv_ref[0], iv_ref[1]], 1), yy, preferred_element_type=F32)
        for cc in range(PER):
            r = pl.multiple_of((u * PER + cc) * CH, CH)
            oa_buf[par, pl.ds(r, CH), :] = (
                y[:, cc * 128:(cc + 1) * 128] * qb[par, pl.ds(r, CH), :].astype(F32)).astype(BF16)

    def b_qkv(par, sec, g, first):
        x = _bf([xs[par][c] for c in range(NG)])
        r = jnp.dot(x, _bf([w_p[sec * NG + g], w_p[sec * NG + g + 1]]), preferred_element_type=F32)
        for e in range(2):
            rr = r[:, e * 128:(e + 1) * 128]
            if sec == 0:
                qs[par][g + e, 0:TM, :] = rr
            else:
                dst = (ks, vs)[sec - 1]
                dst[par][g + e, HIST:HIST + TM, :] = rr
                top = lax.broadcasted_iota(jnp.int32, (8, 128), 0) < 2
                for j in range(HIST // RT):
                    o = TM + RT * j
                    prev = 0.0 if first else dst[1 - par][g + e, o + 14:o + 22, :]
                    dst[par][g + e, RT * j:RT * j + 8, :] = jnp.where(top, prev, dst[par][g + e, o - 2:o + 6, :])
                    dst[par][g + e, RT * j + 8:RT * j + 16, :] = dst[par][g + e, o + 6:o + 14, :]

    def b_qk(par, u, tt, first):
        lane = lax.broadcasted_iota(jnp.int32, (RT, 128), 1)
        b4, b0 = (lane & 16) != 0, (lane & 1) != 0
        cexp = float(DH ** -0.5 * np.log2(np.e))
        r0 = pl.multiple_of((u * PER + tt) * RT, RT)
        acc = [[None] * WIN for _ in range(2)]
        for wg in range(0, WIN, CB):
            for hf in range(2):
                rq = pl.ds(pl.multiple_of(r0 + 8 * hf + 8 * zero(wg), 8), 8)
                for g in range(NG):
                    q = link(qs[par][g, rq, :])
                    for w in range(wg, wg + CB):
                        pr = q * ks[par][g, pl.ds(HIST + r0 - RT * w + 8 * hf, 8), :]
                        acc[hf][w] = pr if g == 0 else acc[hf][w] + pr
                    if g < NG - 1:
                        mark(acc[hf][wg + g % CB])
                for w in range(wg, wg + CB):
                    mark(acc[hf][w], True)
        lg = [jnp.concatenate([acc[0][w], acc[1][w]], axis=0) for w in range(WIN)]
        lg = [l + jnp.where(b4, pltpu.roll(l, 16, 1), pltpu.roll(l, 112, 1)) for l in lg]
        lg = [l + jnp.where(b0, pltpu.roll(l, 1, 1), pltpu.roll(l, 127, 1)) for l in lg]
        if first:
            pair = (lax.broadcasted_iota(jnp.int32, (RT, 128), 0) // DIL) * RT + (u * PER + tt)
            lg = [jnp.where(pair >= w, lg[w], -1e9 * DH ** 0.5) for w in range(WIN)]
        m = lg[0]
        for w in range(1, WIN):
            m = jnp.maximum(m, lg[w])
        p = [jnp.exp2((l - m) * cexp) for l in lg]
        den = p[0]
        for w in range(1, WIN):
            den = den + p[w]
        inv = pl.reciprocal(den, approx=True)
        inv = inv * (2.0 - den * inv)
        return [e * inv for e in p]

    def b_pv(par, u, tt, p):
        r0 = pl.multiple_of((u * PER + tt) * RT, RT)
        for gg in range(0, NG, CB):
            acc = [[None] * CB for _ in range(2)]
            for hf in range(2):
                for w in range(WIN):
                    pw = link(p[w][8 * hf:8 * hf + 8])
                    for j in range(CB):
                        pr = pw * vs[par][gg + j, pl.ds(HIST + r0 - RT * w + 8 * hf, 8), :]
                        acc[hf][j] = pr if w == 0 else acc[hf][j] + pr
                    if w < WIN - 1:
                        mark(acc[hf][w % CB])
                for j in range(CB):
                    mark(acc[hf][j], True)
            for j in range(CB):
                o = jnp.concatenate([acc[0][j], acc[1][j]], axis=0).astype(BF16)
                ob[par][gg + j, pl.ds(u * PER + tt, 8, stride=PITCH), :] = pltpu.bitcast(o, U32)

    def b_out(par, g):
        o = _bf([_cat([ob[par][c, b * PITCH:b * PITCH + 16, :] for b in range(8)], 0) for c in range(NG)])
        r = jnp.dot(o, _bf([wo_p[g], wo_p[g + 1]]), preferred_element_type=F32)
        obuf[par, :, pl.ds(pl.multiple_of(g * 128, 256), 256)] = r.astype(BF16)

    def loop(fn, lb=1, unr=1):
        def body(u, carry):
            chain[:] = []
            lane = lax.broadcasted_iota(jnp.int32, (8, 128), 1)
            cur.update(lb=max(lb, 1), u=u, link=lb > 0, lane=lane, never=lane > u + 1000)
            for j in range(unr):
                fn(u * unr + j)
            return carry
        lax.fori_loop(0, NI // unr, body, 0)

    def step(s, par, s1, s2, s3, first2=False):
        def body(u):
            cur['side'] = x_prep(1 - par, u) if s1 else iter(())
            if first2:
                wo_copy(u).wait()
                _permute_rows(wo_r, wo_tmp, wo_p, u)
            mm = []
            if s1:
                mm += [lambda sec=sec: b_qkv(par, sec, u * GPI, False) for sec in range(3)]
            if s3:
                mm += [lambda: b_out(par, u * GPI)]
                a_inv(par, u)
            for i in range(PER):
                if i < len(mm):
                    mm[i]()
                if s2:
                    p = b_qk(1 - par, u, i, first2)
                    for m in range(3):
                        a_conv(1 - par, u, i, m)
                    b_pv(1 - par, u, i, p)
            if s1:
                gate(a_fwd(par, s, u))
            if not s2:
                start(out_copies(s, par, u))

        loop(body, 1 if s1 else 3, UNR if (s1 and s3) else 1)
        if s2 and s3:
            start(out_copies(s, par))

    start(x_in(0, 0) + w_copy(0))
    kf[0:8, :] = jnp.zeros((8, 128), F32)
    wait(x_in(0, 0))
    for n in range(1, LA):
        start(w_copy(n))
    extra = dict(zip(EXT, a_in(0, 0) + x_in(1, 1) + a_in(1, 1) + x_in(2, 0) + [wo_copy(n) for n in range(4)]))

    def head(sec, u):
        n = sec * 4 + u
        if sec < 3:
            wait(w_copy(n))

            @pl.when(n + LA < 12)
            def _():
                start(w_copy(n + LA))
        for j in range(4):
            if sec * 4 + j in extra:
                pl.when(u == j)(extra[sec * 4 + j].start)
        if sec > 0:
            b_qkv(0, sec - 1, u * GPI, True)
        if sec < 3:
            _permute_cols(w_r, w_p, sec, u)
        if sec == 3:
            a_fwd(0, 0, u)
        if sec % 3 == 0:
            list(x_prep(sec // 3, u))

    for sec in range(4):
        if sec == 3:
            wait(a_in(0, 0) + x_in(1, 1))
        loop(lambda u, sec=sec: head(sec, u), 0)

    start([cp for n, cp in extra.items() if n >= 16])
    wait(a_in(1, 1) + x_in(2, 0))
    start(a_in(2, 0) + x_in(3, 1) + q_in(0, 0))
    step(1, 1, True, True, False, first2=True)

    def steady(j, carry):
        for par in range(2):
            s = 2 * j + par
            wait(a_in(s, par) + q_in(s - 2, par))
            start(q_in(s - 1, 1 - par))

            if par == 0:
                wait(x_in(s + 1, 1))
                start(a_in(s + 1, 1))

            @pl.when(j < NG // 2 - 1)
            def _():
                if par == 1:
                    wait(x_in(s + 1, 0))
                    start(a_in(s + 1, 0))
                start(x_in(s + 2, par))

            @pl.when(j > 1)
            def _():
                wait(out_copies(s - 2, par))
            step(s, par, True, True, True)
        return carry

    lax.fori_loop(1, NG // 2, steady, 0)
    wait(q_in(NG - 2, 0) + out_copies(NG - 2, 0))
    start(q_in(NG - 1, 1))
    step(NG, 0, False, True, True)
    wait(q_in(NG - 1, 1) + out_copies(NG - 1, 1))
    step(NG + 1, 1, False, False, True)
    wait(out_copies(NG, 0) + sum([out_copies(NG + 1, 1, u) for u in range(NI)], []))


@jax.jit
def pallas_concat_heads__ssm_conv_h3__sliding_local_dilated__prompt_kernel(
    A_q, A_k, A_v, A_shift_k, A_ssm_k, A_ssm_D, B_x, B_wqkv, B_wo,
):
    fw, iv = _dft_mats()
    sp3, sp2 = pltpu.VMEM((NCH, 3, CH + 8, 128), F32), pltpu.VMEM((NCH, 2, CH, 128), F32)
    qsp, ksp = pltpu.VMEM((NG, TM + 8, 128), F32), pltpu.VMEM((NG, HIST + TM + 8, 128), F32)
    xsp, osp = pltpu.VMEM((NG, TM // 2, 128), U32), pltpu.VMEM((NG, 8 * PITCH, 128), U32)
    col = pltpu.VMEM((2, S, 128), BF16)
    hbm, vmem = pl.BlockSpec(memory_space=pl.ANY), pl.BlockSpec(memory_space=pltpu.VMEM)
    out = pl.pallas_call(
        _kernel,
        in_specs=[hbm, hbm, hbm, vmem, hbm, vmem, hbm, hbm, hbm, vmem, vmem],
        out_specs=hbm,
        out_shape=jax.ShapeDtypeStruct((S, 2 * D), BF16),
        scratch_shapes=[
            pltpu.VMEM((3, D, D), BF16), pltpu.VMEM((4, D, 256), BF16),
            pltpu.VMEM((3 * NG, D // 2, 128), U32), pltpu.VMEM((NG, D // 2, 128), U32),
            pltpu.VMEM((2, 8 * 72, 128), U32),
            col, col, col, pltpu.VMEM((2, 128, S), BF16), pltpu.VMEM((2, TM, D), BF16),
            pltpu.VMEM((8 + S, 128), F32), pltpu.VMEM((GPI, 8 * PITCH, 128), U32), xsp, xsp,
            pltpu.VMEM((2, CH, 128), F32),
            sp3, sp3, sp3, sp3, sp2, sp2, qsp, qsp, ksp, ksp, ksp, ksp, osp, osp,
            col, pltpu.VMEM((2, TM, D), BF16),
            pltpu.SemaphoreType.DMA((16,)), pltpu.SemaphoreType.DMA((10,)),
            pltpu.SemaphoreType.DMA((4 + 2 * NI,)),
        ],
        compiler_params=pltpu.CompilerParams(vmem_limit_bytes=100 * 2 ** 20),
    )(A_q.reshape(S, D), A_k.reshape(S, D), A_v.reshape(S, D), A_shift_k.T, A_ssm_k,
      A_ssm_D.reshape(1, D), B_x.reshape(S, D), B_wqkv, B_wo, fw, iv)
    return out.reshape(1, S, 2 * D)
```

```python
import numpy as np
import jax
import jax.numpy as jnp
from jax import lax
import jax.experimental.pallas as pl
import jax.experimental.pallas.tpu as pltpu

S = 2048
D = 1024
NG = D // 128
CH = 128
NCH = S // CH
TM = S // NG
HIST = 112
PITCH = 24
WIN, DIL, DH = 8, 2, 32
RT = 16
NI = 4
PER = NCH // NI
CB = 4
UNR = 2
LA = 3
SUB = 2
EXT = (2, 4, 6, 8, 9, 10, 11, 12, 13, 14, 15, 16)
GPI = NG // NI
F32, BF16, U32 = jnp.float32, jnp.bfloat16, jnp.uint32


def _dft_mats():
    r = np.arange(CH)
    k = (16 * (r // 16) + 2 * (r % 8) + (r // 8) % 2).astype(np.float64)
    th = 2.0 * np.pi * (k + 0.5) / (2 * CH)
    ang = th[:, None] * np.arange(CH, dtype=np.float64)[None, :]
    fwd = np.concatenate([np.cos(ang), -np.sin(ang)], axis=0)
    inv = fwd.T / CH
    fwd = fwd.reshape(2, CH // 8, 8, CH).transpose(1, 0, 2, 3).reshape(2 * CH, CH)
    return jnp.asarray(fwd, BF16), jnp.asarray(np.stack([inv[:, :CH], inv[:, CH:]]), BF16)


def _permute_cols(w_ref, wp_ref, sec, q):
    lane = lax.broadcasted_iota(jnp.int32, (8, 128), 1)
    bits = [(lane & (2 << st)) != 0 for st in range(3)]

    def first(i):
        r = pl.ds(pl.multiple_of(q * 256 + i * 16, 16), 16)
        v = [pltpu.bitcast(w_ref[sec, r, g * 128:(g + 1) * 128], U32) for g in range(NG)]
        return [v[0]] + [pltpu.roll(v[g], 2 * g, 1) for g in range(1, NG)]

    def second(i, v):
        t = [v[(-e) % NG] for e in range(NG)]
        for st in range(3):
            t = [jnp.where(bits[st], t[(e - (1 << st)) % NG], t[e]) for e in range(NG)]
        t = [t[0]] + [pltpu.roll(t[e], 128 - 2 * e, 1) for e in range(1, NG)]
        for e in range(NG):
            wp_ref[sec * NG + e, pl.ds(pl.multiple_of(q * 128 + i * 8, 8), 8), :] = t[e]

    ahead = 2
    vs = [first(i) for i in range(ahead)]
    for i in range(16):
        if i + ahead < 16:
            vs.append(first(i + ahead))
        second(i, vs[i])


def _permute_rows(wo_ref, tmp_ref, wp_ref, q):
    for e in range(2):
        w = pltpu.bitcast(wo_ref[q, :, e * 128:(e + 1) * 128], U32)
        for b in range(8):
            tmp_ref[e, b * 72:b * 72 + 64, :] = w[b * 64:(b + 1) * 64, :]
        for a in range(8):
            t = jnp.concatenate([tmp_ref[e, pl.ds(m * 8 + a, 8, stride=72), :] for m in range(8)], axis=0)
            wp_ref[2 * q + e, a * 64:(a + 1) * 64, :] = t


def _cat(parts, axis):
    return parts[0] if len(parts) == 1 else jnp.concatenate(parts, axis=axis)


def _bf(parts):
    return jnp.concatenate([pltpu.bitcast(x, BF16) for x in parts], axis=1)


def _kernel(q_hbm, k_hbm, v_hbm, sk_hbm, h_hbm, dd_hbm, x_hbm, w_hbm, wo_hbm, fw_hbm, iv_hbm,
            o_hbm,
            sk_ref, dd_ref, fw_ref, iv_ref,
            w_r, wo_r, w_p, wo_p, wo_tmp, qb, kb, vb, hb, xb, kf, xn, xs0, xs1, hprev, ddf,
            us0, us1, hs0, hs1, ys0, ys1, qs0, qs1, ks0, ks1, vs0, vs1, ob0, ob1,
            oa_buf, obuf, wsem, isem, osem):
    us, hs, ys, xs = (us0, us1), (hs0, hs1), (ys0, ys1), (xs0, xs1)
    qs, ks, vs, ob = (qs0, qs1), (ks0, ks1), (vs0, vs1), (ob0, ob1)
    cur = {}

    chain = []

    def link(x):
        if len(chain) < cur['lb'] or not cur['link']:
            return x
        return jnp.where(cur['never'], chain.pop(0), x)

    def mark(x, must=False):
        if must or len(chain) < cur['lb']:
            chain.append(x)

    def zero(i):
        return lax.shift_right_logical(cur['u'] + i, 8) if cur['link'] else 0

    def gate(r):
        t = r[r.shape[0] - 8:, r.shape[1] - 128:]
        chain[:] = [jnp.where(cur['lane'] > cur['u'] + 1001, t, y) for y in chain]

    def out_copies(step, par, u=None):
        t = step - 2
        n, k = (1, 2 * par) if u is None else (NI, 4 + 2 * u)
        ra = pl.ds(0 if u is None else pl.multiple_of(u * (S // n), S // n), S // n)
        cb = 0 if u is None else pl.multiple_of(u * (D // n), D // n)
        return [pltpu.make_async_copy(oa_buf.at[par, ra], o_hbm.at[ra, pl.ds(pl.multiple_of(t * 128, 128), 128)],
                                      osem.at[k]),
                pltpu.make_async_copy(obuf.at[par, :, pl.ds(cb, D // n)],
                                      o_hbm.at[pl.ds(pl.multiple_of(t * TM, TM), TM), pl.ds(D + cb, D // n)],
                                      osem.at[k + 1])]

    def w_copy(n):
        sec, m = n // 4, 256 // SUB
        rows = [pl.ds(pl.multiple_of((n % 4) * 256 + j * m, m), m) for j in range(SUB)]
        return [pltpu.make_async_copy(w_hbm.at[r, pl.ds(pl.multiple_of(sec * D, D), D)], w_r.at[sec, r], wsem.at[n])
                for r in rows]

    def wo_copy(n):
        return pltpu.make_async_copy(wo_hbm.at[:, pl.ds(pl.multiple_of(n * 256, 256), 256)], wo_r.at[n],
                                     wsem.at[12 + n])

    def a_in(t, par):
        c = pl.ds(pl.multiple_of(t * 128, 128), 128)
        return [pltpu.make_async_copy(k_hbm.at[:, c], kb.at[par], isem.at[par * 5]),
                pltpu.make_async_copy(v_hbm.at[:, c], vb.at[par], isem.at[par * 5 + 1]),
                pltpu.make_async_copy(h_hbm.at[c, :], hb.at[par], isem.at[par * 5 + 2])]

    def q_in(t, par):
        return [pltpu.make_async_copy(q_hbm.at[:, pl.ds(pl.multiple_of(t * 128, 128), 128)], qb.at[par],
                                      isem.at[par * 5 + 3])]

    def x_in(t, par):
        return [pltpu.make_async_copy(x_hbm.at[pl.ds(pl.multiple_of(t * TM, TM), TM), :], xb.at[par],
                                      isem.at[par * 5 + 4])]

    def start(cps):
        for cp in cps:
            cp.start()

    def wait(cps):
        for cp in cps:
            cp.wait()

    def pin(x):
        x = link(pltpu.bitcast(x, F32))
        mark(x, True)
        return pltpu.bitcast(x, U32)

    def x_prep(par, u):
        for e in range(GPI):
            g = u * GPI + e
            for b in range(8):
                xv = pltpu.bitcast(xb[par, b * 32:(b + 1) * 32, pl.ds(pl.multiple_of(g * 128, 128), 128)], U32)
                xn[e, b * PITCH:b * PITCH + 8, :] = pin(xv[:8])
                xn[e, b * PITCH + 8:b * PITCH + 16, :] = xv[8:]
                yield
        for e in range(GPI):
            for n in range(16):
                xs[par][u * GPI + e, n * 8:(n + 1) * 8, :] = pin(xn[e, pl.ds(n, 8, stride=PITCH), :])
                yield

    def a_fwd(par, t, u):
        ch = pl.ds(pl.multiple_of(t * 128, 128), 128)
        skt = sk_ref[:, ch].astype(F32)
        skt = [jnp.broadcast_to(skt[j:j + 1, :], (8, 128)) for j in range(4)]
        kvs, hch = [], []
        for cc in range(PER):
            r = pl.multiple_of((u * PER + cc) * CH, CH)
            kf[pl.ds(8 + r, CH), :] = kb[par, pl.ds(r, CH), :].astype(F32)
            vv = vb[par, pl.ds(r, CH), :].astype(F32)
            kv = []
            for f in range(0, CH, 8):
                k0 = kf[pl.ds(8 + r + f, 8), :]
                if f % 16 == 0:
                    tk = link(skt[0])
                pr = [k0 * tk] + [kf[pl.ds(8 + r + f - j, 8), :] * skt[j] for j in range(1, 4)]
                kv.append(((pr[0] + pr[1]) + (pr[2] + pr[3])) * vv[f:f + 8])
                if f % 16 == 8:
                    mark(kv[-1 - (f // 16) % 2])
            kvs.append(_cat(kv, 0))
            hch.append(hb[par, :, pl.ds(r, CH)])
        fw = fw_ref[...]
        hh = lax.dot_general(fw, _cat(hch, 0), (((1,), (1,)), ((), ())), preferred_element_type=F32)
        uu = jnp.dot(fw, _cat(kvs, 1).astype(BF16), preferred_element_type=F32)
        dvec = ddf[pl.ds(t, 1), :]
        dsel = jnp.where(u == 0, dvec, 0.0)
        for f in range(CH // 8):
            t, re, im = slice(8 * f, 8 * f + 8), slice(16 * f, 16 * f + 8), slice(16 * f + 8, 16 * f + 16)
            pc, pd = jnp.where(u == 0, 0.0, hprev[0, t, :]), jnp.where(u == 0, 0.0, hprev[1, t, :])
            for cc in range(PER):
                c, l = u * PER + cc, slice(cc * 128, (cc + 1) * 128)
                hc, hd = hh[re, l], hh[im, l]
                gc = (hc - pd) if f % 2 == 0 else (hc + pd)
                gd = (hd + pc) if f % 2 == 0 else (hd - pc)
                if cc == 0:
                    gc = gc + dsel
                hs[par][c, 0, t, :] = gc
                hs[par][c, 1, t, :] = gd - gc
                hs[par][c, 2, t, :] = gd + gc
                pc, pd = hc, hd
                us[par][c, 0, t, :] = uu[re, l] + uu[im, l]
                us[par][c, 1, t, :] = uu[re, l]
                us[par][c, 2, t, :] = uu[im, l]
            hprev[0, t, :] = pc
            hprev[1, t, :] = pd
        return uu

    def a_conv(par, u, ff, m):
        t0 = pl.ds(pl.multiple_of((u * PER + ff) * 8, 8), 8)
        for blk in range(NCH // CB):
            i0 = blk * CB
            t = pl.ds(pl.multiple_of((u * PER + ff + zero(blk)) * 8, 8), 8)
            acc = [None] * CB if m == 0 else [ys[par][i0 + j, 0, t0, :] for j in range(CB)]
            win = {}
            for c in range(i0 + CB):
                a = link(us[par][c, m, t, :])
                for j in range(CB):
                    d = i0 + j - c
                    if d < 0:
                        continue
                    if d not in win:
                        win[d] = hs[par][d, m, t, :]
                    pr = a * win[d]
                    acc[j] = pr if acc[j] is None else (acc[j] - pr if m == 2 else acc[j] + pr)
                mark(acc[c % CB], c >= i0)
            for j in range(CB):
                ys[par][i0 + j, m % 2, t0, :] = acc[j]
            next(cur['side'], None)

    def a_inv(par, u):
        yy = _cat([_cat([ys[par][u * PER + cc, 0], ys[par][u * PER + cc, 1]], 0) for cc in range(PER)], 1).astype(BF16)
        y = jnp.dot(_cat([iv_ref[0], iv_ref[1]], 1), yy, preferred_element_type=F32)
        for cc in range(PER):
            r = pl.multiple_of((u * PER + cc) * CH, CH)
            oa_buf[par, pl.ds(r, CH), :] = (
                y[:, cc * 128:(cc + 1) * 128] * qb[par, pl.ds(r, CH), :].astype(F32)).astype(BF16)

    def b_qkv(par, sec, g, first):
        x = _bf([xs[par][c] for c in range(NG)])
        r = jnp.dot(x, _bf([w_p[sec * NG + g], w_p[sec * NG + g + 1]]), preferred_element_type=F32)
        for e in range(2):
            rr = r[:, e * 128:(e + 1) * 128]
            if sec == 0:
                qs[par][g + e, 0:TM, :] = rr
            else:
                dst = (ks, vs)[sec - 1]
                dst[par][g + e, HIST:HIST + TM, :] = rr
                top = lax.broadcasted_iota(jnp.int32, (8, 128), 0) < 2
                for j in range(HIST // RT):
                    o = TM + RT * j
                    prev = 0.0 if first else dst[1 - par][g + e, o + 14:o + 22, :]
                    dst[par][g + e, RT * j:RT * j + 8, :] = jnp.where(top, prev, dst[par][g + e, o - 2:o + 6, :])
                    dst[par][g + e, RT * j + 8:RT * j + 16, :] = dst[par][g + e, o + 6:o + 14, :]

    def b_qk(par, u, tt, first):
        lane = lax.broadcasted_iota(jnp.int32, (RT, 128), 1)
        b4, b0 = (lane & 16) != 0, (lane & 1) != 0
        cexp = float(DH ** -0.5 * np.log2(np.e))
        r0 = pl.multiple_of((u * PER + tt) * RT, RT)
        acc = [[None] * WIN for _ in range(2)]
        for wg in range(0, WIN, CB):
            for hf in range(2):
                rq = pl.ds(pl.multiple_of(r0 + 8 * hf + 8 * zero(wg), 8), 8)
                for g in range(NG):
                    q = link(qs[par][g, rq, :])
                    for w in range(wg, wg + CB):
                        pr = q * ks[par][g, pl.ds(HIST + r0 - RT * w + 8 * hf, 8), :]
                        acc[hf][w] = pr if g == 0 else acc[hf][w] + pr
                    if g < NG - 1:
                        mark(acc[hf][wg + g % CB])
                for w in range(wg, wg + CB):
                    mark(acc[hf][w], True)
        lg = [jnp.concatenate([acc[0][w], acc[1][w]], axis=0) for w in range(WIN)]
        lg = [l + jnp.where(b4, pltpu.roll(l, 16, 1), pltpu.roll(l, 112, 1)) for l in lg]
        lg = [l + jnp.where(b0, pltpu.roll(l, 1, 1), pltpu.roll(l, 127, 1)) for l in lg]
        if first:
            pair = (lax.broadcasted_iota(jnp.int32, (RT, 128), 0) // DIL) * RT + (u * PER + tt)
            lg = [jnp.where(pair >= w, lg[w], -1e9 * DH ** 0.5) for w in range(WIN)]
        m = lg[0]
        for w in range(1, WIN):
            m = jnp.maximum(m, lg[w])
        p = [jnp.exp2((l - m) * cexp) for l in lg]
        den = p[0]
        for w in range(1, WIN):
            den = den + p[w]
        inv = pl.reciprocal(den, approx=True)
        inv = inv * (2.0 - den * inv)
        return [e * inv for e in p]

    def b_pv(par, u, tt, p):
        r0 = pl.multiple_of((u * PER + tt) * RT, RT)
        for gg in range(0, NG, CB):
            acc = [[None] * CB for _ in range(2)]
            for hf in range(2):
                for w in range(WIN):
                    pw = link(p[w][8 * hf:8 * hf + 8])
                    for j in range(CB):
                        pr = pw * vs[par][gg + j, pl.ds(HIST + r0 - RT * w + 8 * hf, 8), :]
                        acc[hf][j] = pr if w == 0 else acc[hf][j] + pr
                    if w < WIN - 1:
                        mark(acc[hf][w % CB])
                for j in range(CB):
                    mark(acc[hf][j], True)
            for j in range(CB):
                o = jnp.concatenate([acc[0][j], acc[1][j]], axis=0).astype(BF16)
                ob[par][gg + j, pl.ds(u * PER + tt, 8, stride=PITCH), :] = pltpu.bitcast(o, U32)

    def b_out(par, g):
        o = _bf([_cat([ob[par][c, b * PITCH:b * PITCH + 16, :] for b in range(8)], 0) for c in range(NG)])
        r = jnp.dot(o, _bf([wo_p[g], wo_p[g + 1]]), preferred_element_type=F32)
        obuf[par, :, pl.ds(pl.multiple_of(g * 128, 256), 256)] = r.astype(BF16)

    def loop(fn, lb=1, unr=1):
        def body(u, carry):
            chain[:] = []
            lane = lax.broadcasted_iota(jnp.int32, (8, 128), 1)
            cur.update(lb=max(lb, 1), u=u, link=lb > 0, lane=lane, never=lane > u + 1000)
            for j in range(unr):
                fn(u * unr + j)
            return carry
        lax.fori_loop(0, NI // unr, body, 0)

    def step(s, par, s1, s2, s3, first2=False):
        def body(u):
            cur['side'] = x_prep(1 - par, u) if s1 else iter(())
            if first2:
                wo_copy(u).wait()
                _permute_rows(wo_r, wo_tmp, wo_p, u)
            mm = []
            if s1:
                mm += [lambda sec=sec: b_qkv(par, sec, u * GPI, False) for sec in range(3)]
            if s3:
                mm += [lambda: b_out(par, u * GPI)]
                a_inv(par, u)
            for i in range(PER):
                if i < len(mm):
                    mm[i]()
                if s2:
                    p = b_qk(1 - par, u, i, first2)
                    for m in range(3):
                        a_conv(1 - par, u, i, m)
                    b_pv(1 - par, u, i, p)
            if s1:
                gate(a_fwd(par, s, u))
            if not s2:
                start(out_copies(s, par, u))

        loop(body, 1 if s1 else 3, UNR if (s1 and s3) else 1)
        if s2 and s3:
            start(out_copies(s, par))

    start(x_in(0, 0) + w_copy(0))
    kf[0:8, :] = jnp.zeros((8, 128), F32)
    wait(x_in(0, 0))
    for n in range(1, LA):
        start(w_copy(n))
    small = [pltpu.make_async_copy(a, b, isem.at[10 + i]) for i, (a, b) in enumerate(
        [(sk_hbm, sk_ref), (dd_hbm, dd_ref), (fw_hbm, fw_ref), (iv_hbm, iv_ref)])]
    start(small)
    extra = dict(zip(EXT, a_in(0, 0) + x_in(1, 1) + a_in(1, 1) + x_in(2, 0) + [wo_copy(n) for n in range(4)]))

    def head(sec, u):
        n = sec * 4 + u
        if sec < 3:
            wait(w_copy(n))

            @pl.when(n + LA < 12)
            def _():
                start(w_copy(n + LA))
        for j in range(4):
            if sec * 4 + j in extra:
                pl.when(u == j)(extra[sec * 4 + j].start)
        if sec > 0:
            b_qkv(0, sec - 1, u * GPI, True)
        if sec < 3:
            _permute_cols(w_r, w_p, sec, u)
        if sec == 3:
            a_fwd(0, 0, u)
        if sec % 3 == 0:
            list(x_prep(sec // 3, u))

    for sec in range(4):
        if sec == 3:
            wait(small + a_in(0, 0) + x_in(1, 1))
            ddf[...] = dd_ref[...].astype(F32)
        loop(lambda u, sec=sec: head(sec, u), 0)

    start([cp for n, cp in extra.items() if n >= 16])
    wait(a_in(1, 1) + x_in(2, 0))
    start(a_in(2, 0) + x_in(3, 1) + q_in(0, 0))
    step(1, 1, True, True, False, first2=True)

    def steady(j, carry):
        for par in range(2):
            s = 2 * j + par
            wait(a_in(s, par) + q_in(s - 2, par))
            start(q_in(s - 1, 1 - par))

            if par == 0:
                wait(x_in(s + 1, 1))
                start(a_in(s + 1, 1))

            @pl.when(j < NG // 2 - 1)
            def _():
                if par == 1:
                    wait(x_in(s + 1, 0))
                    start(a_in(s + 1, 0))
                start(x_in(s + 2, par))

            @pl.when(j > 1)
            def _():
                wait(out_copies(s - 2, par))
            step(s, par, True, True, True)
        return carry

    lax.fori_loop(1, NG // 2, steady, 0)
    wait(q_in(NG - 2, 0) + out_copies(NG - 2, 0))
    start(q_in(NG - 1, 1))
    step(NG, 0, False, True, True)
    wait(q_in(NG - 1, 1) + out_copies(NG - 1, 1))
    step(NG + 1, 1, False, False, True)
    wait(out_copies(NG, 0) + sum([out_copies(NG + 1, 1, u) for u in range(NI)], []))


@jax.jit
def pallas_concat_heads__ssm_conv_h3__sliding_local_dilated__prompt_kernel(
    A_q, A_k, A_v, A_shift_k, A_ssm_k, A_ssm_D, B_x, B_wqkv, B_wo,
):
    fw, iv = _dft_mats()
    sp3, sp2 = pltpu.VMEM((NCH, 3, CH + 8, 128), F32), pltpu.VMEM((NCH, 2, CH, 128), F32)
    qsp, ksp = pltpu.VMEM((NG, TM + 8, 128), F32), pltpu.VMEM((NG, HIST + TM + 8, 128), F32)
    xsp, osp = pltpu.VMEM((NG, TM // 2, 128), U32), pltpu.VMEM((NG, 8 * PITCH, 128), U32)
    col = pltpu.VMEM((2, S, 128), BF16)
    hbm = pl.BlockSpec(memory_space=pl.ANY)
    out = pl.pallas_call(
        _kernel,
        in_specs=[hbm] * 11,
        out_specs=hbm,
        out_shape=jax.ShapeDtypeStruct((S, 2 * D), BF16),
        scratch_shapes=[
            pltpu.VMEM((4, D), BF16), pltpu.VMEM((NG, 128), BF16), pltpu.VMEM(fw.shape, BF16), pltpu.VMEM(iv.shape, BF16),
            pltpu.VMEM((3, D, D), BF16), pltpu.VMEM((4, D, 256), BF16),
            pltpu.VMEM((3 * NG, D // 2, 128), U32), pltpu.VMEM((NG, D // 2, 128), U32),
            pltpu.VMEM((2, 8 * 72, 128), U32),
            col, col, col, pltpu.VMEM((2, 128, S), BF16), pltpu.VMEM((2, TM, D), BF16),
            pltpu.VMEM((8 + S, 128), F32), pltpu.VMEM((GPI, 8 * PITCH, 128), U32), xsp, xsp,
            pltpu.VMEM((2, CH, 128), F32), pltpu.VMEM((NG, 128), F32),
            sp3, sp3, sp3, sp3, sp2, sp2, qsp, qsp, ksp, ksp, ksp, ksp, osp, osp,
            col, pltpu.VMEM((2, TM, D), BF16),
            pltpu.SemaphoreType.DMA((16,)), pltpu.SemaphoreType.DMA((14,)),
            pltpu.SemaphoreType.DMA((4 + 2 * NI,)),
        ],
        compiler_params=pltpu.CompilerParams(vmem_limit_bytes=100 * 2 ** 20),
    )(A_q.reshape(S, D), A_k.reshape(S, D), A_v.reshape(S, D), A_shift_k.T, A_ssm_k,
      A_ssm_D.reshape(NG, 128), B_x.reshape(S, D), B_wqkv, B_wo, fw, iv)
    return out.reshape(1, S, 2 * D)
```

```python
import numpy as np
import jax
import jax.numpy as jnp
from jax import lax
import jax.experimental.pallas as pl
import jax.experimental.pallas.tpu as pltpu

S = 2048
D = 1024
NG = D // 128
CH = 128
NCH = S // CH
TM = S // NG
HIST = 112
PITCH = 24
WIN, DIL, DH = 8, 2, 32
RT = 16
NI = 4
PER = NCH // NI
CB = 4
UNR = 2
LA = 3
SUB = 2
EXT = (2, 4, 6, 7, 9, 10, 10, 11, 11, 12, 12, 13)
GPI = NG // NI
F32, BF16, U32 = jnp.float32, jnp.bfloat16, jnp.uint32


def _dft_mats():
    r = np.arange(CH)
    k = (16 * (r // 16) + 2 * (r % 8) + (r // 8) % 2).astype(np.float64)
    th = 2.0 * np.pi * (k + 0.5) / (2 * CH)
    ang = th[:, None] * np.arange(CH, dtype=np.float64)[None, :]
    fwd = np.concatenate([np.cos(ang), -np.sin(ang)], axis=0)
    inv = fwd.T / CH
    fwd = fwd.reshape(2, CH // 8, 8, CH).transpose(1, 0, 2, 3).reshape(2 * CH, CH)
    return jnp.asarray(fwd, BF16), jnp.asarray(np.stack([inv[:, :CH], inv[:, CH:]]), BF16)


def _permute_cols(w_ref, wp_ref, sec, q):
    lane = lax.broadcasted_iota(jnp.int32, (8, 128), 1)
    bits = [(lane & (2 << st)) != 0 for st in range(3)]

    def first(i):
        r = pl.ds(pl.multiple_of(q * 256 + i * 16, 16), 16)
        v = [pltpu.bitcast(w_ref[sec, r, g * 128:(g + 1) * 128], U32) for g in range(NG)]
        return [v[0]] + [pltpu.roll(v[g], 2 * g, 1) for g in range(1, NG)]

    def second(i, v):
        t = [v[(-e) % NG] for e in range(NG)]
        for st in range(3):
            t = [jnp.where(bits[st], t[(e - (1 << st)) % NG], t[e]) for e in range(NG)]
        t = [t[0]] + [pltpu.roll(t[e], 128 - 2 * e, 1) for e in range(1, NG)]
        for e in range(NG):
            wp_ref[sec * NG + e, pl.ds(pl.multiple_of(q * 128 + i * 8, 8), 8), :] = t[e]

    ahead = 2
    vs = [first(i) for i in range(ahead)]
    for i in range(16):
        if i + ahead < 16:
            vs.append(first(i + ahead))
        second(i, vs[i])


def _permute_rows(wo_ref, tmp_ref, wp_ref, q):
    for e in range(2):
        w = pltpu.bitcast(wo_ref[q, :, e * 128:(e + 1) * 128], U32)
        for b in range(8):
            tmp_ref[e, b * 72:b * 72 + 64, :] = w[b * 64:(b + 1) * 64, :]
        for a in range(8):
            t = jnp.concatenate([tmp_ref[e, pl.ds(m * 8 + a, 8, stride=72), :] for m in range(8)], axis=0)
            wp_ref[2 * q + e, a * 64:(a + 1) * 64, :] = t


def _cat(parts, axis):
    return parts[0] if len(parts) == 1 else jnp.concatenate(parts, axis=axis)


def _bf(parts):
    return jnp.concatenate([pltpu.bitcast(x, BF16) for x in parts], axis=1)


def _kernel(q_hbm, k_hbm, v_hbm, sk_hbm, h_hbm, dd_hbm, x_hbm, w_hbm, wo_hbm, fw_hbm, iv_hbm,
            o_hbm,
            sk_ref, dd_ref, fw_ref, iv_ref,
            w_r, wo_r, w_p, wo_p, wo_tmp, qb, kb, vb, hb, xb, kf, xn, xs0, xs1, hprev, ddf,
            us0, us1, hs0, hs1, ys0, ys1, qs0, qs1, ks0, ks1, vs0, vs1, ob0, ob1,
            oa_buf, obuf, wsem, isem, osem):
    us, hs, ys, xs = (us0, us1), (hs0, hs1), (ys0, ys1), (xs0, xs1)
    qs, ks, vs, ob = (qs0, qs1), (ks0, ks1), (vs0, vs1), (ob0, ob1)
    cur = {}

    chain = []

    def link(x):
        if len(chain) < cur['lb'] or not cur['link']:
            return x
        return jnp.where(cur['never'], chain.pop(0), x)

    def mark(x, must=False):
        if must or len(chain) < cur['lb']:
            chain.append(x)

    def zero(i):
        return lax.shift_right_logical(cur['u'] + i, 8) if cur['link'] else 0

    def gate(r):
        t = r[r.shape[0] - 8:, r.shape[1] - 128:]
        chain[:] = [jnp.where(cur['lane'] > cur['u'] + 1001, t, y) for y in chain]

    def out_copies(step, par, u=None):
        t = step - 2
        n, k = (1, 2 * par) if u is None else (NI, 4 + 2 * u)
        ra = pl.ds(0 if u is None else pl.multiple_of(u * (S // n), S // n), S // n)
        cb = 0 if u is None else pl.multiple_of(u * (D // n), D // n)
        return [pltpu.make_async_copy(oa_buf.at[par, ra], o_hbm.at[ra, pl.ds(pl.multiple_of(t * 128, 128), 128)],
                                      osem.at[k]),
                pltpu.make_async_copy(obuf.at[par, :, pl.ds(cb, D // n)],
                                      o_hbm.at[pl.ds(pl.multiple_of(t * TM, TM), TM), pl.ds(D + cb, D // n)],
                                      osem.at[k + 1])]

    def w_copy(n):
        sec, m = 2 - n // 4, 256 // SUB
        rows = [pl.ds(pl.multiple_of((n % 4) * 256 + j * m, m), m) for j in range(SUB)]
        return [pltpu.make_async_copy(w_hbm.at[r, pl.ds(pl.multiple_of(sec * D, D), D)], w_r.at[sec, r], wsem.at[n])
                for r in rows]

    def wo_copy(n):
        return pltpu.make_async_copy(wo_hbm.at[:, pl.ds(pl.multiple_of(n * 256, 256), 256)], wo_r.at[n],
                                     wsem.at[12 + n])

    def a_in(t, par):
        c = pl.ds(pl.multiple_of(t * 128, 128), 128)
        return [pltpu.make_async_copy(k_hbm.at[:, c], kb.at[par], isem.at[par * 5]),
                pltpu.make_async_copy(v_hbm.at[:, c], vb.at[par], isem.at[par * 5 + 1]),
                pltpu.make_async_copy(h_hbm.at[c, :], hb.at[par], isem.at[par * 5 + 2])]

    def q_in(t, par):
        return [pltpu.make_async_copy(q_hbm.at[:, pl.ds(pl.multiple_of(t * 128, 128), 128)], qb.at[par],
                                      isem.at[par * 5 + 3])]

    def x_in(t, par):
        return [pltpu.make_async_copy(x_hbm.at[pl.ds(pl.multiple_of(t * TM, TM), TM), :], xb.at[par],
                                      isem.at[par * 5 + 4])]

    def start(cps):
        for cp in cps:
            cp.start()

    def wait(cps):
        for cp in cps:
            cp.wait()

    def pin(x):
        x = link(pltpu.bitcast(x, F32))
        mark(x, True)
        return pltpu.bitcast(x, U32)

    def x_prep(par, u):
        for e in range(GPI):
            g = u * GPI + e
            for b in range(8):
                xv = pltpu.bitcast(xb[par, b * 32:(b + 1) * 32, pl.ds(pl.multiple_of(g * 128, 128), 128)], U32)
                xn[e, b * PITCH:b * PITCH + 8, :] = pin(xv[:8])
                xn[e, b * PITCH + 8:b * PITCH + 16, :] = xv[8:]
                yield
        for e in range(GPI):
            for n in range(16):
                xs[par][u * GPI + e, n * 8:(n + 1) * 8, :] = pin(xn[e, pl.ds(n, 8, stride=PITCH), :])
                yield

    def a_fwd(par, t, u):
        ch = pl.ds(pl.multiple_of(t * 128, 128), 128)
        skt = sk_ref[:, ch].astype(F32)
        skt = [jnp.broadcast_to(skt[j:j + 1, :], (8, 128)) for j in range(4)]
        kvs, hch = [], []
        for cc in range(PER):
            r = pl.multiple_of((u * PER + cc) * CH, CH)
            kf[pl.ds(8 + r, CH), :] = kb[par, pl.ds(r, CH), :].astype(F32)
            vv = vb[par, pl.ds(r, CH), :].astype(F32)
            kv = []
            for f in range(0, CH, 8):
                k0 = kf[pl.ds(8 + r + f, 8), :]
                if f % 16 == 0:
                    tk = link(skt[0])
                pr = [k0 * tk] + [kf[pl.ds(8 + r + f - j, 8), :] * skt[j] for j in range(1, 4)]
                kv.append(((pr[0] + pr[1]) + (pr[2] + pr[3])) * vv[f:f + 8])
                if f % 16 == 8:
                    mark(kv[-1 - (f // 16) % 2])
            kvs.append(_cat(kv, 0))
            hch.append(hb[par, :, pl.ds(r, CH)])
        fw = fw_ref[...]
        hh = lax.dot_general(fw, _cat(hch, 0), (((1,), (1,)), ((), ())), preferred_element_type=F32)
        uu = jnp.dot(fw, _cat(kvs, 1).astype(BF16), preferred_element_type=F32)
        dvec = ddf[pl.ds(t, 1), :]
        dsel = jnp.where(u == 0, dvec, 0.0)
        for f in range(CH // 8):
            t, re, im = slice(8 * f, 8 * f + 8), slice(16 * f, 16 * f + 8), slice(16 * f + 8, 16 * f + 16)
            pc, pd = jnp.where(u == 0, 0.0, hprev[0, t, :]), jnp.where(u == 0, 0.0, hprev[1, t, :])
            for cc in range(PER):
                c, l = u * PER + cc, slice(cc * 128, (cc + 1) * 128)
                hc, hd = hh[re, l], hh[im, l]
                gc = (hc - pd) if f % 2 == 0 else (hc + pd)
                gd = (hd + pc) if f % 2 == 0 else (hd - pc)
                if cc == 0:
                    gc = gc + dsel
                hs[par][c, 0, t, :] = gc
                hs[par][c, 1, t, :] = gd - gc
                hs[par][c, 2, t, :] = gd + gc
                pc, pd = hc, hd
                us[par][c, 0, t, :] = uu[re, l] + uu[im, l]
                us[par][c, 1, t, :] = uu[re, l]
                us[par][c, 2, t, :] = uu[im, l]
            hprev[0, t, :] = pc
            hprev[1, t, :] = pd
        return uu

    def a_conv(par, u, ff, m):
        t0 = pl.ds(pl.multiple_of((u * PER + ff) * 8, 8), 8)
        for blk in range(NCH // CB):
            i0 = blk * CB
            t = pl.ds(pl.multiple_of((u * PER + ff + zero(blk)) * 8, 8), 8)
            acc = [None] * CB if m == 0 else [ys[par][i0 + j, 0, t0, :] for j in range(CB)]
            win = {}
            for c in range(i0 + CB):
                a = link(us[par][c, m, t, :])
                for j in range(CB):
                    d = i0 + j - c
                    if d < 0:
                        continue
                    if d not in win:
                        win[d] = hs[par][d, m, t, :]
                    pr = a * win[d]
                    acc[j] = pr if acc[j] is None else (acc[j] - pr if m == 2 else acc[j] + pr)
                mark(acc[c % CB], c >= i0)
            for j in range(CB):
                ys[par][i0 + j, m % 2, t0, :] = acc[j]
            next(cur['side'], None)

    def a_inv(par, u):
        yy = _cat([_cat([ys[par][u * PER + cc, 0], ys[par][u * PER + cc, 1]], 0) for cc in range(PER)], 1).astype(BF16)
        y = jnp.dot(_cat([iv_ref[0], iv_ref[1]], 1), yy, preferred_element_type=F32)
        for cc in range(PER):
            r = pl.multiple_of((u * PER + cc) * CH, CH)
            oa_buf[par, pl.ds(r, CH), :] = (
                y[:, cc * 128:(cc + 1) * 128] * qb[par, pl.ds(r, CH), :].astype(F32)).astype(BF16)

    def history(dst, par, g, first):
        top = lax.broadcasted_iota(jnp.int32, (8, 128), 0) < 2
        for j in range(HIST // RT):
            o = TM + RT * j
            prev = 0.0 if first else dst[1 - par][g, o + 14:o + 22, :]
            dst[par][g, RT * j:RT * j + 8, :] = jnp.where(top, prev, dst[par][g, o - 2:o + 6, :])
            dst[par][g, RT * j + 8:RT * j + 16, :] = dst[par][g, o + 6:o + 14, :]

    def b_qkv(par, sec, g):
        x = _bf([xs[par][c] for c in range(NG)])
        r = jnp.dot(x, _bf([w_p[sec * NG + g], w_p[sec * NG + g + 1]]), preferred_element_type=F32)
        for e in range(2):
            rr = r[:, e * 128:(e + 1) * 128]
            if sec == 0:
                qs[par][g + e, 0:TM, :] = rr
            else:
                (ks, vs)[sec - 1][par][g + e, HIST:HIST + TM, :] = rr
                history((ks, vs)[sec - 1], par, g + e, False)

    def b_qkv0(sec, u):
        x = _bf([xs0[GPI * u + e] for e in range(GPI)])
        k = pl.ds(pl.multiple_of(u * 128, 128), 128)
        dst, o = (qs0, ks0, vs0)[sec], HIST if sec else 0
        for g in range(0, NG, 2):
            r = jnp.dot(x, _bf([w_p[sec * NG + g + e, k, :] for e in range(2)]), preferred_element_type=F32)
            for e in range(2):
                dst[g + e, o:o + TM, :] = jnp.where(u == 0, 0.0, dst[g + e, o:o + TM, :]) + r[:, e * 128:(e + 1) * 128]

    def b_qk(par, u, tt, first):
        lane = lax.broadcasted_iota(jnp.int32, (RT, 128), 1)
        b4, b0 = (lane & 16) != 0, (lane & 1) != 0
        cexp = float(DH ** -0.5 * np.log2(np.e))
        r0 = pl.multiple_of((u * PER + tt) * RT, RT)
        acc = [[None] * WIN for _ in range(2)]
        for wg in range(0, WIN, CB):
            for hf in range(2):
                rq = pl.ds(pl.multiple_of(r0 + 8 * hf + 8 * zero(wg), 8), 8)
                for g in range(NG):
                    q = link(qs[par][g, rq, :])
                    for w in range(wg, wg + CB):
                        pr = q * ks[par][g, pl.ds(HIST + r0 - RT * w + 8 * hf, 8), :]
                        acc[hf][w] = pr if g == 0 else acc[hf][w] + pr
                    if g < NG - 1:
                        mark(acc[hf][wg + g % CB])
                for w in range(wg, wg + CB):
                    mark(acc[hf][w], True)
        lg = [jnp.concatenate([acc[0][w], acc[1][w]], axis=0) for w in range(WIN)]
        lg = [l + jnp.where(b4, pltpu.roll(l, 16, 1), pltpu.roll(l, 112, 1)) for l in lg]
        lg = [l + jnp.where(b0, pltpu.roll(l, 1, 1), pltpu.roll(l, 127, 1)) for l in lg]
        if first:
            pair = (lax.broadcasted_iota(jnp.int32, (RT, 128), 0) // DIL) * RT + (u * PER + tt)
            lg = [jnp.where(pair >= w, lg[w], -1e9 * DH ** 0.5) for w in range(WIN)]
        m = lg[0]
        for w in range(1, WIN):
            m = jnp.maximum(m, lg[w])
        p = [jnp.exp2((l - m) * cexp) for l in lg]
        den = p[0]
        for w in range(1, WIN):
            den = den + p[w]
        inv = pl.reciprocal(den, approx=True)
        inv = inv * (2.0 - den * inv)
        return [e * inv for e in p]

    def b_pv(par, u, tt, p):
        r0 = pl.multiple_of((u * PER + tt) * RT, RT)
        for gg in range(0, NG, CB):
            acc = [[None] * CB for _ in range(2)]
            for hf in range(2):
                for w in range(WIN):
                    pw = link(p[w][8 * hf:8 * hf + 8])
                    for j in range(CB):
                        pr = pw * vs[par][gg + j, pl.ds(HIST + r0 - RT * w + 8 * hf, 8), :]
                        acc[hf][j] = pr if w == 0 else acc[hf][j] + pr
                    if w < WIN - 1:
                        mark(acc[hf][w % CB])
                for j in range(CB):
                    mark(acc[hf][j], True)
            for j in range(CB):
                o = jnp.concatenate([acc[0][j], acc[1][j]], axis=0).astype(BF16)
                ob[par][gg + j, pl.ds(u * PER + tt, 8, stride=PITCH), :] = pltpu.bitcast(o, U32)

    def b_out(par, g):
        o = _bf([_cat([ob[par][c, b * PITCH:b * PITCH + 16, :] for b in range(8)], 0) for c in range(NG)])
        r = jnp.dot(o, _bf([wo_p[g], wo_p[g + 1]]), preferred_element_type=F32)
        obuf[par, :, pl.ds(pl.multiple_of(g * 128, 256), 256)] = r.astype(BF16)

    def loop(fn, lb=1, unr=1):
        def body(u, carry):
            chain[:] = []
            lane = lax.broadcasted_iota(jnp.int32, (8, 128), 1)
            cur.update(lb=max(lb, 1), u=u, link=lb > 0, lane=lane, never=lane > u + 1000)
            for j in range(unr):
                fn(u * unr + j)
            return carry
        lax.fori_loop(0, NI // unr, body, 0)

    def step(s, par, s1, s2, s3, first2=False):
        def body(u):
            cur['side'] = x_prep(1 - par, u) if s1 else iter(())
            if first2:
                wo_copy(u).wait()
                _permute_rows(wo_r, wo_tmp, wo_p, u)
            mm = []
            if s1:
                mm += [lambda sec=sec: b_qkv(par, sec, u * GPI) for sec in range(3)]
            if s3:
                mm += [lambda: b_out(par, u * GPI)]
                a_inv(par, u)
            for i in range(PER):
                if i < len(mm):
                    mm[i]()
                if s2:
                    p = b_qk(1 - par, u, i, first2)
                    for m in range(3):
                        a_conv(1 - par, u, i, m)
                    b_pv(1 - par, u, i, p)
            if s1:
                gate(a_fwd(par, s, u))
            if not s2:
                start(out_copies(s, par, u))

        loop(body, 1 if s1 else 3, UNR if (s1 and s3) else 1)
        if s2 and s3:
            start(out_copies(s, par))

    start(x_in(0, 0) + w_copy(0))
    kf[0:8, :] = jnp.zeros((8, 128), F32)
    wait(x_in(0, 0))
    for n in range(1, LA):
        start(w_copy(n))
    small = [pltpu.make_async_copy(a, b, isem.at[10 + i]) for i, (a, b) in enumerate(
        [(sk_hbm, sk_ref), (dd_hbm, dd_ref), (fw_hbm, fw_ref), (iv_hbm, iv_ref)])]
    start(small)
    extra = {}
    for n, cp in zip(EXT, a_in(0, 0) + x_in(1, 1) + a_in(1, 1) + x_in(2, 0) + [wo_copy(n) for n in range(4)]):
        extra.setdefault(n, []).append(cp)

    def head(ph, u):
        n = ph * 4 + u + 1
        if ph < 2:
            wait(w_copy(n))
        else:
            pl.when(n < 12)(lambda: wait(w_copy(jnp.minimum(n, 11))))
        if ph * 4 + 1 + LA < 12:
            pl.when(n + LA < 12)(lambda: start(w_copy(jnp.minimum(n + LA, 11))))
        for j in range(4):
            if ph * 4 + j + 1 in extra:
                pl.when(u == j)(lambda j=j: start(extra[ph * 4 + j + 1]))
        b_qkv0(2 - ph, u)
        n = jnp.minimum(n, 11)
        _permute_cols(w_r, w_p, 2 - n // 4, n % 4)
        if ph > 0:
            for e in range(GPI):
                history((vs, ks)[ph - 1], 0, GPI * u + e, True)
        if ph == 2:
            a_fwd(0, 0, u)
        if ph != 1:
            list(x_prep(ph // 2, u if ph else jnp.minimum(u + 1, NI - 1)))

    cur.update(lb=1, link=False)
    wait(w_copy(0))
    start(w_copy(LA))
    _permute_cols(w_r, w_p, 2, 0)
    list(x_prep(0, 0))
    for ph in range(3):
        if ph == 2:
            wait(small + a_in(0, 0) + x_in(1, 1))
            ddf[...] = dd_ref[...].astype(F32)
        loop(lambda u, ph=ph: head(ph, u), 0)

    start(extra.get(13, []))
    wait(a_in(1, 1) + x_in(2, 0))
    start(a_in(2, 0) + x_in(3, 1) + q_in(0, 0))
    step(1, 1, True, True, False, first2=True)

    def steady(j, carry):
        for par in range(2):
            s = 2 * j + par
            wait(a_in(s, par) + q_in(s - 2, par))
            start(q_in(s - 1, 1 - par))

            if par == 0:
                wait(x_in(s + 1, 1))
                start(a_in(s + 1, 1))

            @pl.when(j < NG // 2 - 1)
            def _():
                if par == 1:
                    wait(x_in(s + 1, 0))
                    start(a_in(s + 1, 0))
                start(x_in(s + 2, par))

            @pl.when(j > 1)
            def _():
                wait(out_copies(s - 2, par))
            step(s, par, True, True, True)
        return carry

    lax.fori_loop(1, NG // 2, steady, 0)
    wait(q_in(NG - 2, 0) + out_copies(NG - 2, 0))
    start(q_in(NG - 1, 1))
    step(NG, 0, False, True, True)
    wait(q_in(NG - 1, 1) + out_copies(NG - 1, 1))
    step(NG + 1, 1, False, False, True)
    wait(out_copies(NG, 0) + sum([out_copies(NG + 1, 1, u) for u in range(NI)], []))


@jax.jit
def pallas_concat_heads__ssm_conv_h3__sliding_local_dilated__prompt_kernel(
    A_q, A_k, A_v, A_shift_k, A_ssm_k, A_ssm_D, B_x, B_wqkv, B_wo,
):
    fw, iv = _dft_mats()
    sp3, sp2 = pltpu.VMEM((NCH, 3, CH + 8, 128), F32), pltpu.VMEM((NCH, 2, CH, 128), F32)
    qsp, ksp = pltpu.VMEM((NG, TM + 8, 128), F32), pltpu.VMEM((NG, HIST + TM + 8, 128), F32)
    xsp, osp = pltpu.VMEM((NG, TM // 2, 128), U32), pltpu.VMEM((NG, 8 * PITCH, 128), U32)
    col = pltpu.VMEM((2, S, 128), BF16)
    hbm = pl.BlockSpec(memory_space=pl.ANY)
    out = pl.pallas_call(
        _kernel,
        in_specs=[hbm] * 11,
        out_specs=hbm,
        out_shape=jax.ShapeDtypeStruct((S, 2 * D), BF16),
        scratch_shapes=[
            pltpu.VMEM((4, D), BF16), pltpu.VMEM((NG, 128), BF16), pltpu.VMEM(fw.shape, BF16), pltpu.VMEM(iv.shape, BF16),
            pltpu.VMEM((3, D, D), BF16), pltpu.VMEM((4, D, 256), BF16),
            pltpu.VMEM((3 * NG, D // 2, 128), U32), pltpu.VMEM((NG, D // 2, 128), U32),
            pltpu.VMEM((2, 8 * 72, 128), U32),
            col, col, col, pltpu.VMEM((2, 128, S), BF16), pltpu.VMEM((2, TM, D), BF16),
            pltpu.VMEM((8 + S, 128), F32), pltpu.VMEM((GPI, 8 * PITCH, 128), U32), xsp, xsp,
            pltpu.VMEM((2, CH, 128), F32), pltpu.VMEM((NG, 128), F32),
            sp3, sp3, sp3, sp3, sp2, sp2, qsp, qsp, ksp, ksp, ksp, ksp, osp, osp,
            col, pltpu.VMEM((2, TM, D), BF16),
            pltpu.SemaphoreType.DMA((16,)), pltpu.SemaphoreType.DMA((14,)),
            pltpu.SemaphoreType.DMA((4 + 2 * NI,)),
        ],
        compiler_params=pltpu.CompilerParams(vmem_limit_bytes=100 * 2 ** 20),
    )(A_q.reshape(S, D), A_k.reshape(S, D), A_v.reshape(S, D), A_shift_k.T, A_ssm_k,
      A_ssm_D.reshape(NG, 128), B_x.reshape(S, D), B_wqkv, B_wo, fw, iv)
    return out.reshape(1, S, 2 * D)
```

```python
import numpy as np
import jax
import jax.numpy as jnp
from jax import lax
import jax.experimental.pallas as pl
import jax.experimental.pallas.tpu as pltpu

S = 2048
D = 1024
NG = D // 128
CH = 128
NCH = S // CH
TM = S // NG
HIST = 112
PITCH = 24
WIN, DIL, DH = 8, 2, 32
RT = 16
NI = 4
PER = NCH // NI
CB = 4
UNR = 2
LA = 3
SUB = 2
EXT = (2, 5, 7, 9, 10, 11, 12, 13, 14, 11, 12, 13, 14, 15, 15)
EARLY = 1
GPI = NG // NI
F32, BF16, U32 = jnp.float32, jnp.bfloat16, jnp.uint32


def _dft_mats():
    r = np.arange(CH)
    k = (16 * (r // 16) + 2 * (r % 8) + (r // 8) % 2).astype(np.float64)
    th = 2.0 * np.pi * (k + 0.5) / (2 * CH)
    ang = th[:, None] * np.arange(CH, dtype=np.float64)[None, :]
    fwd = np.concatenate([np.cos(ang), -np.sin(ang)], axis=0)
    inv = fwd.T / CH
    fwd = fwd.reshape(2, CH // 8, 8, CH).transpose(1, 0, 2, 3).reshape(2 * CH, CH)
    return jnp.asarray(fwd, BF16), jnp.asarray(np.stack([inv[:, :CH], inv[:, CH:]]), BF16)


def _permute_cols(w_ref, wp_ref, sec, q):
    lane = lax.broadcasted_iota(jnp.int32, (8, 128), 1)
    bits = [(lane & (2 << st)) != 0 for st in range(3)]

    def first(i):
        r = pl.ds(pl.multiple_of(q * 256 + i * 16, 16), 16)
        v = [pltpu.bitcast(w_ref[sec, r, g * 128:(g + 1) * 128], U32) for g in range(NG)]
        return [v[0]] + [pltpu.roll(v[g], 2 * g, 1) for g in range(1, NG)]

    def second(i, v):
        t = [v[(-e) % NG] for e in range(NG)]
        for st in range(3):
            t = [jnp.where(bits[st], t[(e - (1 << st)) % NG], t[e]) for e in range(NG)]
        t = [t[0]] + [pltpu.roll(t[e], 128 - 2 * e, 1) for e in range(1, NG)]
        for e in range(NG):
            wp_ref[sec * NG + e, pl.ds(pl.multiple_of(q * 128 + i * 8, 8), 8), :] = t[e]

    ahead = 2
    vs = [first(i) for i in range(ahead)]
    for i in range(16):
        if i + ahead < 16:
            vs.append(first(i + ahead))
        second(i, vs[i])


def _permute_rows(wo_ref, tmp_ref, wp_ref, q):
    for e in range(2):
        w = pltpu.bitcast(wo_ref[q, :, e * 128:(e + 1) * 128], U32)
        for b in range(8):
            tmp_ref[e, b * 72:b * 72 + 64, :] = w[b * 64:(b + 1) * 64, :]
        for a in range(8):
            t = jnp.concatenate([tmp_ref[e, pl.ds(m * 8 + a, 8, stride=72), :] for m in range(8)], axis=0)
            wp_ref[2 * q + e, a * 64:(a + 1) * 64, :] = t


def _cat(parts, axis):
    return parts[0] if len(parts) == 1 else jnp.concatenate(parts, axis=axis)


def _bf(parts):
    return jnp.concatenate([pltpu.bitcast(x, BF16) for x in parts], axis=1)


def _kernel(q_hbm, k_hbm, v_hbm, sk_hbm, h_hbm, dd_hbm, x_hbm, w_hbm, wo_hbm, fw_hbm, iv_hbm,
            o_hbm,
            sk_ref, dd_ref, fw_ref, iv_ref,
            w_r, wo_r, w_p, wo_p, wo_tmp, qb, kb, vb, hb, xb, kf, xn, xs0, xs1, hprev, ddf,
            us0, us1, hs0, hs1, ys0, ys1, qs0, qs1, ks0, ks1, vs0, vs1, ob0, ob1,
            oa_buf, obuf, wsem, isem, osem):
    us, hs, ys, xs = (us0, us1), (hs0, hs1), (ys0, ys1), (xs0, xs1)
    qs, ks, vs, ob = (qs0, qs1), (ks0, ks1), (vs0, vs1), (ob0, ob1)
    cur = {}

    chain = []

    def link(x):
        if len(chain) < cur['lb'] or not cur['link']:
            return x
        return jnp.where(cur['never'], chain.pop(0), x)

    def mark(x, must=False):
        if must or len(chain) < cur['lb']:
            chain.append(x)

    def zero(i):
        return lax.shift_right_logical(cur['u'] + i, 8) if cur['link'] else 0

    def gate(r):
        t = r[r.shape[0] - 8:, r.shape[1] - 128:]
        chain[:] = [jnp.where(cur['lane'] > cur['u'] + 1001, t, y) for y in chain]

    def out_copies(step, par, u=None):
        t = step - 2
        n, k = (1, 2 * par) if u is None else (NI, 4 + 2 * u)
        ra = pl.ds(0 if u is None else pl.multiple_of(u * (S // n), S // n), S // n)
        cb = 0 if u is None else pl.multiple_of(u * (D // n), D // n)
        return [pltpu.make_async_copy(oa_buf.at[par, ra], o_hbm.at[ra, pl.ds(pl.multiple_of(t * 128, 128), 128)],
                                      osem.at[k]),
                pltpu.make_async_copy(obuf.at[par, :, pl.ds(cb, D // n)],
                                      o_hbm.at[pl.ds(pl.multiple_of(t * TM, TM), TM), pl.ds(D + cb, D // n)],
                                      osem.at[k + 1])]

    def w_copy(n):
        sec, m = 2 - n // 4, 256 // SUB
        rows = [pl.ds(pl.multiple_of((n % 4) * 256 + j * m, m), m) for j in range(SUB)]
        return [pltpu.make_async_copy(w_hbm.at[r, pl.ds(pl.multiple_of(sec * D, D), D)], w_r.at[sec, r], wsem.at[n])
                for r in rows]

    def wo_copy(n):
        return pltpu.make_async_copy(wo_hbm.at[:, pl.ds(pl.multiple_of(n * 256, 256), 256)], wo_r.at[n],
                                     wsem.at[12 + n])

    def a_in(t, par):
        c = pl.ds(pl.multiple_of(t * 128, 128), 128)
        return [pltpu.make_async_copy(k_hbm.at[:, c], kb.at[par], isem.at[par * 5]),
                pltpu.make_async_copy(v_hbm.at[:, c], vb.at[par], isem.at[par * 5 + 1]),
                pltpu.make_async_copy(h_hbm.at[c, :], hb.at[par], isem.at[par * 5 + 2])]

    def early_in(t, u):
        c, sem = pl.ds(t * 128, 128), isem.at[18 + NI * t + u]
        r, xc = pl.ds(pl.multiple_of(u * (S // NI), 128), S // NI), pl.ds(pl.multiple_of(u * 256, 256), 256)
        return [pltpu.make_async_copy(k_hbm.at[r, c], kb.at[t, r], sem),
                pltpu.make_async_copy(v_hbm.at[r, c], vb.at[t, r], sem),
                pltpu.make_async_copy(h_hbm.at[c, r], hb.at[t, :, r], sem),
                pltpu.make_async_copy(x_hbm.at[pl.ds((t + 1) * TM, TM), xc], xb.at[1 - t, :, xc], sem)]

    def q_in(t, par):
        return [pltpu.make_async_copy(q_hbm.at[:, pl.ds(pl.multiple_of(t * 128, 128), 128)], qb.at[par],
                                      isem.at[par * 5 + 3])]

    def x_in(t, par):
        return [pltpu.make_async_copy(x_hbm.at[pl.ds(pl.multiple_of(t * TM, TM), TM), :], xb.at[par],
                                      isem.at[par * 5 + 4])]

    def start(cps):
        for cp in cps:
            cp.start()

    def wait(cps):
        for cp in cps:
            cp.wait()

    def pin(x):
        x = link(pltpu.bitcast(x, F32))
        mark(x, True)
        return pltpu.bitcast(x, U32)

    def x_prep(par, u):
        for e in range(GPI):
            g = u * GPI + e
            for b in range(8):
                xv = pltpu.bitcast(xb[par, b * 32:(b + 1) * 32, pl.ds(pl.multiple_of(g * 128, 128), 128)], U32)
                xn[e, b * PITCH:b * PITCH + 8, :] = pin(xv[:8])
                xn[e, b * PITCH + 8:b * PITCH + 16, :] = xv[8:]
                yield
        for e in range(GPI):
            for n in range(16):
                xs[par][u * GPI + e, n * 8:(n + 1) * 8, :] = pin(xn[e, pl.ds(n, 8, stride=PITCH), :])
                yield

    def a_fwd(par, t, u):
        ch = pl.ds(pl.multiple_of(t * 128, 128), 128)
        skt = sk_ref[:, ch].astype(F32)
        skt = [jnp.broadcast_to(skt[j:j + 1, :], (8, 128)) for j in range(4)]
        kvs, hch = [], []
        for cc in range(PER):
            r = pl.multiple_of((u * PER + cc) * CH, CH)
            kf[pl.ds(8 + r, CH), :] = kb[par, pl.ds(r, CH), :].astype(F32)
            vv = vb[par, pl.ds(r, CH), :].astype(F32)
            kv = []
            for f in range(0, CH, 8):
                k0 = kf[pl.ds(8 + r + f, 8), :]
                if f % 16 == 0:
                    tk = link(skt[0])
                pr = [k0 * tk] + [kf[pl.ds(8 + r + f - j, 8), :] * skt[j] for j in range(1, 4)]
                kv.append(((pr[0] + pr[1]) + (pr[2] + pr[3])) * vv[f:f + 8])
                if f % 16 == 8:
                    mark(kv[-1 - (f // 16) % 2])
            kvs.append(_cat(kv, 0))
            hch.append(hb[par, :, pl.ds(r, CH)])
        fw = fw_ref[...]
        hh = lax.dot_general(fw, _cat(hch, 0), (((1,), (1,)), ((), ())), preferred_element_type=F32)
        uu = jnp.dot(fw, _cat(kvs, 1).astype(BF16), preferred_element_type=F32)
        dvec = ddf[pl.ds(t, 1), :]
        dsel = jnp.where(u == 0, dvec, 0.0)
        for f in range(CH // 8):
            t, re, im = slice(8 * f, 8 * f + 8), slice(16 * f, 16 * f + 8), slice(16 * f + 8, 16 * f + 16)
            pc, pd = jnp.where(u == 0, 0.0, hprev[0, t, :]), jnp.where(u == 0, 0.0, hprev[1, t, :])
            for cc in range(PER):
                c, l = u * PER + cc, slice(cc * 128, (cc + 1) * 128)
                hc, hd = hh[re, l], hh[im, l]
                gc = (hc - pd) if f % 2 == 0 else (hc + pd)
                gd = (hd + pc) if f % 2 == 0 else (hd - pc)
                if cc == 0:
                    gc = gc + dsel
                hs[par][c, 0, t, :] = gc
                hs[par][c, 1, t, :] = gd - gc
                hs[par][c, 2, t, :] = gd + gc
                pc, pd = hc, hd
                us[par][c, 0, t, :] = uu[re, l] + uu[im, l]
                us[par][c, 1, t, :] = uu[re, l]
                us[par][c, 2, t, :] = uu[im, l]
            hprev[0, t, :] = pc
            hprev[1, t, :] = pd
        return uu

    def a_conv(par, u, ff, m):
        t0 = pl.ds(pl.multiple_of((u * PER + ff) * 8, 8), 8)
        for blk in range(NCH // CB):
            i0 = blk * CB
            t = pl.ds(pl.multiple_of((u * PER + ff + zero(blk)) * 8, 8), 8)
            acc = [None] * CB if m == 0 else [ys[par][i0 + j, 0, t0, :] for j in range(CB)]
            win = {}
            for c in range(i0 + CB):
                a = link(us[par][c, m, t, :])
                for j in range(CB):
                    d = i0 + j - c
                    if d < 0:
                        continue
                    if d not in win:
                        win[d] = hs[par][d, m, t, :]
                    pr = a * win[d]
                    acc[j] = pr if acc[j] is None else (acc[j] - pr if m == 2 else acc[j] + pr)
                mark(acc[c % CB], c >= i0)
            for j in range(CB):
                ys[par][i0 + j, m % 2, t0, :] = acc[j]
            next(cur['side'], None)

    def a_inv(par, u):
        yy = _cat([_cat([ys[par][u * PER + cc, 0], ys[par][u * PER + cc, 1]], 0) for cc in range(PER)], 1).astype(BF16)
        y = jnp.dot(_cat([iv_ref[0], iv_ref[1]], 1), yy, preferred_element_type=F32)
        for cc in range(PER):
            r = pl.multiple_of((u * PER + cc) * CH, CH)
            oa_buf[par, pl.ds(r, CH), :] = (
                y[:, cc * 128:(cc + 1) * 128] * qb[par, pl.ds(r, CH), :].astype(F32)).astype(BF16)

    def history(dst, par, g, first):
        top = lax.broadcasted_iota(jnp.int32, (8, 128), 0) < 2
        for j in range(HIST // RT):
            o = TM + RT * j
            prev = 0.0 if first else dst[1 - par][g, o + 14:o + 22, :]
            dst[par][g, RT * j:RT * j + 8, :] = jnp.where(top, prev, dst[par][g, o - 2:o + 6, :])
            dst[par][g, RT * j + 8:RT * j + 16, :] = dst[par][g, o + 6:o + 14, :]

    def b_qkv(par, sec, g):
        x = _bf([xs[par][c] for c in range(NG)])
        r = jnp.dot(x, _bf([w_p[sec * NG + g], w_p[sec * NG + g + 1]]), preferred_element_type=F32)
        for e in range(2):
            rr = r[:, e * 128:(e + 1) * 128]
            if sec == 0:
                qs[par][g + e, 0:TM, :] = rr
            else:
                (ks, vs)[sec - 1][par][g + e, HIST:HIST + TM, :] = rr
                history((ks, vs)[sec - 1], par, g + e, False)

    def b_qkv0(sec, u):
        x = _bf([xs0[GPI * u + e] for e in range(GPI)])
        k = pl.ds(pl.multiple_of(u * 128, 128), 128)
        dst, o = (qs0, ks0, vs0)[sec], HIST if sec else 0
        for g in range(0, NG, 2):
            r = jnp.dot(x, _bf([w_p[sec * NG + g + e, k, :] for e in range(2)]), preferred_element_type=F32)
            for e in range(2):
                dst[g + e, o:o + TM, :] = jnp.where(u == 0, 0.0, dst[g + e, o:o + TM, :]) + r[:, e * 128:(e + 1) * 128]

    def b_qk(par, u, tt, first):
        lane = lax.broadcasted_iota(jnp.int32, (RT, 128), 1)
        b4, b0 = (lane & 16) != 0, (lane & 1) != 0
        cexp = float(DH ** -0.5 * np.log2(np.e))
        r0 = pl.multiple_of((u * PER + tt) * RT, RT)
        acc = [[None] * WIN for _ in range(2)]
        for wg in range(0, WIN, CB):
            for hf in range(2):
                rq = pl.ds(pl.multiple_of(r0 + 8 * hf + 8 * zero(wg), 8), 8)
                for g in range(NG):
                    q = link(qs[par][g, rq, :])
                    for w in range(wg, wg + CB):
                        pr = q * ks[par][g, pl.ds(HIST + r0 - RT * w + 8 * hf, 8), :]
                        acc[hf][w] = pr if g == 0 else acc[hf][w] + pr
                    if g < NG - 1:
                        mark(acc[hf][wg + g % CB])
                for w in range(wg, wg + CB):
                    mark(acc[hf][w], True)
        lg = [jnp.concatenate([acc[0][w], acc[1][w]], axis=0) for w in range(WIN)]
        lg = [l + jnp.where(b4, pltpu.roll(l, 16, 1), pltpu.roll(l, 112, 1)) for l in lg]
        lg = [l + jnp.where(b0, pltpu.roll(l, 1, 1), pltpu.roll(l, 127, 1)) for l in lg]
        if first:
            pair = (lax.broadcasted_iota(jnp.int32, (RT, 128), 0) // DIL) * RT + (u * PER + tt)
            lg = [jnp.where(pair >= w, lg[w], -1e9 * DH ** 0.5) for w in range(WIN)]
        m = lg[0]
        for w in range(1, WIN):
            m = jnp.maximum(m, lg[w])
        p = [jnp.exp2((l - m) * cexp) for l in lg]
        den = p[0]
        for w in range(1, WIN):
            den = den + p[w]
        inv = pl.reciprocal(den, approx=True)
        inv = inv * (2.0 - den * inv)
        return [e * inv for e in p]

    def b_pv(par, u, tt, p):
        r0 = pl.multiple_of((u * PER + tt) * RT, RT)
        for gg in range(0, NG, CB):
            acc = [[None] * CB for _ in range(2)]
            for hf in range(2):
                for w in range(WIN):
                    pw = link(p[w][8 * hf:8 * hf + 8])
                    for j in range(CB):
                        pr = pw * vs[par][gg + j, pl.ds(HIST + r0 - RT * w + 8 * hf, 8), :]
                        acc[hf][j] = pr if w == 0 else acc[hf][j] + pr
                    if w < WIN - 1:
                        mark(acc[hf][w % CB])
                for j in range(CB):
                    mark(acc[hf][j], True)
            for j in range(CB):
                o = jnp.concatenate([acc[0][j], acc[1][j]], axis=0).astype(BF16)
                ob[par][gg + j, pl.ds(u * PER + tt, 8, stride=PITCH), :] = pltpu.bitcast(o, U32)

    def b_out(par, g):
        o = _bf([_cat([ob[par][c, b * PITCH:b * PITCH + 16, :] for b in range(8)], 0) for c in range(NG)])
        r = jnp.dot(o, _bf([wo_p[g], wo_p[g + 1]]), preferred_element_type=F32)
        obuf[par, :, pl.ds(pl.multiple_of(g * 128, 256), 256)] = r.astype(BF16)

    def loop(fn, lb=1, unr=1):
        def body(u, carry):
            chain[:] = []
            lane = lax.broadcasted_iota(jnp.int32, (8, 128), 1)
            cur.update(lb=max(lb, 1), u=u, link=lb > 0, lane=lane, never=lane > u + 1000)
            for j in range(unr):
                fn(u * unr + j)
            return carry
        lax.fori_loop(0, NI // unr, body, 0)

    def step(s, par, s1, s2, s3, first2=False):
        def body(u):
            cur['side'] = x_prep(1 - par, u) if s1 else iter(())
            if first2:
                wait([wo_copy(u)] + early_in(1, u))
                issue(3, u)
                _permute_rows(wo_r, wo_tmp, wo_p, u)
            mm = []
            if s1:
                mm += [lambda sec=sec: b_qkv(par, sec, u * GPI) for sec in range(3)]
            if s3:
                mm += [lambda: b_out(par, u * GPI)]
                a_inv(par, u)
            for i in range(PER):
                if i < len(mm):
                    mm[i]()
                if s2:
                    p = b_qk(1 - par, u, i, first2)
                    for m in range(3):
                        a_conv(1 - par, u, i, m)
                    b_pv(1 - par, u, i, p)
            if s1:
                gate(a_fwd(par, s, u))
            if not s2:
                start(out_copies(s, par, u))

        loop(body, 1 if s1 else 3, UNR if (s1 and s3) else 1)
        if s2 and s3:
            start(out_copies(s, par))

    def x0_in(n):
        c = pl.ds(pl.multiple_of(n * 256, 256), 256)
        return [pltpu.make_async_copy(x_hbm.at[0:TM, c], xb.at[0, :, c], isem.at[14 + n])]

    start(w_copy(0) + x0_in(0))
    kf[0:8, :] = jnp.zeros((8, 128), F32)
    if not EARLY:
        wait(x0_in(0))
    for n in range(1, LA):
        start(w_copy(n) + x0_in(n))
    if EARLY:
        wait(x0_in(0))
    small = [pltpu.make_async_copy(a, b, isem.at[10 + i]) for i, (a, b) in enumerate(
        [(sk_hbm, sk_ref), (dd_hbm, dd_ref), (fw_hbm, fw_ref), (iv_hbm, iv_ref)])]
    extra = {n - LA: x0_in(n) for n in range(LA + 1, NI)}
    later = ([small] + [early_in(t, u) for t in range(2) for u in range(NI)] + [[wo_copy(n)] for n in range(4)]
             + [a_in(2, 0), x_in(3, 1) + q_in(0, 0)])
    for n, cps in zip(EXT, later):
        extra[n] = extra.get(n, []) + cps

    def issue(ph, u):
        for j in range(NI):
            if ph * 4 + j + 1 in extra:
                pl.when(u == j)(lambda j=j: start(extra[ph * 4 + j + 1]))

    def head(ph, u):
        n = ph * 4 + u + 1
        if ph == 0:
            pl.when(n < NI)(lambda: wait(x0_in(jnp.minimum(n, NI - 1))))
        if ph < 2:
            wait(w_copy(n))
        else:
            pl.when(n < 12)(lambda: wait(w_copy(jnp.minimum(n, 11))))
            wait(early_in(0, u))
        if ph * 4 + 1 + LA < 12:
            pl.when(n + LA < 12)(lambda: start(w_copy(jnp.minimum(n + LA, 11))))
        issue(ph, u)
        b_qkv0(2 - ph, u)
        n = jnp.minimum(n, 11)
        _permute_cols(w_r, w_p, 2 - n // 4, n % 4)
        if ph > 0:
            for e in range(GPI):
                history((vs, ks)[ph - 1], 0, GPI * u + e, True)
        if ph == 2:
            a_fwd(0, 0, u)
        if ph != 1:
            list(x_prep(ph // 2, u if ph else jnp.minimum(u + 1, NI - 1)))

    cur.update(lb=1, link=False)
    list(x_prep(0, 0))
    wait(w_copy(0))
    start(w_copy(LA) + x0_in(LA))
    _permute_cols(w_r, w_p, 2, 0)
    for ph in range(3):
        if ph == 2:
            wait(small)
            ddf[...] = dd_ref[...].astype(F32)
        loop(lambda u, ph=ph: head(ph, u), 0)

    step(1, 1, True, True, False, first2=True)

    def steady(j, carry):
        for par in range(2):
            s = 2 * j + par
            wait(a_in(s, par) + q_in(s - 2, par))
            start(q_in(s - 1, 1 - par))

            if par == 0:
                wait(x_in(s + 1, 1))
                start(a_in(s + 1, 1))

            @pl.when(j < NG // 2 - 1)
            def _():
                if par == 1:
                    wait(x_in(s + 1, 0))
                    start(a_in(s + 1, 0))
                start(x_in(s + 2, par))

            @pl.when(j > 1)
            def _():
                wait(out_copies(s - 2, par))
            step(s, par, True, True, True)
        return carry

    lax.fori_loop(1, NG // 2, steady, 0)
    wait(q_in(NG - 2, 0) + out_copies(NG - 2, 0))
    start(q_in(NG - 1, 1))
    step(NG, 0, False, True, True)
    wait(q_in(NG - 1, 1) + out_copies(NG - 1, 1))
    step(NG + 1, 1, False, False, True)
    wait(out_copies(NG, 0) + sum([out_copies(NG + 1, 1, u) for u in range(NI)], []))


@jax.jit
def pallas_concat_heads__ssm_conv_h3__sliding_local_dilated__prompt_kernel(
    A_q, A_k, A_v, A_shift_k, A_ssm_k, A_ssm_D, B_x, B_wqkv, B_wo,
):
    fw, iv = _dft_mats()
    sp3, sp2 = pltpu.VMEM((NCH, 3, CH + 8, 128), F32), pltpu.VMEM((NCH, 2, CH, 128), F32)
    qsp, ksp = pltpu.VMEM((NG, TM + 8, 128), F32), pltpu.VMEM((NG, HIST + TM + 8, 128), F32)
    xsp, osp = pltpu.VMEM((NG, TM // 2, 128), U32), pltpu.VMEM((NG, 8 * PITCH, 128), U32)
    col = pltpu.VMEM((2, S, 128), BF16)
    hbm = pl.BlockSpec(memory_space=pl.ANY)
    out = pl.pallas_call(
        _kernel,
        in_specs=[hbm] * 11,
        out_specs=hbm,
        out_shape=jax.ShapeDtypeStruct((S, 2 * D), BF16),
        scratch_shapes=[
            pltpu.VMEM((4, D), BF16), pltpu.VMEM((NG, 128), BF16), pltpu.VMEM(fw.shape, BF16), pltpu.VMEM(iv.shape, BF16),
            pltpu.VMEM((3, D, D), BF16), pltpu.VMEM((4, D, 256), BF16),
            pltpu.VMEM((3 * NG, D // 2, 128), U32), pltpu.VMEM((NG, D // 2, 128), U32),
            pltpu.VMEM((2, 8 * 72, 128), U32),
            col, col, col, pltpu.VMEM((2, 128, S), BF16), pltpu.VMEM((2, TM, D), BF16),
            pltpu.VMEM((8 + S, 128), F32), pltpu.VMEM((GPI, 8 * PITCH, 128), U32), xsp, xsp,
            pltpu.VMEM((2, CH, 128), F32), pltpu.VMEM((NG, 128), F32),
            sp3, sp3, sp3, sp3, sp2, sp2, qsp, qsp, ksp, ksp, ksp, ksp, osp, osp,
            col, pltpu.VMEM((2, TM, D), BF16),
            pltpu.SemaphoreType.DMA((16,)), pltpu.SemaphoreType.DMA((26,)),
            pltpu.SemaphoreType.DMA((4 + 2 * NI,)),
        ],
        compiler_params=pltpu.CompilerParams(vmem_limit_bytes=100 * 2 ** 20),
    )(A_q.reshape(S, D), A_k.reshape(S, D), A_v.reshape(S, D), A_shift_k.T, A_ssm_k,
      A_ssm_D.reshape(NG, 128), B_x.reshape(S, D), B_wqkv, B_wo, fw, iv)
    return out.reshape(1, S, 2 * D)
```

```python
import itertools

import numpy as np
import jax
import jax.numpy as jnp
from jax import lax
import jax.experimental.pallas as pl
import jax.experimental.pallas.tpu as pltpu

S = 2048
D = 1024
NG = D // 128
CH = 128
NCH = S // CH
TM = S // NG
HIST = 112
PITCH = 24
WIN, DIL, DH = 8, 2, 32
RT = 16
NI = 4
PER = NCH // NI
CB = 4
UNR = 2
LA = 3
SUB = 2
EXT = (1, 4, 6, 8, 9, 10, 11, 12, 13, 10, 11, 12, 13, 14, 14)
EARLY = 1
LB1 = 1
FW1 = 1
GPI = NG // NI
F32, BF16, U32 = jnp.float32, jnp.bfloat16, jnp.uint32


def _dft_mats():
    r = np.arange(CH)
    k = (16 * (r // 16) + 2 * (r % 8) + (r // 8) % 2).astype(np.float64)
    th = 2.0 * np.pi * (k + 0.5) / (2 * CH)
    ang = th[:, None] * np.arange(CH, dtype=np.float64)[None, :]
    fwd = np.concatenate([np.cos(ang), -np.sin(ang)], axis=0)
    inv = fwd.T / CH
    fwd = fwd.reshape(2, CH // 8, 8, CH).transpose(1, 0, 2, 3).reshape(2 * CH, CH)
    return jnp.asarray(fwd, BF16), jnp.asarray(np.stack([inv[:, :CH], inv[:, CH:]]), BF16)


def _permute_cols(w_ref, wp_ref, sec, q):
    lane = lax.broadcasted_iota(jnp.int32, (8, 128), 1)
    bits = [(lane & (2 << st)) != 0 for st in range(3)]

    def first(i):
        r = pl.ds(pl.multiple_of(q * 256 + i * 16, 16), 16)
        v = [pltpu.bitcast(w_ref[sec, r, g * 128:(g + 1) * 128], U32) for g in range(NG)]
        return [v[0]] + [pltpu.roll(v[g], 2 * g, 1) for g in range(1, NG)]

    def second(i, v):
        t = [v[(-e) % NG] for e in range(NG)]
        for st in range(3):
            t = [jnp.where(bits[st], t[(e - (1 << st)) % NG], t[e]) for e in range(NG)]
        t = [t[0]] + [pltpu.roll(t[e], 128 - 2 * e, 1) for e in range(1, NG)]
        for e in range(NG):
            wp_ref[sec * NG + e, pl.ds(pl.multiple_of(q * 128 + i * 8, 8), 8), :] = t[e]

    ahead = 2
    vs = [first(i) for i in range(ahead)]
    for i in range(16):
        if i + ahead < 16:
            vs.append(first(i + ahead))
        second(i, vs[i])


def _permute_rows(wo_ref, tmp_ref, wp_ref, q, hook):
    def anchor(t):
        hook(((t[0] | t[1]) | (t[2] | t[3])) | ((t[4] | t[5]) | (t[6] | t[7])))

    for e in range(2):
        for b in range(8):
            w = pltpu.bitcast(wo_ref[q, b * 128:(b + 1) * 128, e * 128:(e + 1) * 128], U32)
            anchor([w[m * 8:m * 8 + 8] for m in range(8)])
            tmp_ref[e, b * 72:b * 72 + 64, :] = w
            yield
        for a in range(8):
            t = [tmp_ref[e, pl.ds(m * 8 + a, 8, stride=72), :] for m in range(8)]
            anchor(t)
            wp_ref[2 * q + e, a * 64:(a + 1) * 64, :] = jnp.concatenate(t, axis=0)
            yield


def _cat(parts, axis):
    return parts[0] if len(parts) == 1 else jnp.concatenate(parts, axis=axis)


def _bf(parts):
    return jnp.concatenate([pltpu.bitcast(x, BF16) for x in parts], axis=1)


def _kernel(q_hbm, k_hbm, v_hbm, sk_hbm, h_hbm, dd_hbm, x_hbm, w_hbm, wo_hbm, fw_hbm, iv_hbm,
            o_hbm,
            sk_ref, dd_ref, fw_ref, iv_ref,
            w_r, wo_r, w_p, wo_p, wo_tmp, qb, kb, vb, hb, xb, kf, xn, xs0, xs1, hprev, ddf,
            us0, us1, hs0, hs1, ys0, ys1, qs0, qs1, ks0, ks1, vs0, vs1, ob0, ob1,
            oa_buf, obuf, wsem, isem, osem):
    us, hs, ys, xs = (us0, us1), (hs0, hs1), (ys0, ys1), (xs0, xs1)
    qs, ks, vs, ob = (qs0, qs1), (ks0, ks1), (vs0, vs1), (ob0, ob1)
    cur = {}

    chain = []

    def link(x):
        if len(chain) < cur['lb'] or not cur['link']:
            return x
        return jnp.where(cur['never'], chain.pop(0), x)

    def mark(x, must=False):
        if must or len(chain) < cur['lb']:
            chain.append(x)

    def zero(i):
        return lax.shift_right_logical(cur['u'] + i, 8) if cur['link'] else 0

    def gate(r):
        t = r[r.shape[0] - 8:, r.shape[1] - 128:]
        chain[:] = [jnp.where(cur['lane'] > cur['u'] + 1001, t, y) for y in chain]

    def out_copies(step, par, u=None):
        t = step - 2
        n, k = (1, 2 * par) if u is None else (NI, 4 + 2 * u)
        ra = pl.ds(0 if u is None else pl.multiple_of(u * (S // n), S // n), S // n)
        cb = 0 if u is None else pl.multiple_of(u * (D // n), D // n)
        return [pltpu.make_async_copy(oa_buf.at[par, ra], o_hbm.at[ra, pl.ds(pl.multiple_of(t * 128, 128), 128)],
                                      osem.at[k]),
                pltpu.make_async_copy(obuf.at[par, :, pl.ds(cb, D // n)],
                                      o_hbm.at[pl.ds(pl.multiple_of(t * TM, TM), TM), pl.ds(D + cb, D // n)],
                                      osem.at[k + 1])]

    def w_copy(n):
        sec, m = 2 - n // 4, 256 // SUB
        rows = [pl.ds(pl.multiple_of((n % 4) * 256 + j * m, m), m) for j in range(SUB)]
        return [pltpu.make_async_copy(w_hbm.at[r, pl.ds(pl.multiple_of(sec * D, D), D)], w_r.at[sec, r], wsem.at[n])
                for r in rows]

    def wo_copy(n):
        return pltpu.make_async_copy(wo_hbm.at[:, pl.ds(pl.multiple_of(n * 256, 256), 256)], wo_r.at[n],
                                     wsem.at[12 + n])

    def a_in(t, par):
        c = pl.ds(pl.multiple_of(t * 128, 128), 128)
        return [pltpu.make_async_copy(k_hbm.at[:, c], kb.at[par], isem.at[par * 5]),
                pltpu.make_async_copy(v_hbm.at[:, c], vb.at[par], isem.at[par * 5 + 1]),
                pltpu.make_async_copy(h_hbm.at[c, :], hb.at[par], isem.at[par * 5 + 2])]

    def early_in(t, u):
        c, sem = pl.ds(t * 128, 128), isem.at[18 + NI * t + u]
        r, xc = pl.ds(pl.multiple_of(u * (S // NI), 128), S // NI), pl.ds(pl.multiple_of(u * 256, 256), 256)
        return [pltpu.make_async_copy(k_hbm.at[r, c], kb.at[t, r], sem),
                pltpu.make_async_copy(v_hbm.at[r, c], vb.at[t, r], sem),
                pltpu.make_async_copy(h_hbm.at[c, r], hb.at[t, :, r], sem),
                pltpu.make_async_copy(x_hbm.at[pl.ds((t + 1) * TM, TM), xc], xb.at[1 - t, :, xc], sem)]

    def q_in(t, par):
        return [pltpu.make_async_copy(q_hbm.at[:, pl.ds(pl.multiple_of(t * 128, 128), 128)], qb.at[par],
                                      isem.at[par * 5 + 3])]

    def x_in(t, par):
        return [pltpu.make_async_copy(x_hbm.at[pl.ds(pl.multiple_of(t * TM, TM), TM), :], xb.at[par],
                                      isem.at[par * 5 + 4])]

    def start(cps):
        for cp in cps:
            cp.start()

    def wait(cps):
        for cp in cps:
            cp.wait()

    def pin(x):
        x = link(pltpu.bitcast(x, F32))
        mark(x, True)
        return pltpu.bitcast(x, U32)

    def hook(x):
        chain[-1] = pltpu.bitcast(pltpu.bitcast(chain[-1], U32) | x, F32)

    def x_prep(par, u):
        for e in range(GPI):
            g = u * GPI + e
            for b in range(8):
                xv = pltpu.bitcast(xb[par, b * 32:(b + 1) * 32, pl.ds(pl.multiple_of(g * 128, 128), 128)], U32)
                xn[e, b * PITCH:b * PITCH + 8, :] = pin(xv[:8])
                xn[e, b * PITCH + 8:b * PITCH + 16, :] = xv[8:]
                yield
        for e in range(GPI):
            for n in range(16):
                xs[par][u * GPI + e, n * 8:(n + 1) * 8, :] = pin(xn[e, pl.ds(n, 8, stride=PITCH), :])
                yield

    def a_fwd(par, t, u):
        ch = pl.ds(pl.multiple_of(t * 128, 128), 128)
        skt = sk_ref[:, ch].astype(F32)
        skt = [jnp.broadcast_to(skt[j:j + 1, :], (8, 128)) for j in range(4)]
        kvs, hch = [], []
        for cc in range(PER):
            r = pl.multiple_of((u * PER + cc) * CH, CH)
            kf[pl.ds(8 + r, CH), :] = kb[par, pl.ds(r, CH), :].astype(F32)
            vv = vb[par, pl.ds(r, CH), :].astype(F32)
            kv = []
            for f in range(0, CH, 8):
                k0 = kf[pl.ds(8 + r + f, 8), :]
                if f % 16 == 0:
                    tk = link(skt[0])
                pr = [k0 * tk] + [kf[pl.ds(8 + r + f - j, 8), :] * skt[j] for j in range(1, 4)]
                kv.append(((pr[0] + pr[1]) + (pr[2] + pr[3])) * vv[f:f + 8])
                if f % 16 == 8:
                    mark(kv[-1 - (f // 16) % 2])
            kvs.append(_cat(kv, 0))
            hch.append(hb[par, :, pl.ds(r, CH)])
        fw = fw_ref[...]
        hh = lax.dot_general(fw, _cat(hch, 0), (((1,), (1,)), ((), ())), preferred_element_type=F32)
        uu = jnp.dot(fw, _cat(kvs, 1).astype(BF16), preferred_element_type=F32)
        dvec = ddf[pl.ds(t, 1), :]
        dsel = jnp.where(u == 0, dvec, 0.0)
        for f in range(CH // 8):
            t, re, im = slice(8 * f, 8 * f + 8), slice(16 * f, 16 * f + 8), slice(16 * f + 8, 16 * f + 16)
            pc, pd = jnp.where(u == 0, 0.0, hprev[0, t, :]), jnp.where(u == 0, 0.0, hprev[1, t, :])
            for cc in range(PER):
                c, l = u * PER + cc, slice(cc * 128, (cc + 1) * 128)
                hc, hd = hh[re, l], hh[im, l]
                gc = (hc - pd) if f % 2 == 0 else (hc + pd)
                gd = (hd + pc) if f % 2 == 0 else (hd - pc)
                if cc == 0:
                    gc = gc + dsel
                hs[par][c, 0, t, :] = gc
                hs[par][c, 1, t, :] = gd - gc
                hs[par][c, 2, t, :] = gd + gc
                pc, pd = hc, hd
                us[par][c, 0, t, :] = uu[re, l] + uu[im, l]
                us[par][c, 1, t, :] = uu[re, l]
                us[par][c, 2, t, :] = uu[im, l]
            hprev[0, t, :] = pc
            hprev[1, t, :] = pd
        return uu

    def a_conv(par, u, ff, m):
        t0 = pl.ds(pl.multiple_of((u * PER + ff) * 8, 8), 8)
        for blk in range(NCH // CB):
            i0 = blk * CB
            t = pl.ds(pl.multiple_of((u * PER + ff + zero(blk)) * 8, 8), 8)
            acc = [None] * CB if m == 0 else [ys[par][i0 + j, 0, t0, :] for j in range(CB)]
            win = {}
            for c in range(i0 + CB):
                a = link(us[par][c, m, t, :])
                for j in range(CB):
                    d = i0 + j - c
                    if d < 0:
                        continue
                    if d not in win:
                        win[d] = hs[par][d, m, t, :]
                    pr = a * win[d]
                    acc[j] = pr if acc[j] is None else (acc[j] - pr if m == 2 else acc[j] + pr)
                mark(acc[c % CB], c >= i0)
            for j in range(CB):
                ys[par][i0 + j, m % 2, t0, :] = acc[j]
            next(cur['side'], None)

    def a_inv(par, u):
        yy = _cat([_cat([ys[par][u * PER + cc, 0], ys[par][u * PER + cc, 1]], 0) for cc in range(PER)], 1).astype(BF16)
        y = jnp.dot(_cat([iv_ref[0], iv_ref[1]], 1), yy, preferred_element_type=F32)
        for cc in range(PER):
            r = pl.multiple_of((u * PER + cc) * CH, CH)
            oa_buf[par, pl.ds(r, CH), :] = (
                y[:, cc * 128:(cc + 1) * 128] * qb[par, pl.ds(r, CH), :].astype(F32)).astype(BF16)

    def history(dst, par, g, first):
        top = lax.broadcasted_iota(jnp.int32, (8, 128), 0) < 2
        for j in range(HIST // RT):
            o = TM + RT * j
            prev = 0.0 if first else dst[1 - par][g, o + 14:o + 22, :]
            dst[par][g, RT * j:RT * j + 8, :] = jnp.where(top, prev, dst[par][g, o - 2:o + 6, :])
            dst[par][g, RT * j + 8:RT * j + 16, :] = dst[par][g, o + 6:o + 14, :]

    def b_qkv(par, sec, g):
        x = _bf([xs[par][c] for c in range(NG)])
        r = jnp.dot(x, _bf([w_p[sec * NG + g], w_p[sec * NG + g + 1]]), preferred_element_type=F32)
        for e in range(2):
            rr = r[:, e * 128:(e + 1) * 128]
            if sec == 0:
                qs[par][g + e, 0:TM, :] = rr
            else:
                (ks, vs)[sec - 1][par][g + e, HIST:HIST + TM, :] = rr
                history((ks, vs)[sec - 1], par, g + e, False)

    def b_qkv0(sec, u):
        x = _bf([xs0[GPI * u + e] for e in range(GPI)])
        k = pl.ds(pl.multiple_of(u * 128, 128), 128)
        dst, o = (qs0, ks0, vs0)[sec], HIST if sec else 0
        for g in range(0, NG, 2):
            r = jnp.dot(x, _bf([w_p[sec * NG + g + e, k, :] for e in range(2)]), preferred_element_type=F32)
            for e in range(2):
                dst[g + e, o:o + TM, :] = jnp.where(u == 0, 0.0, dst[g + e, o:o + TM, :]) + r[:, e * 128:(e + 1) * 128]

    def b_qk(par, u, tt, first):
        lane = lax.broadcasted_iota(jnp.int32, (RT, 128), 1)
        b4, b0 = (lane & 16) != 0, (lane & 1) != 0
        cexp = float(DH ** -0.5 * np.log2(np.e))
        r0 = pl.multiple_of((u * PER + tt) * RT, RT)
        acc = [[None] * WIN for _ in range(2)]
        for wg in range(0, WIN, CB):
            for hf in range(2):
                rq = pl.ds(pl.multiple_of(r0 + 8 * hf + 8 * zero(wg), 8), 8)
                for g in range(NG):
                    q = link(qs[par][g, rq, :])
                    for w in range(wg, wg + CB):
                        pr = q * ks[par][g, pl.ds(HIST + r0 - RT * w + 8 * hf, 8), :]
                        acc[hf][w] = pr if g == 0 else acc[hf][w] + pr
                    if g < NG - 1:
                        mark(acc[hf][wg + g % CB])
                for w in range(wg, wg + CB):
                    mark(acc[hf][w], True)
        lg = [jnp.concatenate([acc[0][w], acc[1][w]], axis=0) for w in range(WIN)]
        lg = [l + jnp.where(b4, pltpu.roll(l, 16, 1), pltpu.roll(l, 112, 1)) for l in lg]
        lg = [l + jnp.where(b0, pltpu.roll(l, 1, 1), pltpu.roll(l, 127, 1)) for l in lg]
        if first:
            pair = (lax.broadcasted_iota(jnp.int32, (RT, 128), 0) // DIL) * RT + (u * PER + tt)
            lg = [jnp.where(pair >= w, lg[w], -1e9 * DH ** 0.5) for w in range(WIN)]
        m = lg[0]
        for w in range(1, WIN):
            m = jnp.maximum(m, lg[w])
        p = [jnp.exp2((l - m) * cexp) for l in lg]
        den = p[0]
        for w in range(1, WIN):
            den = den + p[w]
        inv = pl.reciprocal(den, approx=True)
        inv = inv * (2.0 - den * inv)
        return [e * inv for e in p]

    def b_pv(par, u, tt, p):
        r0 = pl.multiple_of((u * PER + tt) * RT, RT)
        for gg in range(0, NG, CB):
            acc = [[None] * CB for _ in range(2)]
            for hf in range(2):
                for w in range(WIN):
                    pw = link(p[w][8 * hf:8 * hf + 8])
                    for j in range(CB):
                        pr = pw * vs[par][gg + j, pl.ds(HIST + r0 - RT * w + 8 * hf, 8), :]
                        acc[hf][j] = pr if w == 0 else acc[hf][j] + pr
                    if w < WIN - 1:
                        mark(acc[hf][w % CB])
                for j in range(CB):
                    mark(acc[hf][j], True)
            for j in range(CB):
                o = jnp.concatenate([acc[0][j], acc[1][j]], axis=0).astype(BF16)
                ob[par][gg + j, pl.ds(u * PER + tt, 8, stride=PITCH), :] = pltpu.bitcast(o, U32)

    def b_out(par, g):
        o = _bf([_cat([ob[par][c, b * PITCH:b * PITCH + 16, :] for b in range(8)], 0) for c in range(NG)])
        r = jnp.dot(o, _bf([wo_p[g], wo_p[g + 1]]), preferred_element_type=F32)
        obuf[par, :, pl.ds(pl.multiple_of(g * 128, 256), 256)] = r.astype(BF16)

    def loop(fn, lb=1, unr=1):
        def body(u, carry):
            chain[:] = []
            lane = lax.broadcasted_iota(jnp.int32, (8, 128), 1)
            cur.update(lb=max(lb, 1), u=u, link=lb > 0, lane=lane, never=lane > u + 1000)
            for j in range(unr):
                fn(u * unr + j)
            return carry
        lax.fori_loop(0, NI // unr, body, 0)

    def step(s, par, s1, s2, s3, first2=False):
        def body(u):
            cur['side'] = x_prep(1 - par, u) if s1 else iter(())
            if first2:
                wait([wo_copy(u)] + early_in(1, u))
                issue(3, u)
                cur['side'] = itertools.zip_longest(cur['side'], _permute_rows(wo_r, wo_tmp, wo_p, u, hook))
            mm = []
            if s1:
                mm += [lambda sec=sec: b_qkv(par, sec, u * GPI) for sec in range(3)]
            if s3:
                mm += [lambda: b_out(par, u * GPI)]
                a_inv(par, u)
            for i in range(PER):
                if i < len(mm):
                    mm[i]()
                if s2:
                    p = b_qk(1 - par, u, i, first2)
                    for m in range(3):
                        a_conv(1 - par, u, i, m)
                    b_pv(1 - par, u, i, p)
                if first2 and i == FW1:
                    a_fwd(par, s, u)
            if s1 and not first2:
                gate(a_fwd(par, s, u))
            if not s2:
                start(out_copies(s, par, u))

        loop(body, LB1 if first2 else 1 if s1 else 3, UNR if (s1 and s3) else 1)
        if s2 and s3:
            start(out_copies(s, par))

    def x0_in(n):
        c = pl.ds(pl.multiple_of(n * 256, 256), 256)
        return [pltpu.make_async_copy(x_hbm.at[0:TM, c], xb.at[0, :, c], isem.at[14 + n])]

    start(w_copy(0) + x0_in(0))
    kf[0:8, :] = jnp.zeros((8, 128), F32)
    if not EARLY:
        wait(x0_in(0))
    for n in range(1, LA):
        start(w_copy(n) + x0_in(n))
    if EARLY:
        wait(x0_in(0))
    small = [pltpu.make_async_copy(a, b, isem.at[10 + i]) for i, (a, b) in enumerate(
        [(sk_hbm, sk_ref), (dd_hbm, dd_ref), (fw_hbm, fw_ref), (iv_hbm, iv_ref)])]
    extra = {n - LA: x0_in(n) for n in range(LA + 1, NI)}
    later = ([small] + [early_in(t, u) for t in range(2) for u in range(NI)] + [[wo_copy(n)] for n in range(4)]
             + [a_in(2, 0), x_in(3, 1) + q_in(0, 0)])
    for n, cps in zip(EXT, later):
        extra[n] = extra.get(n, []) + cps

    def issue(ph, u):
        for j in range(NI):
            if ph * 4 + j + 1 in extra:
                pl.when(u == j)(lambda j=j: start(extra[ph * 4 + j + 1]))

    def head(ph, u):
        n = ph * 4 + u + 1
        if ph == 0:
            pl.when(n < NI)(lambda: wait(x0_in(jnp.minimum(n, NI - 1))))
        if ph < 2:
            wait(w_copy(n))
        else:
            pl.when(n < 12)(lambda: wait(w_copy(jnp.minimum(n, 11))))
            wait(early_in(0, u))
        if ph * 4 + 1 + LA < 12:
            pl.when(n + LA < 12)(lambda: start(w_copy(jnp.minimum(n + LA, 11))))
        issue(ph, u)
        b_qkv0(2 - ph, u)
        n = jnp.minimum(n, 11)
        _permute_cols(w_r, w_p, 2 - n // 4, n % 4)
        if ph > 0:
            for e in range(GPI):
                history((vs, ks)[ph - 1], 0, GPI * u + e, True)
        if ph == 2:
            a_fwd(0, 0, u)
        if ph != 1:
            list(x_prep(ph // 2, u if ph else jnp.minimum(u + 1, NI - 1)))

    cur.update(lb=1, link=False)
    list(x_prep(0, 0))
    wait(w_copy(0))
    start(w_copy(LA) + x0_in(LA))
    _permute_cols(w_r, w_p, 2, 0)
    for ph in range(3):
        if ph == 2:
            wait(small)
            ddf[...] = dd_ref[...].astype(F32)
        loop(lambda u, ph=ph: head(ph, u), 0)

    step(1, 1, True, True, False, first2=True)

    def steady(j, carry):
        for par in range(2):
            s = 2 * j + par
            wait(a_in(s, par) + q_in(s - 2, par))
            start(q_in(s - 1, 1 - par))

            if par == 0:
                wait(x_in(s + 1, 1))
                start(a_in(s + 1, 1))

            @pl.when(j < NG // 2 - 1)
            def _():
                if par == 1:
                    wait(x_in(s + 1, 0))
                    start(a_in(s + 1, 0))
                start(x_in(s + 2, par))

            @pl.when(j > 1)
            def _():
                wait(out_copies(s - 2, par))
            step(s, par, True, True, True)
        return carry

    lax.fori_loop(1, NG // 2, steady, 0)
    wait(q_in(NG - 2, 0) + out_copies(NG - 2, 0))
    start(q_in(NG - 1, 1))
    step(NG, 0, False, True, True)
    wait(q_in(NG - 1, 1) + out_copies(NG - 1, 1))
    step(NG + 1, 1, False, False, True)
    wait(out_copies(NG, 0) + sum([out_copies(NG + 1, 1, u) for u in range(NI)], []))


@jax.jit
def pallas_concat_heads__ssm_conv_h3__sliding_local_dilated__prompt_kernel(
    A_q, A_k, A_v, A_shift_k, A_ssm_k, A_ssm_D, B_x, B_wqkv, B_wo,
):
    fw, iv = _dft_mats()
    sp3, sp2 = pltpu.VMEM((NCH, 3, CH + 8, 128), F32), pltpu.VMEM((NCH, 2, CH, 128), F32)
    qsp, ksp = pltpu.VMEM((NG, TM + 8, 128), F32), pltpu.VMEM((NG, HIST + TM + 8, 128), F32)
    xsp, osp = pltpu.VMEM((NG, TM // 2, 128), U32), pltpu.VMEM((NG, 8 * PITCH, 128), U32)
    col = pltpu.VMEM((2, S, 128), BF16)
    hbm = pl.BlockSpec(memory_space=pl.ANY)
    out = pl.pallas_call(
        _kernel,
        in_specs=[hbm] * 11,
        out_specs=hbm,
        out_shape=jax.ShapeDtypeStruct((S, 2 * D), BF16),
        scratch_shapes=[
            pltpu.VMEM((4, D), BF16), pltpu.VMEM((NG, 128), BF16), pltpu.VMEM(fw.shape, BF16), pltpu.VMEM(iv.shape, BF16),
            pltpu.VMEM((3, D, D), BF16), pltpu.VMEM((4, D, 256), BF16),
            pltpu.VMEM((3 * NG, D // 2, 128), U32), pltpu.VMEM((NG, D // 2, 128), U32),
            pltpu.VMEM((2, 8 * 72, 128), U32),
            col, col, col, pltpu.VMEM((2, 128, S), BF16), pltpu.VMEM((2, TM, D), BF16),
            pltpu.VMEM((8 + S, 128), F32), pltpu.VMEM((GPI, 8 * PITCH, 128), U32), xsp, xsp,
            pltpu.VMEM((2, CH, 128), F32), pltpu.VMEM((NG, 128), F32),
            sp3, sp3, sp3, sp3, sp2, sp2, qsp, qsp, ksp, ksp, ksp, ksp, osp, osp,
            col, pltpu.VMEM((2, TM, D), BF16),
            pltpu.SemaphoreType.DMA((16,)), pltpu.SemaphoreType.DMA((26,)),
            pltpu.SemaphoreType.DMA((4 + 2 * NI,)),
        ],
        compiler_params=pltpu.CompilerParams(vmem_limit_bytes=100 * 2 ** 20),
    )(A_q.reshape(S, D), A_k.reshape(S, D), A_v.reshape(S, D), A_shift_k.T, A_ssm_k,
      A_ssm_D.reshape(NG, 128), B_x.reshape(S, D), B_wqkv, B_wo, fw, iv)
    return out.reshape(1, S, 2 * D)
```

```python
import itertools

import numpy as np
import jax
import jax.numpy as jnp
from jax import lax
import jax.experimental.pallas as pl
import jax.experimental.pallas.tpu as pltpu

S = 2048
D = 1024
NG = D // 128
CH = 128
NCH = S // CH
TM = S // NG
HIST = 112
PITCH = 24
WIN, DIL, DH = 8, 2, 32
RT = 16
NI = 4
PER = NCH // NI
CB = 4
UNR = 2
LA = 3
SUB = 2
EXT = (1, 4, 6, 8, 9, 10, 11, 12, 13, 10, 11, 12, 13, 14, 14)
EARLY = 1
L8 = 2
FW1 = 2
FW2 = 4
SLOW = 4
GPI = NG // NI
F32, BF16, U32 = jnp.float32, jnp.bfloat16, jnp.uint32


def _dft_mats():
    r = np.arange(CH)
    k = (16 * (r // 16) + 2 * (r % 8) + (r // 8) % 2).astype(np.float64)
    th = 2.0 * np.pi * (k + 0.5) / (2 * CH)
    ang = th[:, None] * np.arange(CH, dtype=np.float64)[None, :]
    fwd = np.concatenate([np.cos(ang), -np.sin(ang)], axis=0)
    inv = fwd.T / CH
    fwd = fwd.reshape(2, CH // 8, 8, CH).transpose(1, 0, 2, 3).reshape(2 * CH, CH)
    return jnp.asarray(fwd, BF16), jnp.asarray(np.stack([inv[:, :CH], inv[:, CH:]]), BF16)


def _permute_cols(w_ref, wp_ref, sec, q):
    lane = lax.broadcasted_iota(jnp.int32, (8, 128), 1)
    bits = [(lane & (2 << st)) != 0 for st in range(3)]

    def first(i):
        r = pl.ds(pl.multiple_of(q * 256 + i * 16, 16), 16)
        v = [pltpu.bitcast(w_ref[sec, r, g * 128:(g + 1) * 128], U32) for g in range(NG)]
        return [v[0]] + [pltpu.roll(v[g], 2 * g, 1) for g in range(1, NG)]

    def second(i, v):
        t = [v[(-e) % NG] for e in range(NG)]
        for st in range(3):
            t = [jnp.where(bits[st], t[(e - (1 << st)) % NG], t[e]) for e in range(NG)]
        t = [t[0]] + [pltpu.roll(t[e], 128 - 2 * e, 1) for e in range(1, NG)]
        for e in range(NG):
            wp_ref[sec * NG + e, pl.ds(pl.multiple_of(q * 128 + i * 8, 8), 8), :] = t[e]

    ahead = 2
    vs = [first(i) for i in range(ahead)]
    for i in range(16):
        if i + ahead < 16:
            vs.append(first(i + ahead))
        second(i, vs[i])


def _permute_rows(wo_ref, tmp_ref, wp_ref, q, hook):
    def anchor(t):
        hook(((t[0] | t[1]) | (t[2] | t[3])) | ((t[4] | t[5]) | (t[6] | t[7])))

    for e in range(2):
        for b in range(8):
            w = pltpu.bitcast(wo_ref[q, b * 128:(b + 1) * 128, e * 128:(e + 1) * 128], U32)
            anchor([w[m * 8:m * 8 + 8] for m in range(8)])
            tmp_ref[e, b * 72:b * 72 + 64, :] = w
            yield
        for a in range(8):
            t = [tmp_ref[e, pl.ds(m * 8 + a, 8, stride=72), :] for m in range(8)]
            anchor(t)
            wp_ref[2 * q + e, a * 64:(a + 1) * 64, :] = jnp.concatenate(t, axis=0)
            yield


def _cat(parts, axis):
    return parts[0] if len(parts) == 1 else jnp.concatenate(parts, axis=axis)


def _bf(parts):
    return jnp.concatenate([pltpu.bitcast(x, BF16) for x in parts], axis=1)


def _kernel(q_hbm, k_hbm, v_hbm, sk_hbm, h_hbm, dd_hbm, x_hbm, w_hbm, wo_hbm, fw_hbm, iv_hbm,
            o_hbm,
            sk_ref, dd_ref, fw_ref, iv_ref,
            w_r, wo_r, w_p, wo_p, wo_tmp, qb, kb, vb, hb, xb, kf, xn, xs0, xs1, hprev, ddf,
            us0, us1, hs0, hs1, ys0, ys1, qs0, qs1, ks0, ks1, vs0, vs1, ob0, ob1, ob2,
            oa_buf, obuf, wsem, isem, osem):
    us, hs, ys, xs = (us0, us1), (hs0, hs1), (ys0, ys1), (xs0, xs1)
    qs, ks, vs, ob = (qs0, qs1), (ks0, ks1), (vs0, vs1), (ob0, ob1)
    cur = {}

    chain = []

    def link(x):
        if len(chain) < cur['lb'] or not cur['link']:
            return x
        y = jnp.where(cur['never'], chain.pop(0), x)
        cur['n'] += cur['slow']
        for k in range(cur['n'] // 8):
            y = jnp.where(cur['lane'] > cur['u'] + 1002 + k, x, y)
        cur['n'] %= 8
        return y

    def mark(x, must=False):
        if must or len(chain) < cur['lb']:
            chain.append(x)

    def zero(i):
        return lax.shift_right_logical(cur['u'] + i, 8) if cur['link'] else 0

    def gate(r):
        t = r[r.shape[0] - 8:, r.shape[1] - 128:]
        chain[:] = [jnp.where(cur['lane'] > cur['u'] + 1001, t, y) for y in chain]

    def out_copies(step, par, u=None):
        t = step - 2
        n, k = (1, 2 * par) if u is None else (NI, 4 + 2 * (NI * par + u))
        ra = pl.ds(0 if u is None else pl.multiple_of(u * (S // n), S // n), S // n)
        cb = 0 if u is None else pl.multiple_of(u * (D // n), D // n)
        return [pltpu.make_async_copy(oa_buf.at[par, ra], o_hbm.at[ra, pl.ds(pl.multiple_of(t * 128, 128), 128)],
                                      osem.at[k]),
                pltpu.make_async_copy(obuf.at[par, :, pl.ds(cb, D // n)],
                                      o_hbm.at[pl.ds(pl.multiple_of(t * TM, TM), TM), pl.ds(D + cb, D // n)],
                                      osem.at[k + 1])]

    def w_copy(n):
        sec, m = 2 - n // 4, 256 // SUB
        rows = [pl.ds(pl.multiple_of((n % 4) * 256 + j * m, m), m) for j in range(SUB)]
        return [pltpu.make_async_copy(w_hbm.at[r, pl.ds(pl.multiple_of(sec * D, D), D)], w_r.at[sec, r], wsem.at[n])
                for r in rows]

    def wo_copy(n):
        return pltpu.make_async_copy(wo_hbm.at[:, pl.ds(pl.multiple_of(n * 256, 256), 256)], wo_r.at[n],
                                     wsem.at[12 + n])

    def a_in(t, par):
        c = pl.ds(pl.multiple_of(t * 128, 128), 128)
        return [pltpu.make_async_copy(k_hbm.at[:, c], kb.at[par], isem.at[par * 5]),
                pltpu.make_async_copy(v_hbm.at[:, c], vb.at[par], isem.at[par * 5 + 1]),
                pltpu.make_async_copy(h_hbm.at[c, :], hb.at[par], isem.at[par * 5 + 2])]

    def early_in(t, u):
        c, sem = pl.ds(t * 128, 128), isem.at[18 + NI * t + u]
        r, xc = pl.ds(pl.multiple_of(u * (S // NI), 128), S // NI), pl.ds(pl.multiple_of(u * 256, 256), 256)
        return [pltpu.make_async_copy(k_hbm.at[r, c], kb.at[t, r], sem),
                pltpu.make_async_copy(v_hbm.at[r, c], vb.at[t, r], sem),
                pltpu.make_async_copy(h_hbm.at[c, r], hb.at[t, :, r], sem),
                pltpu.make_async_copy(x_hbm.at[pl.ds((t + 1) * TM, TM), xc], xb.at[1 - t, :, xc], sem)]

    def q_in(t, par):
        return [pltpu.make_async_copy(q_hbm.at[:, pl.ds(pl.multiple_of(t * 128, 128), 128)], qb.at[par],
                                      isem.at[par * 5 + 3])]

    def x_in(t, par):
        return [pltpu.make_async_copy(x_hbm.at[pl.ds(pl.multiple_of(t * TM, TM), TM), :], xb.at[par],
                                      isem.at[par * 5 + 4])]

    def start(cps):
        for cp in cps:
            cp.start()

    def wait(cps):
        for cp in cps:
            cp.wait()

    def pin(x):
        x = link(pltpu.bitcast(x, F32))
        mark(x, True)
        return pltpu.bitcast(x, U32)

    def hook(x):
        chain[-1] = pltpu.bitcast(pltpu.bitcast(chain[-1], U32) | x, F32)

    def x_prep(par, u):
        for e in range(GPI):
            g = u * GPI + e
            for b in range(8):
                xv = pltpu.bitcast(xb[par, b * 32:(b + 1) * 32, pl.ds(pl.multiple_of(g * 128, 128), 128)], U32)
                xn[e, b * PITCH:b * PITCH + 8, :] = pin(xv[:8])
                xn[e, b * PITCH + 8:b * PITCH + 16, :] = xv[8:]
                yield
        for e in range(GPI):
            for n in range(16):
                xs[par][u * GPI + e, n * 8:(n + 1) * 8, :] = pin(xn[e, pl.ds(n, 8, stride=PITCH), :])
                yield

    def a_fwd(par, t, u):
        ch = pl.ds(pl.multiple_of(t * 128, 128), 128)
        skt = sk_ref[:, ch].astype(F32)
        skt = [jnp.broadcast_to(skt[j:j + 1, :], (8, 128)) for j in range(4)]
        kvs, hch = [], []
        for cc in range(PER):
            r = pl.multiple_of((u * PER + cc) * CH, CH)
            kf[pl.ds(8 + r, CH), :] = kb[par, pl.ds(r, CH), :].astype(F32)
            vv = vb[par, pl.ds(r, CH), :].astype(F32)
            kv = []
            for f in range(0, CH, 8):
                k0 = kf[pl.ds(8 + r + f, 8), :]
                if f % 16 == 0:
                    tk = link(skt[0])
                pr = [k0 * tk] + [kf[pl.ds(8 + r + f - j, 8), :] * skt[j] for j in range(1, 4)]
                kv.append(((pr[0] + pr[1]) + (pr[2] + pr[3])) * vv[f:f + 8])
                if f % 16 == 8:
                    mark(kv[-1 - (f // 16) % 2])
            kvs.append(_cat(kv, 0))
            hch.append(hb[par, :, pl.ds(r, CH)])
        fw = fw_ref[...]
        hh = lax.dot_general(fw, _cat(hch, 0), (((1,), (1,)), ((), ())), preferred_element_type=F32)
        uu = jnp.dot(fw, _cat(kvs, 1).astype(BF16), preferred_element_type=F32)
        dvec = ddf[pl.ds(t, 1), :]
        dsel = jnp.where(u == 0, dvec, 0.0)
        for f in range(CH // 8):
            t, re, im = slice(8 * f, 8 * f + 8), slice(16 * f, 16 * f + 8), slice(16 * f + 8, 16 * f + 16)
            pc, pd = jnp.where(u == 0, 0.0, hprev[0, t, :]), jnp.where(u == 0, 0.0, hprev[1, t, :])
            for cc in range(PER):
                c, l = u * PER + cc, slice(cc * 128, (cc + 1) * 128)
                hc, hd = hh[re, l], hh[im, l]
                gc = (hc - pd) if f % 2 == 0 else (hc + pd)
                gd = (hd + pc) if f % 2 == 0 else (hd - pc)
                if cc == 0:
                    gc = gc + dsel
                hs[par][c, 0, t, :] = gc
                hs[par][c, 1, t, :] = gd - gc
                hs[par][c, 2, t, :] = gd + gc
                pc, pd = hc, hd
                us[par][c, 0, t, :] = uu[re, l] + uu[im, l]
                us[par][c, 1, t, :] = uu[re, l]
                us[par][c, 2, t, :] = uu[im, l]
            hprev[0, t, :] = pc
            hprev[1, t, :] = pd
        return uu

    def a_conv(par, u, ff, m):
        t0 = pl.ds(pl.multiple_of((u * PER + ff) * 8, 8), 8)
        for blk in range(NCH // CB):
            i0 = blk * CB
            t = pl.ds(pl.multiple_of((u * PER + ff + zero(blk)) * 8, 8), 8)
            acc = [None] * CB if m == 0 else [ys[par][i0 + j, 0, t0, :] for j in range(CB)]
            win = {}
            for c in range(i0 + CB):
                a = link(us[par][c, m, t, :])
                for j in range(CB):
                    d = i0 + j - c
                    if d < 0:
                        continue
                    if d not in win:
                        win[d] = hs[par][d, m, t, :]
                    pr = a * win[d]
                    acc[j] = pr if acc[j] is None else (acc[j] - pr if m == 2 else acc[j] + pr)
                mark(acc[c % CB], c >= i0)
            for j in range(CB):
                ys[par][i0 + j, m % 2, t0, :] = acc[j]
            next(cur['side'], None)

    def a_inv(par, u):
        yy = _cat([_cat([ys[par][u * PER + cc, 0], ys[par][u * PER + cc, 1]], 0) for cc in range(PER)], 1).astype(BF16)
        y = jnp.dot(_cat([iv_ref[0], iv_ref[1]], 1), yy, preferred_element_type=F32)
        for cc in range(PER):
            r = pl.multiple_of((u * PER + cc) * CH, CH)
            oa_buf[par, pl.ds(r, CH), :] = (
                y[:, cc * 128:(cc + 1) * 128] * qb[par, pl.ds(r, CH), :].astype(F32)).astype(BF16)

    def history(dst, par, g, first):
        top = lax.broadcasted_iota(jnp.int32, (8, 128), 0) < 2
        for j in range(HIST // RT):
            o = TM + RT * j
            prev = 0.0 if first else dst[1 - par][g, o + 14:o + 22, :]
            dst[par][g, RT * j:RT * j + 8, :] = jnp.where(top, prev, dst[par][g, o - 2:o + 6, :])
            dst[par][g, RT * j + 8:RT * j + 16, :] = dst[par][g, o + 6:o + 14, :]

    def b_qkv(par, sec, g):
        x = _bf([xs[par][c] for c in range(NG)])
        r = jnp.dot(x, _bf([w_p[sec * NG + g], w_p[sec * NG + g + 1]]), preferred_element_type=F32)
        for e in range(2):
            rr = r[:, e * 128:(e + 1) * 128]
            if sec == 0:
                qs[par][g + e, 0:TM, :] = rr
            else:
                (ks, vs)[sec - 1][par][g + e, HIST:HIST + TM, :] = rr
                history((ks, vs)[sec - 1], par, g + e, False)

    def b_qkv0(sec, u):
        x = _bf([xs0[GPI * u + e] for e in range(GPI)])
        k = pl.ds(pl.multiple_of(u * 128, 128), 128)
        dst, o = (qs0, ks0, vs0)[sec], HIST if sec else 0
        for g in range(0, NG, 2):
            r = jnp.dot(x, _bf([w_p[sec * NG + g + e, k, :] for e in range(2)]), preferred_element_type=F32)
            for e in range(2):
                dst[g + e, o:o + TM, :] = jnp.where(u == 0, 0.0, dst[g + e, o:o + TM, :]) + r[:, e * 128:(e + 1) * 128]

    def b_qk(par, u, tt, first):
        lane = lax.broadcasted_iota(jnp.int32, (RT, 128), 1)
        b4, b0 = (lane & 16) != 0, (lane & 1) != 0
        cexp = float(DH ** -0.5 * np.log2(np.e))
        r0 = pl.multiple_of((u * PER + tt) * RT, RT)
        acc = [[None] * WIN for _ in range(2)]
        for wg in range(0, WIN, CB):
            for hf in range(2):
                rq = pl.ds(pl.multiple_of(r0 + 8 * hf + 8 * zero(wg), 8), 8)
                for g in range(NG):
                    q = link(qs[par][g, rq, :])
                    for w in range(wg, wg + CB):
                        pr = q * ks[par][g, pl.ds(HIST + r0 - RT * w + 8 * hf, 8), :]
                        acc[hf][w] = pr if g == 0 else acc[hf][w] + pr
                    if g < NG - 1:
                        mark(acc[hf][wg + g % CB])
                for w in range(wg, wg + CB):
                    mark(acc[hf][w], True)
        lg = [jnp.concatenate([acc[0][w], acc[1][w]], axis=0) for w in range(WIN)]
        lg = [l + jnp.where(b4, pltpu.roll(l, 16, 1), pltpu.roll(l, 112, 1)) for l in lg]
        lg = [l + jnp.where(b0, pltpu.roll(l, 1, 1), pltpu.roll(l, 127, 1)) for l in lg]
        if first:
            pair = (lax.broadcasted_iota(jnp.int32, (RT, 128), 0) // DIL) * RT + (u * PER + tt)
            lg = [jnp.where(pair >= w, lg[w], -1e9 * DH ** 0.5) for w in range(WIN)]
        m = lg[0]
        for w in range(1, WIN):
            m = jnp.maximum(m, lg[w])
        p = [jnp.exp2((l - m) * cexp) for l in lg]
        den = p[0]
        for w in range(1, WIN):
            den = den + p[w]
        inv = pl.reciprocal(den, approx=True)
        inv = inv * (2.0 - den * inv)
        return [e * inv for e in p]

    def b_pv(par, u, tt, p, dst):
        r0 = pl.multiple_of((u * PER + tt) * RT, RT)
        for gg in range(0, NG, CB):
            acc = [[None] * CB for _ in range(2)]
            for hf in range(2):
                for w in range(WIN):
                    pw = link(p[w][8 * hf:8 * hf + 8])
                    for j in range(CB):
                        pr = pw * vs[par][gg + j, pl.ds(HIST + r0 - RT * w + 8 * hf, 8), :]
                        acc[hf][j] = pr if w == 0 else acc[hf][j] + pr
                    if w < WIN - 1:
                        mark(acc[hf][w % CB])
                for j in range(CB):
                    mark(acc[hf][j], True)
            for j in range(CB):
                o = jnp.concatenate([acc[0][j], acc[1][j]], axis=0).astype(BF16)
                dst[gg + j, pl.ds(u * PER + tt, 8, stride=PITCH), :] = pltpu.bitcast(o, U32)

    def b_out(par, g):
        o = _bf([_cat([ob[par][c, b * PITCH:b * PITCH + 16, :] for b in range(8)], 0) for c in range(NG)])
        r = jnp.dot(o, _bf([wo_p[g], wo_p[g + 1]]), preferred_element_type=F32)
        obuf[par, :, pl.ds(pl.multiple_of(g * 128, 256), 256)] = r.astype(BF16)

    def b_half(src, par, k):
        g, h = (k // 2) * 2, k % 2
        o = _bf([_cat([src[c, pl.ds(pl.multiple_of(b * PITCH + 8 * h, 8), 8), :] for b in range(8)], 0)
                 for c in range(NG)])
        r = jnp.dot(o, _bf([wo_p[g], wo_p[g + 1]]), preferred_element_type=F32).astype(BF16)
        for b in range(8):
            obuf[par, pl.ds(pl.multiple_of(b * 32 + 16 * h, 16), 16), pl.ds(pl.multiple_of(g * 128, 256), 256)] = (
                r[b * 16:(b + 1) * 16])

    def loop(fn, lb=1, unr=1, slow=0, lo=0, hi=NI):
        def body(u, carry):
            chain[:] = []
            lane = lax.broadcasted_iota(jnp.int32, (8, 128), 1)
            cur.update(lb=max(lb, 1), u=u, link=lb > 0, lane=lane, never=lane > u + 1000,
                       n=0, slow=slow)
            for j in range(unr):
                fn(u * unr + j)
            return carry
        lax.fori_loop(lo // unr, hi // unr, body, 0)

    def step(s, par, s1, s2, s3, first2=False, tail=0):
        def body(u):
            cur['side'] = x_prep(1 - par, u) if s1 else iter(())
            if first2:
                wait([wo_copy(u)] + early_in(1, u))
                issue(3, u)
                cur['side'] = itertools.zip_longest(cur['side'], _permute_rows(wo_r, wo_tmp, wo_p, u, hook))
            mm = []
            if s1:
                mm += [lambda sec=sec: b_qkv(par, sec, u * GPI) for sec in range(3)]
            if s3:
                units = {0: [], 1: [(ob0, 0, 3 * u + j) for j in range(3)],
                         2: [(ob0, 0, u + 4), (ob1, 1, 4 * u - 8), (ob1, 1, 4 * u - 6)], 3: [(ob2, 1, 2 * u + 1)]}[tail]
                mm += [lambda a=a: b_half(*a) for a in units] if tail else [lambda: b_out(par, u * GPI)]
                a_inv(par, u)
            for i in range(PER):
                if i < len(mm):
                    mm[i]()
                if s2:
                    p = b_qk(1 - par, u, i, first2)
                    for m in range(3):
                        a_conv(1 - par, u, i, m)
                    b_pv(1 - par, u, i, p, ob2 if tail == 2 else ob[1 - par])
                if s1 and i == (FW1 if first2 else FW2):
                    a_fwd(par, s, u)
            if s1 and not first2 and FW2 == 4:
                gate(a_fwd(par, s, u))
            if not s2:
                start(out_copies(s, par, u))

        loop(body, 1 if s1 else L8, UNR if (s1 and s3) else 1,
             SLOW if (s1 and s3) else 0, 2 if tail == 2 else 0, 2 if tail == 1 else NI)
        if s3 and not tail:
            start(out_copies(s, par))

    def x0_in(n):
        c = pl.ds(pl.multiple_of(n * 256, 256), 256)
        return [pltpu.make_async_copy(x_hbm.at[0:TM, c], xb.at[0, :, c], isem.at[14 + n])]

    start(w_copy(0) + x0_in(0))
    kf[0:8, :] = jnp.zeros((8, 128), F32)
    if not EARLY:
        wait(x0_in(0))
    for n in range(1, LA):
        start(w_copy(n) + x0_in(n))
    if EARLY:
        wait(x0_in(0))
    small = [pltpu.make_async_copy(a, b, isem.at[10 + i]) for i, (a, b) in enumerate(
        [(sk_hbm, sk_ref), (dd_hbm, dd_ref), (fw_hbm, fw_ref), (iv_hbm, iv_ref)])]
    extra = {n - LA: x0_in(n) for n in range(LA + 1, NI)}
    later = ([small] + [early_in(t, u) for t in range(2) for u in range(NI)] + [[wo_copy(n)] for n in range(4)]
             + [a_in(2, 0), x_in(3, 1) + q_in(0, 0)])
    for n, cps in zip(EXT, later):
        extra[n] = extra.get(n, []) + cps

    def issue(ph, u):
        for j in range(NI):
            if ph * 4 + j + 1 in extra:
                pl.when(u == j)(lambda j=j: start(extra[ph * 4 + j + 1]))

    def head(ph, u):
        n = ph * 4 + u + 1
        if ph == 0:
            pl.when(n < NI)(lambda: wait(x0_in(jnp.minimum(n, NI - 1))))
        if ph < 2:
            wait(w_copy(n))
        else:
            pl.when(n < 12)(lambda: wait(w_copy(jnp.minimum(n, 11))))
            wait(early_in(0, u))
        if ph * 4 + 1 + LA < 12:
            pl.when(n + LA < 12)(lambda: start(w_copy(jnp.minimum(n + LA, 11))))
        issue(ph, u)
        b_qkv0(2 - ph, u)
        n = jnp.minimum(n, 11)
        _permute_cols(w_r, w_p, 2 - n // 4, n % 4)
        if ph > 0:
            for e in range(GPI):
                history((vs, ks)[ph - 1], 0, GPI * u + e, True)
        if ph == 2:
            a_fwd(0, 0, u)
        if ph != 1:
            list(x_prep(ph // 2, u if ph else jnp.minimum(u + 1, NI - 1)))

    cur.update(lb=1, link=False)
    list(x_prep(0, 0))
    wait(w_copy(0))
    start(w_copy(LA) + x0_in(LA))
    _permute_cols(w_r, w_p, 2, 0)
    for ph in range(3):
        if ph == 2:
            wait(small)
            ddf[...] = dd_ref[...].astype(F32)
        loop(lambda u, ph=ph: head(ph, u), 0)

    step(1, 1, True, True, False, first2=True)

    def steady(j, carry):
        for par in range(2):
            s = 2 * j + par
            wait(a_in(s, par) + q_in(s - 2, par))
            start(q_in(s - 1, 1 - par))

            if par == 0:
                wait(x_in(s + 1, 1))
                start(a_in(s + 1, 1))

            @pl.when(j < NG // 2 - 1)
            def _():
                if par == 1:
                    wait(x_in(s + 1, 0))
                    start(a_in(s + 1, 0))
                start(x_in(s + 2, par))

            @pl.when(j > 1)
            def _():
                wait(out_copies(s - 2, par))
            step(s, par, True, True, True)
        return carry

    lax.fori_loop(1, NG // 2, steady, 0)
    wait(q_in(NG - 2, 0) + out_copies(NG - 2, 0))
    start(q_in(NG - 1, 1))
    last = [out_copies(NG + par, par, u) for par in range(2) for u in range(NI)]
    step(NG, 0, False, True, True, tail=1)
    start(last[0] + last[1] + last[2][1:])
    wait(q_in(NG - 1, 1) + out_copies(NG - 1, 1))
    step(NG, 0, False, True, True, tail=2)
    start(last[2][:1] + last[3])
    step(NG + 1, 1, False, False, True, tail=3)
    wait(sum(last, []))


@jax.jit
def pallas_concat_heads__ssm_conv_h3__sliding_local_dilated__prompt_kernel(
    A_q, A_k, A_v, A_shift_k, A_ssm_k, A_ssm_D, B_x, B_wqkv, B_wo,
):
    fw, iv = _dft_mats()
    sp3, sp2 = pltpu.VMEM((NCH, 3, CH + 8, 128), F32), pltpu.VMEM((NCH, 2, CH, 128), F32)
    qsp, ksp = pltpu.VMEM((NG, TM + 8, 128), F32), pltpu.VMEM((NG, HIST + TM + 8, 128), F32)
    xsp, osp = pltpu.VMEM((NG, TM // 2, 128), U32), pltpu.VMEM((NG, 8 * PITCH, 128), U32)
    col = pltpu.VMEM((2, S, 128), BF16)
    hbm = pl.BlockSpec(memory_space=pl.ANY)
    out = pl.pallas_call(
        _kernel,
        in_specs=[hbm] * 11,
        out_specs=hbm,
        out_shape=jax.ShapeDtypeStruct((S, 2 * D), BF16),
        scratch_shapes=[
            pltpu.VMEM((4, D), BF16), pltpu.VMEM((NG, 128), BF16), pltpu.VMEM(fw.shape, BF16), pltpu.VMEM(iv.shape, BF16),
            pltpu.VMEM((3, D, D), BF16), pltpu.VMEM((4, D, 256), BF16),
            pltpu.VMEM((3 * NG, D // 2, 128), U32), pltpu.VMEM((NG, D // 2, 128), U32),
            pltpu.VMEM((2, 8 * 72, 128), U32),
            col, col, col, pltpu.VMEM((2, 128, S), BF16), pltpu.VMEM((2, TM, D), BF16),
            pltpu.VMEM((8 + S, 128), F32), pltpu.VMEM((GPI, 8 * PITCH, 128), U32), xsp, xsp,
            pltpu.VMEM((2, CH, 128), F32), pltpu.VMEM((NG, 128), F32),
            sp3, sp3, sp3, sp3, sp2, sp2, qsp, qsp, ksp, ksp, ksp, ksp, osp, osp, osp,
            col, pltpu.VMEM((2, TM, D), BF16),
            pltpu.SemaphoreType.DMA((16,)), pltpu.SemaphoreType.DMA((26,)),
            pltpu.SemaphoreType.DMA((4 + 4 * NI,)),
        ],
        compiler_params=pltpu.CompilerParams(vmem_limit_bytes=100 * 2 ** 20),
    )(A_q.reshape(S, D), A_k.reshape(S, D), A_v.reshape(S, D), A_shift_k.T, A_ssm_k,
      A_ssm_D.reshape(NG, 128), B_x.reshape(S, D), B_wqkv, B_wo, fw, iv)
    return out.reshape(1, S, 2 * D)
```

```python
import itertools

import numpy as np
import jax
import jax.numpy as jnp
from jax import lax
import jax.experimental.pallas as pl
import jax.experimental.pallas.tpu as pltpu

S = 2048
D = 1024
NG = D // 128
CH = 128
NCH = S // CH
TM = S // NG
HIST = 112
PITCH = 24
WIN, DIL, DH = 8, 2, 32
RT = 16
NI = 4
PER = NCH // NI
CB = 4
UNR = 2
LA = 3
SUB = 2
EXT = (1, 4, 6, 8, 9, 10, 11, 12, 13, 10, 11, 12, 13, 14, 14)
EARLY = 1
L8 = 2
FW1 = 2
FW2 = 4
SLOW = (2, 2, 2)
GPI = NG // NI
F32, BF16, U32 = jnp.float32, jnp.bfloat16, jnp.uint32


def _dft_mats():
    r = np.arange(CH)
    k = (16 * (r // 16) + 2 * (r % 8) + (r // 8) % 2).astype(np.float64)
    th = 2.0 * np.pi * (k + 0.5) / (2 * CH)
    ang = th[:, None] * np.arange(CH, dtype=np.float64)[None, :]
    fwd = np.concatenate([np.cos(ang), -np.sin(ang)], axis=0)
    inv = fwd.T / CH
    fwd = fwd.reshape(2, CH // 8, 8, CH).transpose(1, 0, 2, 3).reshape(2 * CH, CH)
    return jnp.asarray(fwd, BF16), jnp.asarray(np.stack([inv[:, :CH], inv[:, CH:]]), BF16)


def _permute_cols(w_ref, wp_ref, sec, q):
    lane = lax.broadcasted_iota(jnp.int32, (8, 128), 1)
    bits = [(lane & (2 << st)) != 0 for st in range(3)]

    def first(i):
        r = pl.ds(pl.multiple_of(q * 256 + i * 16, 16), 16)
        v = [pltpu.bitcast(w_ref[sec, r, g * 128:(g + 1) * 128], U32) for g in range(NG)]
        return [v[0]] + [pltpu.roll(v[g], 2 * g, 1) for g in range(1, NG)]

    def second(i, v):
        t = [v[(-e) % NG] for e in range(NG)]
        for st in range(3):
            t = [jnp.where(bits[st], t[(e - (1 << st)) % NG], t[e]) for e in range(NG)]
        t = [t[0]] + [pltpu.roll(t[e], 128 - 2 * e, 1) for e in range(1, NG)]
        for e in range(NG):
            wp_ref[sec * NG + e, pl.ds(pl.multiple_of(q * 128 + i * 8, 8), 8), :] = t[e]

    ahead = 2
    vs = [first(i) for i in range(ahead)]
    for i in range(16):
        if i + ahead < 16:
            vs.append(first(i + ahead))
        second(i, vs[i])


def _permute_rows(wo_ref, tmp_ref, wp_ref, q, hook):
    def anchor(t):
        hook(((t[0] | t[1]) | (t[2] | t[3])) | ((t[4] | t[5]) | (t[6] | t[7])))

    for e in range(2):
        for b in range(8):
            w = pltpu.bitcast(wo_ref[q, b * 128:(b + 1) * 128, e * 128:(e + 1) * 128], U32)
            anchor([w[m * 8:m * 8 + 8] for m in range(8)])
            tmp_ref[e, b * 72:b * 72 + 64, :] = w
            yield
        for a in range(8):
            t = [tmp_ref[e, pl.ds(m * 8 + a, 8, stride=72), :] for m in range(8)]
            anchor(t)
            wp_ref[2 * q + e, a * 64:(a + 1) * 64, :] = jnp.concatenate(t, axis=0)
            yield


def _cat(parts, axis):
    return parts[0] if len(parts) == 1 else jnp.concatenate(parts, axis=axis)


def _bf(parts):
    return jnp.concatenate([pltpu.bitcast(x, BF16) for x in parts], axis=1)


def _kernel(q_hbm, k_hbm, v_hbm, sk_hbm, h_hbm, dd_hbm, x_hbm, w_hbm, wo_hbm, fw_hbm, iv_hbm,
            o_hbm,
            sk_ref, dd_ref, fw_ref, iv_ref,
            w_r, wo_r, w_p, wo_p, wo_tmp, qb, kb, vb, hb, xb, kf, xn, xs0, xs1, hprev, ddf,
            us0, us1, hs0, hs1, ys0, ys1, qs0, qs1, ks0, ks1, vs0, vs1, ob0, ob1, ob2,
            oa_buf, obuf, wsem, isem, osem):
    us, hs, ys, xs = (us0, us1), (hs0, hs1), (ys0, ys1), (xs0, xs1)
    qs, ks, vs, ob = (qs0, qs1), (ks0, ks1), (vs0, vs1), (ob0, ob1)
    cur = {}

    chain = []

    def link(x, kind=0):
        if len(chain) < cur['lb'] or not cur['link']:
            return x
        y = jnp.where(cur['never'], chain.pop(0), x)
        cur['n'] += cur['slow'][kind]
        for k in range(cur['n'] // 8):
            y = jnp.where(cur['lane'] > cur['u'] + 1002 + k, x, y)
        cur['n'] %= 8
        return y

    def mark(x, must=False):
        if must or len(chain) < cur['lb']:
            chain.append(x)

    def zero(i):
        return lax.shift_right_logical(cur['u'] + i, 8) if cur['link'] else 0

    def gate(r):
        t = r[r.shape[0] - 8:, r.shape[1] - 128:]
        chain[:] = [jnp.where(cur['lane'] > cur['u'] + 1001, t, y) for y in chain]

    def out_copies(step, par, u=None):
        t = step - 2
        n, k = (1, 2 * par) if u is None else (NI, 4 + 2 * (NI * par + u))
        ra = pl.ds(0 if u is None else pl.multiple_of(u * (S // n), S // n), S // n)
        cb = 0 if u is None else pl.multiple_of(u * (D // n), D // n)
        return [pltpu.make_async_copy(oa_buf.at[par, ra], o_hbm.at[ra, pl.ds(pl.multiple_of(t * 128, 128), 128)],
                                      osem.at[k]),
                pltpu.make_async_copy(obuf.at[par, :, pl.ds(cb, D // n)],
                                      o_hbm.at[pl.ds(pl.multiple_of(t * TM, TM), TM), pl.ds(D + cb, D // n)],
                                      osem.at[k + 1])]

    def w_copy(n):
        sec, m = 2 - n // 4, 256 // SUB
        rows = [pl.ds(pl.multiple_of((n % 4) * 256 + j * m, m), m) for j in range(SUB)]
        return [pltpu.make_async_copy(w_hbm.at[r, pl.ds(pl.multiple_of(sec * D, D), D)], w_r.at[sec, r], wsem.at[n])
                for r in rows]

    def wo_copy(n):
        return pltpu.make_async_copy(wo_hbm.at[:, pl.ds(pl.multiple_of(n * 256, 256), 256)], wo_r.at[n],
                                     wsem.at[12 + n])

    def a_in(t, par):
        c = pl.ds(pl.multiple_of(t * 128, 128), 128)
        return [pltpu.make_async_copy(k_hbm.at[:, c], kb.at[par], isem.at[par * 5]),
                pltpu.make_async_copy(v_hbm.at[:, c], vb.at[par], isem.at[par * 5 + 1]),
                pltpu.make_async_copy(h_hbm.at[c, :], hb.at[par], isem.at[par * 5 + 2])]

    def early_in(t, u):
        c, sem = pl.ds(t * 128, 128), isem.at[18 + NI * t + u]
        r, xc = pl.ds(pl.multiple_of(u * (S // NI), 128), S // NI), pl.ds(pl.multiple_of(u * 256, 256), 256)
        return [pltpu.make_async_copy(k_hbm.at[r, c], kb.at[t, r], sem),
                pltpu.make_async_copy(v_hbm.at[r, c], vb.at[t, r], sem),
                pltpu.make_async_copy(h_hbm.at[c, r], hb.at[t, :, r], sem),
                pltpu.make_async_copy(x_hbm.at[pl.ds((t + 1) * TM, TM), xc], xb.at[1 - t, :, xc], sem)]

    def q_in(t, par):
        return [pltpu.make_async_copy(q_hbm.at[:, pl.ds(pl.multiple_of(t * 128, 128), 128)], qb.at[par],
                                      isem.at[par * 5 + 3])]

    def x_in(t, par):
        return [pltpu.make_async_copy(x_hbm.at[pl.ds(pl.multiple_of(t * TM, TM), TM), :], xb.at[par],
                                      isem.at[par * 5 + 4])]

    def start(cps):
        for cp in cps:
            cp.start()

    def wait(cps):
        for cp in cps:
            cp.wait()

    def pin(x):
        x = link(pltpu.bitcast(x, F32))
        mark(x, True)
        return pltpu.bitcast(x, U32)

    def hook(x):
        chain[-1] = pltpu.bitcast(pltpu.bitcast(chain[-1], U32) | x, F32)

    def x_prep(par, u):
        for e in range(GPI):
            g = u * GPI + e
            for b in range(8):
                xv = pltpu.bitcast(xb[par, b * 32:(b + 1) * 32, pl.ds(pl.multiple_of(g * 128, 128), 128)], U32)
                xn[e, b * PITCH:b * PITCH + 8, :] = pin(xv[:8])
                xn[e, b * PITCH + 8:b * PITCH + 16, :] = xv[8:]
                yield
        for e in range(GPI):
            for n in range(16):
                xs[par][u * GPI + e, n * 8:(n + 1) * 8, :] = pin(xn[e, pl.ds(n, 8, stride=PITCH), :])
                yield

    def a_fwd(par, t, u):
        ch = pl.ds(pl.multiple_of(t * 128, 128), 128)
        skt = sk_ref[:, ch].astype(F32)
        skt = [jnp.broadcast_to(skt[j:j + 1, :], (8, 128)) for j in range(4)]
        kvs, hch = [], []
        for cc in range(PER):
            r = pl.multiple_of((u * PER + cc) * CH, CH)
            kf[pl.ds(8 + r, CH), :] = kb[par, pl.ds(r, CH), :].astype(F32)
            vv = vb[par, pl.ds(r, CH), :].astype(F32)
            kv = []
            for f in range(0, CH, 8):
                k0 = kf[pl.ds(8 + r + f, 8), :]
                if f % 16 == 0:
                    tk = link(skt[0])
                pr = [k0 * tk] + [kf[pl.ds(8 + r + f - j, 8), :] * skt[j] for j in range(1, 4)]
                kv.append(((pr[0] + pr[1]) + (pr[2] + pr[3])) * vv[f:f + 8])
                if f % 16 == 8:
                    mark(kv[-1 - (f // 16) % 2])
            kvs.append(_cat(kv, 0))
            hch.append(hb[par, :, pl.ds(r, CH)])
        fw = fw_ref[...]
        hh = lax.dot_general(fw, _cat(hch, 0), (((1,), (1,)), ((), ())), preferred_element_type=F32)
        uu = jnp.dot(fw, _cat(kvs, 1).astype(BF16), preferred_element_type=F32)
        dvec = ddf[pl.ds(t, 1), :]
        dsel = jnp.where(u == 0, dvec, 0.0)
        for f in range(CH // 8):
            t, re, im = slice(8 * f, 8 * f + 8), slice(16 * f, 16 * f + 8), slice(16 * f + 8, 16 * f + 16)
            pc, pd = jnp.where(u == 0, 0.0, hprev[0, t, :]), jnp.where(u == 0, 0.0, hprev[1, t, :])
            for cc in range(PER):
                c, l = u * PER + cc, slice(cc * 128, (cc + 1) * 128)
                hc, hd = hh[re, l], hh[im, l]
                gc = (hc - pd) if f % 2 == 0 else (hc + pd)
                gd = (hd + pc) if f % 2 == 0 else (hd - pc)
                if cc == 0:
                    gc = gc + dsel
                hs[par][c, 0, t, :] = gc
                hs[par][c, 1, t, :] = gd - gc
                hs[par][c, 2, t, :] = gd + gc
                pc, pd = hc, hd
                us[par][c, 0, t, :] = uu[re, l] + uu[im, l]
                us[par][c, 1, t, :] = uu[re, l]
                us[par][c, 2, t, :] = uu[im, l]
            hprev[0, t, :] = pc
            hprev[1, t, :] = pd
        return uu

    def a_conv(par, u, ff, m):
        t0 = pl.ds(pl.multiple_of((u * PER + ff) * 8, 8), 8)
        for blk in range(NCH // CB):
            i0 = blk * CB
            t = pl.ds(pl.multiple_of((u * PER + ff + zero(blk)) * 8, 8), 8)
            acc = [None] * CB if m == 0 else [ys[par][i0 + j, 0, t0, :] for j in range(CB)]
            win = {}
            for c in range(i0 + CB):
                a = link(us[par][c, m, t, :])
                for j in range(CB):
                    d = i0 + j - c
                    if d < 0:
                        continue
                    if d not in win:
                        win[d] = hs[par][d, m, t, :]
                    pr = a * win[d]
                    acc[j] = pr if acc[j] is None else (acc[j] - pr if m == 2 else acc[j] + pr)
                mark(acc[c % CB], c >= i0)
            for j in range(CB):
                ys[par][i0 + j, m % 2, t0, :] = acc[j]
            next(cur['side'], None)

    def a_inv(par, u):
        yy = _cat([_cat([ys[par][u * PER + cc, 0], ys[par][u * PER + cc, 1]], 0) for cc in range(PER)], 1).astype(BF16)
        y = jnp.dot(_cat([iv_ref[0], iv_ref[1]], 1), yy, preferred_element_type=F32)
        for cc in range(PER):
            r = pl.multiple_of((u * PER + cc) * CH, CH)
            oa_buf[par, pl.ds(r, CH), :] = (
                y[:, cc * 128:(cc + 1) * 128] * qb[par, pl.ds(r, CH), :].astype(F32)).astype(BF16)

    def history(dst, par, g, first):
        top = lax.broadcasted_iota(jnp.int32, (8, 128), 0) < 2
        for j in range(HIST // RT):
            o = TM + RT * j
            prev = 0.0 if first else dst[1 - par][g, o + 14:o + 22, :]
            dst[par][g, RT * j:RT * j + 8, :] = jnp.where(top, prev, dst[par][g, o - 2:o + 6, :])
            dst[par][g, RT * j + 8:RT * j + 16, :] = dst[par][g, o + 6:o + 14, :]

    def b_qkv(par, sec, g):
        x = _bf([xs[par][c] for c in range(NG)])
        r = jnp.dot(x, _bf([w_p[sec * NG + g], w_p[sec * NG + g + 1]]), preferred_element_type=F32)
        for e in range(2):
            rr = r[:, e * 128:(e + 1) * 128]
            if sec == 0:
                qs[par][g + e, 0:TM, :] = rr
            else:
                (ks, vs)[sec - 1][par][g + e, HIST:HIST + TM, :] = rr
                history((ks, vs)[sec - 1], par, g + e, False)

    def b_qkv0(sec, u):
        x = _bf([xs0[GPI * u + e] for e in range(GPI)])
        k = pl.ds(pl.multiple_of(u * 128, 128), 128)
        dst, o = (qs0, ks0, vs0)[sec], HIST if sec else 0
        for g in range(0, NG, 2):
            r = jnp.dot(x, _bf([w_p[sec * NG + g + e, k, :] for e in range(2)]), preferred_element_type=F32)
            for e in range(2):
                dst[g + e, o:o + TM, :] = jnp.where(u == 0, 0.0, dst[g + e, o:o + TM, :]) + r[:, e * 128:(e + 1) * 128]

    def b_qk(par, u, tt, first):
        lane = lax.broadcasted_iota(jnp.int32, (RT, 128), 1)
        b4, b0 = (lane & 16) != 0, (lane & 1) != 0
        cexp = float(DH ** -0.5 * np.log2(np.e))
        r0 = pl.multiple_of((u * PER + tt) * RT, RT)
        acc = [[None] * WIN for _ in range(2)]
        for wg in range(0, WIN, CB):
            for hf in range(2):
                rq = pl.ds(pl.multiple_of(r0 + 8 * hf + 8 * zero(wg), 8), 8)
                for g in range(NG):
                    q = link(qs[par][g, rq, :], 1)
                    for w in range(wg, wg + CB):
                        pr = q * ks[par][g, pl.ds(HIST + r0 - RT * w + 8 * hf, 8), :]
                        acc[hf][w] = pr if g == 0 else acc[hf][w] + pr
                    if g < NG - 1:
                        mark(acc[hf][wg + g % CB])
                for w in range(wg, wg + CB):
                    mark(acc[hf][w], True)
        lg = [jnp.concatenate([acc[0][w], acc[1][w]], axis=0) for w in range(WIN)]
        lg = [l + jnp.where(b4, pltpu.roll(l, 16, 1), pltpu.roll(l, 112, 1)) for l in lg]
        lg = [l + jnp.where(b0, pltpu.roll(l, 1, 1), pltpu.roll(l, 127, 1)) for l in lg]
        if first:
            pair = (lax.broadcasted_iota(jnp.int32, (RT, 128), 0) // DIL) * RT + (u * PER + tt)
            lg = [jnp.where(pair >= w, lg[w], -1e9 * DH ** 0.5) for w in range(WIN)]
        m = lg[0]
        for w in range(1, WIN):
            m = jnp.maximum(m, lg[w])
        p = [jnp.exp2((l - m) * cexp) for l in lg]
        den = p[0]
        for w in range(1, WIN):
            den = den + p[w]
        inv = pl.reciprocal(den, approx=True)
        inv = inv * (2.0 - den * inv)
        return [e * inv for e in p]

    def b_pv(par, u, tt, p, dst):
        r0 = pl.multiple_of((u * PER + tt) * RT, RT)
        for gg in range(0, NG, CB):
            acc = [[None] * CB for _ in range(2)]
            for hf in range(2):
                for w in range(WIN):
                    pw = link(p[w][8 * hf:8 * hf + 8], 2)
                    for j in range(CB):
                        pr = pw * vs[par][gg + j, pl.ds(HIST + r0 - RT * w + 8 * hf, 8), :]
                        acc[hf][j] = pr if w == 0 else acc[hf][j] + pr
                    if w < WIN - 1:
                        mark(acc[hf][w % CB])
                for j in range(CB):
                    mark(acc[hf][j], True)
            for j in range(CB):
                o = jnp.concatenate([acc[0][j], acc[1][j]], axis=0).astype(BF16)
                dst[gg + j, pl.ds(u * PER + tt, 8, stride=PITCH), :] = pltpu.bitcast(o, U32)

    def b_out(par, g):
        o = _bf([_cat([ob[par][c, b * PITCH:b * PITCH + 16, :] for b in range(8)], 0) for c in range(NG)])
        r = jnp.dot(o, _bf([wo_p[g], wo_p[g + 1]]), preferred_element_type=F32)
        obuf[par, :, pl.ds(pl.multiple_of(g * 128, 256), 256)] = r.astype(BF16)

    def b_half(src, par, k):
        g, h = (k // 2) * 2, k % 2
        o = _bf([_cat([src[c, pl.ds(pl.multiple_of(b * PITCH + 8 * h, 8), 8), :] for b in range(8)], 0)
                 for c in range(NG)])
        r = jnp.dot(o, _bf([wo_p[g], wo_p[g + 1]]), preferred_element_type=F32).astype(BF16)
        for b in range(8):
            obuf[par, pl.ds(pl.multiple_of(b * 32 + 16 * h, 16), 16), pl.ds(pl.multiple_of(g * 128, 256), 256)] = (
                r[b * 16:(b + 1) * 16])

    def loop(fn, lb=1, unr=1, slow=(0, 0, 0), lo=0, hi=NI):
        def body(u, carry):
            chain[:] = []
            lane = lax.broadcasted_iota(jnp.int32, (8, 128), 1)
            cur.update(lb=max(lb, 1), u=u, link=lb > 0, lane=lane, never=lane > u + 1000,
                       n=0, slow=slow)
            for j in range(unr):
                fn(u * unr + j)
            return carry
        lax.fori_loop(lo // unr, hi // unr, body, 0)

    def step(s, par, s1, s2, s3, first2=False, tail=0):
        def body(u):
            cur['side'] = x_prep(1 - par, u) if s1 else iter(())
            if first2:
                wait([wo_copy(u)] + early_in(1, u))
                issue(3, u)
                cur['side'] = itertools.zip_longest(cur['side'], _permute_rows(wo_r, wo_tmp, wo_p, u, hook))
            mm = []
            if s1:
                mm += [lambda sec=sec: b_qkv(par, sec, u * GPI) for sec in range(3)]
            if s3:
                units = {0: [], 1: [(ob0, 0, 3 * u + j) for j in range(3)],
                         2: [(ob0, 0, u + 4), (ob1, 1, 4 * u - 8), (ob1, 1, 4 * u - 6)], 3: [(ob2, 1, 2 * u + 1)]}[tail]
                mm += [lambda a=a: b_half(*a) for a in units] if tail else [lambda: b_out(par, u * GPI)]
                a_inv(par, u)
            for i in range(PER):
                if i < len(mm):
                    mm[i]()
                if s2:
                    p = b_qk(1 - par, u, i, first2)
                    for m in range(3):
                        a_conv(1 - par, u, i, m)
                    b_pv(1 - par, u, i, p, ob2 if tail == 2 else ob[1 - par])
                if s1 and i == (FW1 if first2 else FW2):
                    a_fwd(par, s, u)
            if s1 and not first2 and FW2 == 4:
                gate(a_fwd(par, s, u))
            if not s2:
                start(out_copies(s, par, u))

        loop(body, 1 if s1 else L8, UNR if (s1 and s3) else 1,
             SLOW if (s1 and s3) else (0, 0, 0), 2 if tail == 2 else 0, 2 if tail == 1 else NI)
        if s3 and not tail:
            start(out_copies(s, par))

    def x0_in(n):
        c = pl.ds(pl.multiple_of(n * 256, 256), 256)
        return [pltpu.make_async_copy(x_hbm.at[0:TM, c], xb.at[0, :, c], isem.at[14 + n])]

    start(w_copy(0) + x0_in(0))
    kf[0:8, :] = jnp.zeros((8, 128), F32)
    if not EARLY:
        wait(x0_in(0))
    for n in range(1, LA):
        start(w_copy(n) + x0_in(n))
    if EARLY:
        wait(x0_in(0))
    small = [pltpu.make_async_copy(a, b, isem.at[10 + i]) for i, (a, b) in enumerate(
        [(sk_hbm, sk_ref), (dd_hbm, dd_ref), (fw_hbm, fw_ref), (iv_hbm, iv_ref)])]
    extra = {n - LA: x0_in(n) for n in range(LA + 1, NI)}
    later = ([small] + [early_in(t, u) for t in range(2) for u in range(NI)] + [[wo_copy(n)] for n in range(4)]
             + [a_in(2, 0), x_in(3, 1) + q_in(0, 0)])
    for n, cps in zip(EXT, later):
        extra[n] = extra.get(n, []) + cps

    def issue(ph, u):
        for j in range(NI):
            if ph * 4 + j + 1 in extra:
                pl.when(u == j)(lambda j=j: start(extra[ph * 4 + j + 1]))

    def head(ph, u):
        n = ph * 4 + u + 1
        if ph == 0:
            pl.when(n < NI)(lambda: wait(x0_in(jnp.minimum(n, NI - 1))))
        if ph < 2:
            wait(w_copy(n))
        else:
            pl.when(n < 12)(lambda: wait(w_copy(jnp.minimum(n, 11))))
            wait(early_in(0, u))
        if ph * 4 + 1 + LA < 12:
            pl.when(n + LA < 12)(lambda: start(w_copy(jnp.minimum(n + LA, 11))))
        issue(ph, u)
        b_qkv0(2 - ph, u)
        n = jnp.minimum(n, 11)
        _permute_cols(w_r, w_p, 2 - n // 4, n % 4)
        if ph > 0:
            for e in range(GPI):
                history((vs, ks)[ph - 1], 0, GPI * u + e, True)
        if ph == 2:
            a_fwd(0, 0, u)
        if ph != 1:
            list(x_prep(ph // 2, u if ph else jnp.minimum(u + 1, NI - 1)))

    cur.update(lb=1, link=False)
    list(x_prep(0, 0))
    wait(w_copy(0))
    start(w_copy(LA) + x0_in(LA))
    _permute_cols(w_r, w_p, 2, 0)
    for ph in range(3):
        if ph == 2:
            wait(small)
            ddf[...] = dd_ref[...].astype(F32)
        loop(lambda u, ph=ph: head(ph, u), 0)

    step(1, 1, True, True, False, first2=True)

    def steady(j, carry):
        for par in range(2):
            s = 2 * j + par
            wait(a_in(s, par) + q_in(s - 2, par))
            start(q_in(s - 1, 1 - par))

            if par == 0:
                wait(x_in(s + 1, 1))
                start(a_in(s + 1, 1))

            @pl.when(j < NG // 2 - 1)
            def _():
                if par == 1:
                    wait(x_in(s + 1, 0))
                    start(a_in(s + 1, 0))
                start(x_in(s + 2, par))

            @pl.when(j > 1)
            def _():
                wait(out_copies(s - 2, par))
            step(s, par, True, True, True)
        return carry

    lax.fori_loop(1, NG // 2, steady, 0)
    wait(q_in(NG - 2, 0) + out_copies(NG - 2, 0))
    start(q_in(NG - 1, 1))
    last = [out_copies(NG + par, par, u) for par in range(2) for u in range(NI)]
    step(NG, 0, False, True, True, tail=1)
    start(last[0] + last[1] + last[2][1:])
    wait(q_in(NG - 1, 1) + out_copies(NG - 1, 1))
    step(NG, 0, False, True, True, tail=2)
    start(last[2][:1] + last[3])
    step(NG + 1, 1, False, False, True, tail=3)
    wait(sum(last, []))


@jax.jit
def pallas_concat_heads__ssm_conv_h3__sliding_local_dilated__prompt_kernel(
    A_q, A_k, A_v, A_shift_k, A_ssm_k, A_ssm_D, B_x, B_wqkv, B_wo,
):
    fw, iv = _dft_mats()
    sp3, sp2 = pltpu.VMEM((NCH, 3, CH + 8, 128), F32), pltpu.VMEM((NCH, 2, CH, 128), F32)
    qsp, ksp = pltpu.VMEM((NG, TM + 8, 128), F32), pltpu.VMEM((NG, HIST + TM + 8, 128), F32)
    xsp, osp = pltpu.VMEM((NG, TM // 2, 128), U32), pltpu.VMEM((NG, 8 * PITCH, 128), U32)
    col = pltpu.VMEM((2, S, 128), BF16)
    hbm = pl.BlockSpec(memory_space=pl.ANY)
    out = pl.pallas_call(
        _kernel,
        in_specs=[hbm] * 11,
        out_specs=hbm,
        out_shape=jax.ShapeDtypeStruct((S, 2 * D), BF16),
        scratch_shapes=[
            pltpu.VMEM((4, D), BF16), pltpu.VMEM((NG, 128), BF16), pltpu.VMEM(fw.shape, BF16), pltpu.VMEM(iv.shape, BF16),
            pltpu.VMEM((3, D, D), BF16), pltpu.VMEM((4, D, 256), BF16),
            pltpu.VMEM((3 * NG, D // 2, 128), U32), pltpu.VMEM((NG, D // 2, 128), U32),
            pltpu.VMEM((2, 8 * 72, 128), U32),
            col, col, col, pltpu.VMEM((2, 128, S), BF16), pltpu.VMEM((2, TM, D), BF16),
            pltpu.VMEM((8 + S, 128), F32), pltpu.VMEM((GPI, 8 * PITCH, 128), U32), xsp, xsp,
            pltpu.VMEM((2, CH, 128), F32), pltpu.VMEM((NG, 128), F32),
            sp3, sp3, sp3, sp3, sp2, sp2, qsp, qsp, ksp, ksp, ksp, ksp, osp, osp, osp,
            col, pltpu.VMEM((2, TM, D), BF16),
            pltpu.SemaphoreType.DMA((16,)), pltpu.SemaphoreType.DMA((26,)),
            pltpu.SemaphoreType.DMA((4 + 4 * NI,)),
        ],
        compiler_params=pltpu.CompilerParams(vmem_limit_bytes=100 * 2 ** 20),
    )(A_q.reshape(S, D), A_k.reshape(S, D), A_v.reshape(S, D), A_shift_k.T, A_ssm_k,
      A_ssm_D.reshape(NG, 128), B_x.reshape(S, D), B_wqkv, B_wo, fw, iv)
    return out.reshape(1, S, 2 * D)
```

```python
import itertools

import numpy as np
import jax
import jax.numpy as jnp
from jax import lax
import jax.experimental.pallas as pl
import jax.experimental.pallas.tpu as pltpu

S = 2048
D = 1024
NG = D // 128
CH = 128
NCH = S // CH
TM = S // NG
HIST = 112
PITCH = 24
WIN, DIL, DH = 8, 2, 32
RT = 16
NI = 4
PER = NCH // NI
CB = 4
UNR = 2
LA = 3
SUB = 2
EXT = (1, 4, 6, 8, 9, 10, 11, 12, 13, 10, 11, 12, 13, 14, 14)
FW0 = 2
FW1 = 2
L8 = 2
SLOW = 2
GPI = NG // NI
F32, BF16, U32 = jnp.float32, jnp.bfloat16, jnp.uint32


def _dft_mats():
    r = np.arange(CH)
    k = (16 * (r // 16) + 2 * (r % 8) + (r // 8) % 2).astype(np.float64)
    th = 2.0 * np.pi * (k + 0.5) / (2 * CH)
    ang = th[:, None] * np.arange(CH, dtype=np.float64)[None, :]
    fwd = np.concatenate([np.cos(ang), -np.sin(ang)], axis=0)
    inv = fwd.T / CH
    fwd = fwd.reshape(2, CH // 8, 8, CH).transpose(1, 0, 2, 3).reshape(2 * CH, CH)
    return jnp.asarray(fwd, BF16), jnp.asarray(np.stack([inv[:, :CH], inv[:, CH:]]), BF16)


def _permute_cols(w_ref, wp_ref, sec, q):
    lane = lax.broadcasted_iota(jnp.int32, (8, 128), 1)
    bits = [(lane & (2 << st)) != 0 for st in range(3)]

    def first(i):
        r = pl.ds(pl.multiple_of(q * 256 + i * 16, 16), 16)
        v = [pltpu.bitcast(w_ref[sec, r, g * 128:(g + 1) * 128], U32) for g in range(NG)]
        return [v[0]] + [pltpu.roll(v[g], 2 * g, 1) for g in range(1, NG)]

    def second(i, v):
        t = [v[(-e) % NG] for e in range(NG)]
        for st in range(3):
            t = [jnp.where(bits[st], t[(e - (1 << st)) % NG], t[e]) for e in range(NG)]
        t = [t[0]] + [pltpu.roll(t[e], 128 - 2 * e, 1) for e in range(1, NG)]
        for e in range(NG):
            wp_ref[sec * NG + e, pl.ds(pl.multiple_of(q * 128 + i * 8, 8), 8), :] = t[e]

    ahead = 2
    vs = [first(i) for i in range(ahead)]
    for i in range(16):
        if i + ahead < 16:
            vs.append(first(i + ahead))
        second(i, vs[i])


def _permute_rows(wo_ref, tmp_ref, wp_ref, q, hook):
    def anchor(t):
        hook(((t[0] | t[1]) | (t[2] | t[3])) | ((t[4] | t[5]) | (t[6] | t[7])))

    for e in range(2):
        for b in range(8):
            w = pltpu.bitcast(wo_ref[q, b * 128:(b + 1) * 128, e * 128:(e + 1) * 128], U32)
            anchor([w[m * 8:m * 8 + 8] for m in range(8)])
            tmp_ref[e, b * 72:b * 72 + 64, :] = w
            yield
        for a in range(8):
            t = [tmp_ref[e, pl.ds(m * 8 + a, 8, stride=72), :] for m in range(8)]
            anchor(t)
            wp_ref[2 * q + e, a * 64:(a + 1) * 64, :] = jnp.concatenate(t, axis=0)
            yield


def _cat(parts, axis):
    return parts[0] if len(parts) == 1 else jnp.concatenate(parts, axis=axis)


def _bf(parts):
    return jnp.concatenate([pltpu.bitcast(x, BF16) for x in parts], axis=1)


def _kernel(q_hbm, k_hbm, v_hbm, sk_hbm, h_hbm, dd_hbm, x_hbm, w_hbm, wo_hbm, fw_hbm, iv_hbm,
            o_hbm,
            sk_ref, dd_ref, fw_ref, iv_ref,
            w_r, wo_r, w_p, wo_p, wo_tmp, qb, kb, vb, hb, xb, kf, xn, xs0, xs1, hprev, ddf,
            us0, us1, hs0, hs1, ys0, ys1, qs0, qs1, ks0, ks1, vs0, vs1, ob0, ob1, ob2,
            oa_buf, obuf, wsem, isem, osem):
    us, hs, ys, xs = (us0, us1), (hs0, hs1), (ys0, ys1), (xs0, xs1)
    qs, ks, vs, ob = (qs0, qs1), (ks0, ks1), (vs0, vs1), (ob0, ob1)
    cur = {}

    chain = []

    def link(x):
        if len(chain) < cur['lb'] or not cur['link']:
            return x
        y = jnp.where(cur['never'], chain.pop(0), x)
        cur['n'] += cur['slow']
        for k in range(cur['n'] // 8):
            y = jnp.where(cur['lane'] > cur['u'] + 1002 + k, x, y)
        cur['n'] %= 8
        return y

    def mark(x, must=False):
        if must or len(chain) < cur['lb']:
            chain.append(x)

    def zero(i):
        return lax.shift_right_logical(cur['u'] + i, 8) if cur['link'] else 0

    def gate(r):
        t = r[r.shape[0] - 8:, r.shape[1] - 128:]
        chain[:] = [jnp.where(cur['lane'] > cur['u'] + 1001, t, y) for y in chain]

    def out_copies(step, par, u=None):
        t = step - 2
        n, k = (1, 2 * par) if u is None else (NI, 4 + 2 * (NI * par + u))
        ra = pl.ds(0 if u is None else pl.multiple_of(u * (S // n), S // n), S // n)
        cb = 0 if u is None else pl.multiple_of(u * (D // n), D // n)
        return [pltpu.make_async_copy(oa_buf.at[par, ra], o_hbm.at[ra, pl.ds(pl.multiple_of(t * 128, 128), 128)],
                                      osem.at[k]),
                pltpu.make_async_copy(obuf.at[par, :, pl.ds(cb, D // n)],
                                      o_hbm.at[pl.ds(pl.multiple_of(t * TM, TM), TM), pl.ds(D + cb, D // n)],
                                      osem.at[k + 1])]

    def w_copy(n):
        sec, m = 2 - n // 4, 256 // SUB
        rows = [pl.ds(pl.multiple_of((n % 4) * 256 + j * m, m), m) for j in range(SUB)]
        return [pltpu.make_async_copy(w_hbm.at[r, pl.ds(pl.multiple_of(sec * D, D), D)], w_r.at[sec, r], wsem.at[n])
                for r in rows]

    def wo_copy(n):
        return pltpu.make_async_copy(wo_hbm.at[:, pl.ds(pl.multiple_of(n * 256, 256), 256)], wo_r.at[n],
                                     wsem.at[12 + n])

    def a_in(t, par):
        c = pl.ds(pl.multiple_of(t * 128, 128), 128)
        return [pltpu.make_async_copy(k_hbm.at[:, c], kb.at[par], isem.at[par * 5]),
                pltpu.make_async_copy(v_hbm.at[:, c], vb.at[par], isem.at[par * 5 + 1]),
                pltpu.make_async_copy(h_hbm.at[c, :], hb.at[par], isem.at[par * 5 + 2])]

    def early_in(t, u):
        c, sem = pl.ds(t * 128, 128), isem.at[18 + NI * t + u]
        r, xc = pl.ds(pl.multiple_of(u * (S // NI), 128), S // NI), pl.ds(pl.multiple_of(u * 256, 256), 256)
        return [pltpu.make_async_copy(k_hbm.at[r, c], kb.at[t, r], sem),
                pltpu.make_async_copy(v_hbm.at[r, c], vb.at[t, r], sem),
                pltpu.make_async_copy(h_hbm.at[c, r], hb.at[t, :, r], sem),
                pltpu.make_async_copy(x_hbm.at[pl.ds((t + 1) * TM, TM), xc], xb.at[1 - t, :, xc], sem)]

    def q_in(t, par):
        return [pltpu.make_async_copy(q_hbm.at[:, pl.ds(pl.multiple_of(t * 128, 128), 128)], qb.at[par],
                                      isem.at[par * 5 + 3])]

    def x_in(t, par):
        return [pltpu.make_async_copy(x_hbm.at[pl.ds(pl.multiple_of(t * TM, TM), TM), :], xb.at[par],
                                      isem.at[par * 5 + 4])]

    def start(cps):
        for cp in cps:
            cp.start()

    def wait(cps):
        for cp in cps:
            cp.wait()

    def pin(x):
        x = link(pltpu.bitcast(x, F32))
        mark(x, True)
        return pltpu.bitcast(x, U32)

    def hook(x):
        chain[-1] = pltpu.bitcast(pltpu.bitcast(chain[-1], U32) | x, F32)

    def x_prep(par, u):
        for e in range(GPI):
            g = u * GPI + e
            for b in range(8):
                xv = pltpu.bitcast(xb[par, b * 32:(b + 1) * 32, pl.ds(pl.multiple_of(g * 128, 128), 128)], U32)
                xn[e, b * PITCH:b * PITCH + 8, :] = pin(xv[:8])
                xn[e, b * PITCH + 8:b * PITCH + 16, :] = xv[8:]
                yield
        for e in range(GPI):
            for n in range(16):
                xs[par][u * GPI + e, n * 8:(n + 1) * 8, :] = pin(xn[e, pl.ds(n, 8, stride=PITCH), :])
                yield

    def a_fwd(par, t, u):
        ch = pl.ds(pl.multiple_of(t * 128, 128), 128)
        skt = sk_ref[:, ch].astype(F32)
        skt = [jnp.broadcast_to(skt[j:j + 1, :], (8, 128)) for j in range(4)]
        kvs, hch = [], []
        for cc in range(PER):
            r = pl.multiple_of((u * PER + cc) * CH, CH)
            kf[pl.ds(8 + r, CH), :] = kb[par, pl.ds(r, CH), :].astype(F32)
            vv = vb[par, pl.ds(r, CH), :].astype(F32)
            kv = []
            for f in range(0, CH, 8):
                k0 = kf[pl.ds(8 + r + f, 8), :]
                if f % 16 == 0:
                    tk = link(skt[0])
                pr = [k0 * tk] + [kf[pl.ds(8 + r + f - j, 8), :] * skt[j] for j in range(1, 4)]
                kv.append(((pr[0] + pr[1]) + (pr[2] + pr[3])) * vv[f:f + 8])
                if f % 16 == 8:
                    mark(kv[-1 - (f // 16) % 2])
            kvs.append(_cat(kv, 0))
            hch.append(hb[par, :, pl.ds(r, CH)])
        fw = fw_ref[...]
        hh = lax.dot_general(fw, _cat(hch, 0), (((1,), (1,)), ((), ())), preferred_element_type=F32)
        uu = jnp.dot(fw, _cat(kvs, 1).astype(BF16), preferred_element_type=F32)
        dvec = ddf[pl.ds(t, 1), :]
        dsel = jnp.where(u == 0, dvec, 0.0)
        for f in range(CH // 8):
            t, re, im = slice(8 * f, 8 * f + 8), slice(16 * f, 16 * f + 8), slice(16 * f + 8, 16 * f + 16)
            pc, pd = jnp.where(u == 0, 0.0, hprev[0, t, :]), jnp.where(u == 0, 0.0, hprev[1, t, :])
            for cc in range(PER):
                c, l = u * PER + cc, slice(cc * 128, (cc + 1) * 128)
                hc, hd = hh[re, l], hh[im, l]
                gc = (hc - pd) if f % 2 == 0 else (hc + pd)
                gd = (hd + pc) if f % 2 == 0 else (hd - pc)
                if cc == 0:
                    gc = gc + dsel
                hs[par][c, 0, t, :] = gc
                hs[par][c, 1, t, :] = gd - gc
                hs[par][c, 2, t, :] = gd + gc
                pc, pd = hc, hd
                us[par][c, 0, t, :] = uu[re, l] + uu[im, l]
                us[par][c, 1, t, :] = uu[re, l]
                us[par][c, 2, t, :] = uu[im, l]
            hprev[0, t, :] = pc
            hprev[1, t, :] = pd
        return uu

    def a_conv(par, u, ff, m):
        t0 = pl.ds(pl.multiple_of((u * PER + ff) * 8, 8), 8)
        for blk in range(NCH // CB):
            i0 = blk * CB
            t = pl.ds(pl.multiple_of((u * PER + ff + zero(blk)) * 8, 8), 8)
            acc = [None] * CB if m == 0 else [ys[par][i0 + j, 0, t0, :] for j in range(CB)]
            win = {}
            for c in range(i0 + CB):
                a = link(us[par][c, m, t, :])
                for j in range(CB):
                    d = i0 + j - c
                    if d < 0:
                        continue
                    if d not in win:
                        win[d] = hs[par][d, m, t, :]
                    pr = a * win[d]
                    acc[j] = pr if acc[j] is None else (acc[j] - pr if m == 2 else acc[j] + pr)
                mark(acc[c % CB], c >= i0)
            for j in range(CB):
                ys[par][i0 + j, m % 2, t0, :] = acc[j]
            next(cur['side'], None)

    def a_inv(par, u):
        yy = _cat([_cat([ys[par][u * PER + cc, 0], ys[par][u * PER + cc, 1]], 0) for cc in range(PER)], 1).astype(BF16)
        y = jnp.dot(_cat([iv_ref[0], iv_ref[1]], 1), yy, preferred_element_type=F32)
        for cc in range(PER):
            r = pl.multiple_of((u * PER + cc) * CH, CH)
            oa_buf[par, pl.ds(r, CH), :] = (
                y[:, cc * 128:(cc + 1) * 128] * qb[par, pl.ds(r, CH), :].astype(F32)).astype(BF16)

    def history(dst, par, g, first):
        top = lax.broadcasted_iota(jnp.int32, (8, 128), 0) < 2
        for j in range(HIST // RT):
            o = TM + RT * j
            prev = 0.0 if first else dst[1 - par][g, o + 14:o + 22, :]
            dst[par][g, RT * j:RT * j + 8, :] = jnp.where(top, prev, dst[par][g, o - 2:o + 6, :])
            dst[par][g, RT * j + 8:RT * j + 16, :] = dst[par][g, o + 6:o + 14, :]

    def b_qkv(par, sec, g):
        x = _bf([xs[par][c] for c in range(NG)])
        r = jnp.dot(x, _bf([w_p[sec * NG + g], w_p[sec * NG + g + 1]]), preferred_element_type=F32)
        for e in range(2):
            rr = r[:, e * 128:(e + 1) * 128]
            if sec == 0:
                qs[par][g + e, 0:TM, :] = rr
            else:
                (ks, vs)[sec - 1][par][g + e, HIST:HIST + TM, :] = rr
                history((ks, vs)[sec - 1], par, g + e, False)

    def b_qkv0(sec, u):
        x = _bf([xs0[GPI * u + e] for e in range(GPI)])
        k = pl.ds(pl.multiple_of(u * 128, 128), 128)
        dst, o = (qs0, ks0, vs0)[sec], HIST if sec else 0
        for g in range(0, NG, 2):
            if sec == 0 and g == FW0:
                a_fwd(0, 0, u)
            r = jnp.dot(x, _bf([w_p[sec * NG + g + e, k, :] for e in range(2)]), preferred_element_type=F32)
            for e in range(2):
                dst[g + e, o:o + TM, :] = jnp.where(u == 0, 0.0, dst[g + e, o:o + TM, :]) + r[:, e * 128:(e + 1) * 128]

    def b_qk(par, u, tt, first):
        lane = lax.broadcasted_iota(jnp.int32, (RT, 128), 1)
        b4, b0 = (lane & 16) != 0, (lane & 1) != 0
        cexp = float(DH ** -0.5 * np.log2(np.e))
        r0 = pl.multiple_of((u * PER + tt) * RT, RT)
        acc = [[None] * WIN for _ in range(2)]
        for wg in range(0, WIN, CB):
            for hf in range(2):
                rq = pl.ds(pl.multiple_of(r0 + 8 * hf + 8 * zero(wg), 8), 8)
                for g in range(NG):
                    q = link(qs[par][g, rq, :])
                    for w in range(wg, wg + CB):
                        pr = q * ks[par][g, pl.ds(HIST + r0 - RT * w + 8 * hf, 8), :]
                        acc[hf][w] = pr if g == 0 else acc[hf][w] + pr
                    if g < NG - 1:
                        mark(acc[hf][wg + g % CB])
                for w in range(wg, wg + CB):
                    mark(acc[hf][w], True)
        lg = [jnp.concatenate([acc[0][w], acc[1][w]], axis=0) for w in range(WIN)]
        lg = [l + jnp.where(b4, pltpu.roll(l, 16, 1), pltpu.roll(l, 112, 1)) for l in lg]
        lg = [l + jnp.where(b0, pltpu.roll(l, 1, 1), pltpu.roll(l, 127, 1)) for l in lg]
        if first:
            pair = (lax.broadcasted_iota(jnp.int32, (RT, 128), 0) // DIL) * RT + (u * PER + tt)
            lg = [jnp.where(pair >= w, lg[w], -1e9 * DH ** 0.5) for w in range(WIN)]
        m = lg[0]
        for w in range(1, WIN):
            m = jnp.maximum(m, lg[w])
        p = [jnp.exp2((l - m) * cexp) for l in lg]
        den = p[0]
        for w in range(1, WIN):
            den = den + p[w]
        inv = pl.reciprocal(den, approx=True)
        inv = inv * (2.0 - den * inv)
        return [e * inv for e in p]

    def b_pv(par, u, tt, p, dst):
        r0 = pl.multiple_of((u * PER + tt) * RT, RT)
        for gg in range(0, NG, CB):
            acc = [[None] * CB for _ in range(2)]
            for hf in range(2):
                for w in range(WIN):
                    pw = link(p[w][8 * hf:8 * hf + 8])
                    for j in range(CB):
                        pr = pw * vs[par][gg + j, pl.ds(HIST + r0 - RT * w + 8 * hf, 8), :]
                        acc[hf][j] = pr if w == 0 else acc[hf][j] + pr
                    if w < WIN - 1:
                        mark(acc[hf][w % CB])
                for j in range(CB):
                    mark(acc[hf][j], True)
            for j in range(CB):
                o = jnp.concatenate([acc[0][j], acc[1][j]], axis=0).astype(BF16)
                dst[gg + j, pl.ds(u * PER + tt, 8, stride=PITCH), :] = pltpu.bitcast(o, U32)

    def b_out(par, g):
        o = _bf([_cat([ob[par][c, b * PITCH:b * PITCH + 16, :] for b in range(8)], 0) for c in range(NG)])
        r = jnp.dot(o, _bf([wo_p[g], wo_p[g + 1]]), preferred_element_type=F32)
        obuf[par, :, pl.ds(pl.multiple_of(g * 128, 256), 256)] = r.astype(BF16)

    def b_half(src, par, k):
        g, h = (k // 2) * 2, k % 2
        o = _bf([_cat([src[c, pl.ds(pl.multiple_of(b * PITCH + 8 * h, 8), 8), :] for b in range(8)], 0)
                 for c in range(NG)])
        r = jnp.dot(o, _bf([wo_p[g], wo_p[g + 1]]), preferred_element_type=F32).astype(BF16)
        for b in range(8):
            obuf[par, pl.ds(pl.multiple_of(b * 32 + 16 * h, 16), 16), pl.ds(pl.multiple_of(g * 128, 256), 256)] = (
                r[b * 16:(b + 1) * 16])

    def loop(fn, lb=1, unr=1, slow=0, lo=0, hi=NI):
        def body(u, carry):
            chain[:] = []
            lane = lax.broadcasted_iota(jnp.int32, (8, 128), 1)
            cur.update(lb=max(lb, 1), u=u, link=lb > 0, lane=lane, never=lane > u + 1000,
                       n=0, slow=slow)
            for j in range(unr):
                fn(u * unr + j)
            return carry
        lax.fori_loop(lo // unr, hi // unr, body, 0)

    def step(s, par, s1, s2, s3, first2=False, tail=0):
        def body(u):
            cur['side'] = x_prep(1 - par, u) if s1 else iter(())
            if first2:
                wait([wo_copy(u)] + early_in(1, u))
                issue(3, u)
                cur['side'] = itertools.zip_longest(cur['side'], _permute_rows(wo_r, wo_tmp, wo_p, u, hook))
            mm = []
            if s1:
                mm += [lambda sec=sec: b_qkv(par, sec, u * GPI) for sec in range(3)]
            if s3:
                units = {0: [], 1: [(ob0, 0, 3 * u + j) for j in range(3)],
                         2: [(ob0, 0, u + 4), (ob1, 1, 4 * u - 8), (ob1, 1, 4 * u - 6)], 3: [(ob2, 1, 2 * u + 1)]}[tail]
                mm += [lambda a=a: b_half(*a) for a in units] if tail else [lambda: b_out(par, u * GPI)]
                a_inv(par, u)
            for i in range(PER):
                if i < len(mm):
                    mm[i]()
                if s2:
                    p = b_qk(1 - par, u, i, first2)
                    for m in range(3):
                        a_conv(1 - par, u, i, m)
                    b_pv(1 - par, u, i, p, ob2 if tail == 2 else ob[1 - par])
                if first2 and i == FW1:
                    a_fwd(par, s, u)
            if s1 and not first2:
                gate(a_fwd(par, s, u))
            if not s2:
                start(out_copies(s, par, u))

        loop(body, 1 if s1 else L8, UNR if (s1 and s3) else 1,
             SLOW if (s1 and s3) else 0, 2 if tail == 2 else 0, 2 if tail == 1 else NI)
        if s3 and not tail:
            start(out_copies(s, par))

    def x0_in(n):
        c = pl.ds(pl.multiple_of(n * 256, 256), 256)
        return [pltpu.make_async_copy(x_hbm.at[0:TM, c], xb.at[0, :, c], isem.at[14 + n])]

    start(w_copy(0) + x0_in(0))
    kf[0:8, :] = jnp.zeros((8, 128), F32)
    for n in range(1, LA):
        start(w_copy(n) + x0_in(n))
    wait(x0_in(0))
    small = [pltpu.make_async_copy(a, b, isem.at[10 + i]) for i, (a, b) in enumerate(
        [(sk_hbm, sk_ref), (dd_hbm, dd_ref), (fw_hbm, fw_ref), (iv_hbm, iv_ref)])]
    extra = {n - LA: x0_in(n) for n in range(LA + 1, NI)}
    later = ([small] + [early_in(t, u) for t in range(2) for u in range(NI)] + [[wo_copy(n)] for n in range(4)]
             + [a_in(2, 0), x_in(3, 1) + q_in(0, 0)])
    for n, cps in zip(EXT, later):
        extra[n] = extra.get(n, []) + cps

    def issue(ph, u):
        for j in range(NI):
            if ph * 4 + j + 1 in extra:
                pl.when(u == j)(lambda j=j: start(extra[ph * 4 + j + 1]))

    def head(ph, u):
        n = ph * 4 + u + 1
        if ph == 0:
            pl.when(n < NI)(lambda: wait(x0_in(jnp.minimum(n, NI - 1))))
        if ph < 2:
            wait(w_copy(n))
        else:
            pl.when(n < 12)(lambda: wait(w_copy(jnp.minimum(n, 11))))
            wait(early_in(0, u))
        if ph * 4 + 1 + LA < 12:
            pl.when(n + LA < 12)(lambda: start(w_copy(jnp.minimum(n + LA, 11))))
        issue(ph, u)
        b_qkv0(2 - ph, u)
        n = jnp.minimum(n, 11)
        _permute_cols(w_r, w_p, 2 - n // 4, n % 4)
        if ph > 0:
            for e in range(GPI):
                history((vs, ks)[ph - 1], 0, GPI * u + e, True)
        if ph != 1:
            list(x_prep(ph // 2, u if ph else jnp.minimum(u + 1, NI - 1)))

    cur.update(lb=1, link=False)
    list(x_prep(0, 0))
    wait(w_copy(0))
    start(w_copy(LA) + x0_in(LA))
    _permute_cols(w_r, w_p, 2, 0)
    for ph in range(3):
        if ph == 2:
            wait(small)
            ddf[...] = dd_ref[...].astype(F32)
        loop(lambda u, ph=ph: head(ph, u), 0)

    step(1, 1, True, True, False, first2=True)

    def steady(j, carry):
        for par in range(2):
            s = 2 * j + par
            wait(a_in(s, par) + q_in(s - 2, par))
            start(q_in(s - 1, 1 - par))

            if par == 0:
                wait(x_in(s + 1, 1))
                start(a_in(s + 1, 1))

            @pl.when(j < NG // 2 - 1)
            def _():
                if par == 1:
                    wait(x_in(s + 1, 0))
                    start(a_in(s + 1, 0))
                start(x_in(s + 2, par))

            @pl.when(j > 1)
            def _():
                wait(out_copies(s - 2, par))
            step(s, par, True, True, True)
        return carry

    lax.fori_loop(1, NG // 2, steady, 0)
    wait(q_in(NG - 2, 0) + out_copies(NG - 2, 0))
    start(q_in(NG - 1, 1))
    last = [out_copies(NG + par, par, u) for par in range(2) for u in range(NI)]
    step(NG, 0, False, True, True, tail=1)
    start(last[0] + last[1] + last[2][1:])
    wait(q_in(NG - 1, 1) + out_copies(NG - 1, 1))
    step(NG, 0, False, True, True, tail=2)
    start(last[2][:1] + last[3])
    step(NG + 1, 1, False, False, True, tail=3)
    wait(sum(last, []))


@jax.jit
def pallas_concat_heads__ssm_conv_h3__sliding_local_dilated__prompt_kernel(
    A_q, A_k, A_v, A_shift_k, A_ssm_k, A_ssm_D, B_x, B_wqkv, B_wo,
):
    fw, iv = _dft_mats()
    sp3, sp2 = pltpu.VMEM((NCH, 3, CH + 8, 128), F32), pltpu.VMEM((NCH, 2, CH, 128), F32)
    qsp, ksp = pltpu.VMEM((NG, TM + 8, 128), F32), pltpu.VMEM((NG, HIST + TM + 8, 128), F32)
    xsp, osp = pltpu.VMEM((NG, TM // 2, 128), U32), pltpu.VMEM((NG, 8 * PITCH, 128), U32)
    col = pltpu.VMEM((2, S, 128), BF16)
    hbm = pl.BlockSpec(memory_space=pl.ANY)
    out = pl.pallas_call(
        _kernel,
        in_specs=[hbm] * 11,
        out_specs=hbm,
        out_shape=jax.ShapeDtypeStruct((S, 2 * D), BF16),
        scratch_shapes=[
            pltpu.VMEM((4, D), BF16), pltpu.VMEM((NG, 128), BF16), pltpu.VMEM(fw.shape, BF16), pltpu.VMEM(iv.shape, BF16),
            pltpu.VMEM((3, D, D), BF16), pltpu.VMEM((4, D, 256), BF16),
            pltpu.VMEM((3 * NG, D // 2, 128), U32), pltpu.VMEM((NG, D // 2, 128), U32),
            pltpu.VMEM((2, 8 * 72, 128), U32),
            col, col, col, pltpu.VMEM((2, 128, S), BF16), pltpu.VMEM((2, TM, D), BF16),
            pltpu.VMEM((8 + S, 128), F32), pltpu.VMEM((GPI, 8 * PITCH, 128), U32), xsp, xsp,
            pltpu.VMEM((2, CH, 128), F32), pltpu.VMEM((NG, 128), F32),
            sp3, sp3, sp3, sp3, sp2, sp2, qsp, qsp, ksp, ksp, ksp, ksp, osp, osp, osp,
            col, pltpu.VMEM((2, TM, D), BF16),
            pltpu.SemaphoreType.DMA((16,)), pltpu.SemaphoreType.DMA((26,)),
            pltpu.SemaphoreType.DMA((4 + 4 * NI,)),
        ],
        compiler_params=pltpu.CompilerParams(vmem_limit_bytes=100 * 2 ** 20),
    )(A_q.reshape(S, D), A_k.reshape(S, D), A_v.reshape(S, D), A_shift_k.T, A_ssm_k,
      A_ssm_D.reshape(NG, 128), B_x.reshape(S, D), B_wqkv, B_wo, fw, iv)
    return out.reshape(1, S, 2 * D)
```
